```python
import jax
import jax.numpy as jnp

def _softmax(x, axis=-1):
    return jax.nn.softmax(x, axis=axis)

def _gelu(x):
    return jax.nn.gelu(x, approximate=True)

def _silu(x):
    return jax.nn.silu(x)

def _sigmoid(x):
    return jax.nn.sigmoid(x)

def _layernorm(x, axis=-1, eps=1e-05):
    m = jnp.mean(x, axis=axis, keepdims=True)
    v = jnp.var(x, axis=axis, keepdims=True)
    return (x - m) / jnp.sqrt(v + eps)

def _scatter_add(tgt, idx, src, axis=0):
    return tgt.at[idx].add(src)

def _segment_sum(src, seg, n):
    return jax.ops.segment_sum(src, seg, n)

class _Rng:

    def __init__(self, key):
        self._k = key

    def _next(self):
        self._k, sub = jax.random.split(self._k)
        return sub

    def normal(self, shape):
        return jax.random.normal(self._next(), shape, dtype=jnp.bfloat16)

    def randint(self, lo, hi, shape):
        return jax.random.randint(self._next(), shape, lo, hi, dtype=jnp.int32)

    def uniform(self, shape, lo=0.0, hi=1.0):
        return jax.random.uniform(self._next(), shape, jnp.bfloat16, lo, hi)

    def permutation(self, n):
        return jax.random.permutation(self._next(), n)
kernel_name = 'gated_mix__compressed_kv_cla__memory_aug_recurrent_mem_tr__prompt'

def setup_inputs():
    _rng = _Rng(jax.random.key(int.from_bytes(__import__("os").urandom(4), "little")))
    _w = lambda a: (lambda t: t.astype(jnp.bfloat16) if jnp.issubdtype(t.dtype, jnp.floating) else t)(jnp.asarray(a))

    def _A_setup():
        B, H, Sq, Sk, D, M = (1, 32, 2048, 2048, 128, 512)
        Dc = 4 * D
        return {'x': _w((lambda *s: _rng.normal(s) * 0.05)(B, Sq, M)), 'c_kv': _w((lambda *s: _rng.normal(s) * 0.05)(B, Sk, Dc)), 'w_q': _w((lambda *s: _rng.normal(s) * 0.05)(M, H, D) * M ** (-0.5)), 'w_uk': _w((lambda *s: _rng.normal(s) * 0.05)(Dc, H, D) * Dc ** (-0.5)), 'w_uv': _w((lambda *s: _rng.normal(s) * 0.05)(Dc, H, D) * Dc ** (-0.5)), 'w_o': _w((lambda *s: _rng.normal(s) * 0.05)(H, D, M) * (H * D) ** (-0.5))}
    _A_in = _A_setup()

    def _B_setup():
        B, S, Dm = (1, 2048, 512)
        H, Dh = (32, 128)
        M, seg = (8, 32)
        seg = min(seg, S)
        S = S // seg * seg
        return {'x': _w((lambda *s: _rng.normal(s) * 0.05)(B, S, Dm)), 'mem0': _w((lambda *s: _rng.normal(s) * 0.05)(B, M, Dm)), 'Wq': _w((lambda *s: _rng.normal(s) * 0.05)(Dm, H, Dh) * Dm ** (-0.5)), 'Wk': _w((lambda *s: _rng.normal(s) * 0.05)(Dm, H, Dh) * Dm ** (-0.5)), 'Wv': _w((lambda *s: _rng.normal(s) * 0.05)(Dm, H, Dh) * Dm ** (-0.5)), 'Wo': _w((lambda *s: _rng.normal(s) * 0.05)(H, Dh, Dm) * (H * Dh) ** (-0.5)), 'seg_len': seg}
    _B_in = _B_setup()
    return {'A_x': _A_in['x'], 'A_c_kv': _A_in['c_kv'], 'A_w_q': _A_in['w_q'], 'A_w_uk': _A_in['w_uk'], 'A_w_uv': _A_in['w_uv'], 'A_w_o': _A_in['w_o'], 'B_x': _B_in['x'], 'B_mem0': _B_in['mem0'], 'B_Wq': _B_in['Wq'], 'B_Wk': _B_in['Wk'], 'B_Wv': _B_in['Wv'], 'B_Wo': _B_in['Wo'], 'B_seg_len': _B_in['seg_len'], 'gate_w': _w((lambda *s: _rng.normal(s) * 0.05)(512))}

def reference(A_x, A_c_kv, A_w_q, A_w_uk, A_w_uv, A_w_o, B_x, B_mem0, B_Wq, B_Wk, B_Wv, B_Wo, B_seg_len, gate_w):

    def _A_ref(x, c_kv, w_q, w_uk, w_uv, w_o):
        B, Sq, M = (x.shape[0], x.shape[1], x.shape[2])
        Sk = c_kv.shape[1]
        H, D = (w_q.shape[1], w_q.shape[2])
        q = jnp.einsum('bqm,mhd->bhqd', x, w_q)
        k = jnp.einsum('bkc,chd->bhkd', c_kv, w_uk)
        v = jnp.einsum('bkc,chd->bhkd', c_kv, w_uv)
        scores = jnp.einsum('bhqd,bhkd->bhqk', q, k) * D ** (-0.5)
        off = Sk - Sq
        qi = jnp.arange(Sq)[:, None]
        kj = jnp.arange(Sk)[None, :]
        cmask = kj <= qi + off
        scores = jnp.where(cmask[None, None], scores, -1000000000.0)
        p = _softmax(scores, axis=-1)
        ctx = jnp.einsum('bhqk,bhkd->bhqd', p, v)
        return jnp.einsum('bhqd,hdm->bqm', ctx, w_o)

    def _B_ref(x, mem0, Wq, Wk, Wv, Wo, seg_len):
        B, S, Dm = x.shape
        H, Dh = (Wq.shape[1], Wq.shape[2])
        M = mem0.shape[1]
        scale = Dh ** (-0.5)
        n_seg = S // seg_len
        L = M + seg_len
        idx = jnp.arange(L)
        mask = (idx[:, None] < M) | (idx[:, None] >= idx[None, :])
        mem = mem0
        outs = []
        for s in range(n_seg):
            xs = x[:, s * seg_len:(s + 1) * seg_len, :].copy()
            h = jnp.concatenate([mem, xs], axis=1)
            q = jnp.einsum('btd,dhe->bhte', h, Wq)
            k = jnp.einsum('btd,dhe->bhte', h, Wk)
            v = jnp.einsum('btd,dhe->bhte', h, Wv)
            scores = jnp.einsum('bhqe,bhke->bhqk', q, k) * scale
            scores = jnp.where(mask[None, None], scores, -1000000000.0)
            p = _softmax(scores, axis=-1)
            o = jnp.einsum('bhqk,bhke->bhqe', p, v)
            o = jnp.einsum('bhte,hed->btd', o, Wo)
            mem = o[:, :M, :].copy()
            outs.append(o[:, M:, :])
        return jnp.concatenate(outs, axis=1)
    x = A_x
    g = _sigmoid((x * gate_w).sum(-1, keepdims=True))
    a = _A_ref(x, A_c_kv, A_w_q, A_w_uk, A_w_uv, A_w_o)
    b = _B_ref(x, B_mem0, B_Wq, B_Wk, B_Wv, B_Wo, B_seg_len)
    return g * a + (1 - g) * b
```

```python
import functools

import jax
import jax.numpy as jnp
import jax.experimental.pallas as pl
import jax.experimental.pallas.tpu as pltpu

bf16 = jnp.bfloat16
f32 = jnp.float32
u32 = jnp.uint32

LOG2E = 1.4426950408889634
NEG = -1e9 * LOG2E
NT = (((1,), (1,)), ((), ()))

BQ = 128
PCH = 512
GB = 4
XPAD = 24
XTAIL = 16
APAD = 64


def _as_bf16(words):
    return pltpu.bitcast(words, bf16)


def _recip(l):
    r = pl.reciprocal(l, approx=True)
    return r * (2.0 - l * r)


def _unpack_head(words, par):
    sh = ((1 - par) * 16).astype(u32)
    w = jnp.bitwise_and(jnp.left_shift(words, sh), jnp.uint32(0xFFFF0000))
    return pltpu.bitcast(w, f32).astype(bf16)


def _a_schedule(nq, bpc):
    npc = nq // bpc
    out = []
    pend = [(kind, c) for c in range(npc) for kind in ("k", "q", "v")]
    done = set()

    def need(kind, c):
        while (kind, c) not in done:
            x = pend.pop(0)
            done.add(x)
            out.append(("P" + x[0], x[1]))

    for t in range(nq + 2):
        if t < nq:
            need("k", t // bpc)
            need("q", t // bpc)
            out.append(("S", t))
        tt = t + bpc
        if tt < nq:
            c, k = tt // bpc, tt % bpc
            for kd in ("k", "q", "v")[: (3 * (k + 1) + bpc - 1) // bpc]:
                need(kd, c)
        if 0 <= t - 1 < nq:
            need("v", (t - 1) // bpc)
            out.append(("O", t - 1))
        if 0 <= t - 2 < nq:
            out.append(("F", t - 2))
    assert not pend
    return out


def _make_kernel(S, M, H, D, NM, SEG):
    assert SEG == 32 and NM == 8 and D == 128 and S % PCH == 0 and H % 2 == 0 and H % GB == 0
    NQ = S // BQ
    NPAIR = S // (2 * SEG)
    NG = H // GB
    HD = H * D
    qscale = D ** -0.5 * LOG2E
    a_sched = _a_schedule(NQ, PCH // BQ)

    def kernel(x_hbm, c_hbm, wq_hbm, wk_hbm, wv_hbm, wo_hbm, mem0_hbm,
               bq_hbm, bk_hbm, bv_hbm, bo_hbm, gw_hbm, out_hbm,
               x_s, c_s, acc, q_s, k_s, v_s, st_a, w_a, wo_a, st_b, w_b, wo_b,
               mem0_s, gw_s, mem_s, qkv_s, ox_s, out_s,
               sem_in, sem_a, sem_b, sem_out):
        a_w_hbm = (wk_hbm, wq_hbm, wv_hbm)
        b_w_hbm = (bq_hbm, bk_hbm, bv_hbm)

        def pair_copy(src, stage, sems, t, p):
            return pltpu.make_async_copy(
                src.bitcast(u32).at[:, p, :], stage.at[p % 2, t], sems.at[t])

        def pair_copies(p):
            return ([pair_copy(a_w_hbm[t], st_a, sem_a, t, p) for t in range(3)]
                    + [pair_copy(b_w_hbm[t], st_b, sem_b, t, p) for t in range(3)])

        cp_x = pltpu.make_async_copy(x_hbm.bitcast(u32), x_s.at[XPAD:XPAD + S // 2, :], sem_in.at[0])
        cp_c = pltpu.make_async_copy(c_hbm.bitcast(u32), c_s, sem_in.at[1])
        cp_woa = pltpu.make_async_copy(wo_hbm.bitcast(u32), wo_a, sem_in.at[2])
        cp_wob = pltpu.make_async_copy(bo_hbm.bitcast(u32), wo_b, sem_in.at[3])
        cp_mem = pltpu.make_async_copy(mem0_hbm, mem0_s, sem_in.at[4])
        cp_gw = pltpu.make_async_copy(gw_hbm, gw_s, sem_in.at[5])

        first = pair_copies(0)
        first[0].start()
        cp_c.start()
        first[1].start()
        cp_x.start()
        first[2].start()
        cp_woa.start()
        for cp in first[3:]:
            cp.start()
        cp_mem.start()
        cp_gw.start()
        cp_wob.start()

        x_s[0:XPAD, :] = jnp.zeros((XPAD, M), u32)
        x_s[XPAD + S // 2:XPAD + S // 2 + XTAIL, :] = jnp.zeros((XTAIL, M), u32)
        acc[...] = jnp.zeros(acc.shape, f32)
        ox_s[...] = jnp.zeros(ox_s.shape, f32)

        def unpack_weights(hn):
            slot = (hn // 2) % 2
            par = hn % 2
            for t in range(3):
                w_a[hn % 2, t] = _unpack_head(st_a[slot, t], par)
            for t in range(3):
                w_b[t * (H + 1) + hn] = _unpack_head(st_b[slot, t], par)

        for cp in first:
            cp.wait()
        unpack_weights(jnp.int32(0))
        cp_c.wait()
        cp_x.wait()
        cp_woa.wait()

        row = jax.lax.broadcasted_iota(jnp.int32, (BQ, BQ), 0)
        col = jax.lax.broadcasted_iota(jnp.int32, (BQ, BQ), 1)
        tri = col <= row

        def ldp(ref, r0, r1):
            return _as_bf16(ref.bitcast(u32)[r0 // 2:r1 // 2, :])

        def a_body(h, carry):
            ws = h % 2

            @pl.when(jnp.logical_and(h % 2 == 0, h + 2 < H))
            def _():
                for cp in pair_copies(h // 2 + 1):
                    cp.start()

            @pl.when(jnp.logical_and(h % 2 == 1, h + 1 < H))
            def _():
                for cp in pair_copies(h // 2 + 1):
                    cp.wait()

            st = {}

            def proj(src, off, t, dst, sc, c):
                r = c * PCH
                w = _as_bf16(w_a.bitcast(u32)[ws, t])
                y = jnp.dot(_as_bf16(src[off + r // 2:off + (r + PCH) // 2, :]), w,
                            preferred_element_type=f32)
                if sc is not None:
                    y = y * sc
                dst[r:r + PCH, :] = y.astype(bf16)

            def scores(i):
                r0 = i * BQ
                q = ldp(q_s, r0, r0 + BQ)
                ss = []
                mm = None
                for j in range(i + 1):
                    s = jax.lax.dot_general(q, ldp(k_s, j * BQ, (j + 1) * BQ), NT,
                                            preferred_element_type=f32)
                    if j == i:
                        s = jnp.where(tri, s, NEG)
                    mm = s if mm is None else jnp.maximum(mm, s)
                    ss.append(s)
                m = jnp.max(mm, axis=1, keepdims=True)
                ps = []
                l = None
                for s in ss:
                    p = jnp.exp2(s - m)
                    l = p if l is None else l + p
                    ps.append(p.astype(bf16))
                st[i] = (ps, _recip(jnp.sum(l, axis=1, keepdims=True)))

            def pv(i):
                ps, rl = st[i]
                o = None
                for j, p in enumerate(ps):
                    t = jnp.dot(p, ldp(v_s, j * BQ, (j + 1) * BQ), preferred_element_type=f32)
                    o = t if o is None else o + t
                st[i] = (o * rl).astype(bf16)

            def outproj(i):
                r0 = APAD + i * BQ
                w = _as_bf16(wo_a[pl.ds(pl.multiple_of(h * (D // 2), D // 2), D // 2), :])
                acc[r0:r0 + BQ, :] += jnp.dot(st[i], w, preferred_element_type=f32)

            for kind, i in a_sched:
                if kind == "Pk":
                    proj(c_s, 0, 0, k_s, None, i)
                elif kind == "Pq":
                    proj(x_s, XPAD, 1, q_s, qscale, i)
                elif kind == "Pv":
                    proj(c_s, 0, 2, v_s, None, i)
                elif kind == "S":
                    scores(i)
                elif kind == "O":
                    pv(i)
                else:
                    outproj(i)
            unpack_weights(h + 1)
            return carry

        jax.lax.fori_loop(0, H, a_body, 0)

        cp_mem.wait()
        cp_gw.wait()
        cp_wob.wait()

        def wb(t, h):
            return _as_bf16(w_b.bitcast(u32)[t * (H + 1) + h])

        def wob(g):
            return _as_bf16(wo_b[g * GB * D // 2:(g + 1) * GB * D // 2, :])

        mem_s[...] = mem0_s[...].astype(f32)
        gw = gw_s[...].astype(f32)

        x0 = _as_bf16(x_s[XPAD:XPAD + SEG // 2, :])
        for t in range(3):
            for h in range(H):
                y = jnp.dot(x0, wb(t, h), preferred_element_type=f32)
                if t == 0:
                    y = y * qscale
                qkv_s[0, :, (t * H + h) * D:(t * H + h + 1) * D] = y

        L = NM + SEG
        r80 = jax.lax.broadcasted_iota(jnp.int32, (2 * L, 2 * L), 0)
        c80 = jax.lax.broadcasted_iota(jnp.int32, (2 * L, 2 * L), 1)
        rhead = jnp.where(r80 < NM, 0, jnp.where(r80 < 2 * NM, 1, jnp.where(r80 < 2 * NM + SEG, 0, 1)))
        chead = jnp.where(c80 < L, 0, 1)
        rpos = jnp.where(r80 < 2 * NM, L - 1,
                         jnp.where(r80 < 2 * NM + SEG, r80 - 2 * NM + NM, r80 - 2 * NM - SEG + NM))
        cpos = jnp.where(c80 < L, c80, c80 - L)
        same = rhead == chead
        valid = jnp.logical_and(same, cpos <= rpos)
        fill = jnp.where(same, NEG, -3e38).astype(f32)

        def gate(j):
            xg = _as_bf16(x_s[pl.ds(pl.multiple_of(j * SEG, SEG), 40), :]).astype(f32)[8:72]
            return jax.nn.sigmoid(jnp.sum(xg * gw, axis=1, keepdims=True))

        def finalize(a0, n, g, z):
            a = acc[pl.ds(a0, n), :]
            acc[pl.ds(a0, n), :] = g * a + (1.0 - g) * z

        def emit_window(j):
            a0 = pl.multiple_of(j * 64, 64)
            out_s[pl.ds(a0, 64), :] = acc[pl.ds(a0, 64), :].astype(bf16)

        def out_copy(j):
            a0 = pl.multiple_of(j * 64, 64)
            return pltpu.make_async_copy(out_s.at[pl.ds(a0, 64), :],
                                         out_hbm.at[pl.ds(a0 - 64, 64), :], sem_out.at[j - 1])

        def b_step(xr, cur, stores, ox_parts):
            lhs = jnp.concatenate([mem_s[...], xr], axis=0).astype(bf16)
            memp, ps, om = {}, {}, {}
            z = None
            for g in range(NG + 3):
                if g < NG:
                    for h in range(g * GB, (g + 1) * GB):
                        r = []
                        for t in range(3):
                            y = jnp.dot(lhs, wb(t, h), preferred_element_type=f32)
                            if t == 0:
                                y = y * qscale
                            c0 = (t * H + h) * D
                            for (y0, n, slot, d0) in stores:
                                qkv_s[slot, d0:d0 + n, c0:c0 + D] = y[y0:y0 + n]
                            r.append(y[:NM])
                        memp[h] = r
                if 0 <= g - 1 < NG:
                    for h0 in range((g - 1) * GB, g * GB, 2):
                        h1 = h0 + 1

                        def xs(t, h):
                            return qkv_s[cur, :, (t * H + h) * D:(t * H + h + 1) * D]
                        q2 = jnp.concatenate([memp[h0][0], memp[h1][0], xs(0, h0), xs(0, h1)], axis=0).astype(bf16)
                        k2 = jnp.concatenate([memp[h0][1], xs(1, h0), memp[h1][1], xs(1, h1)], axis=0).astype(bf16)
                        v2 = jnp.concatenate([memp[h0][2], xs(2, h0), memp[h1][2], xs(2, h1)], axis=0).astype(bf16)
                        sc = jax.lax.dot_general(q2, k2, NT, preferred_element_type=f32)
                        sc = jnp.where(valid, sc, fill)
                        m = jnp.max(sc, axis=1, keepdims=True)
                        p = jnp.exp2(sc - m)
                        l = jnp.sum(p, axis=1, keepdims=True)
                        ps[h0] = (p.astype(bf16), _recip(l), v2)
                if 0 <= g - 2 < NG:
                    for h0 in range((g - 2) * GB, (g - 1) * GB, 2):
                        h1 = h0 + 1
                        p, rl, v2 = ps.pop(h0)
                        o = jnp.dot(p, v2, preferred_element_type=f32) * rl
                        om[h0] = o[0:NM]
                        om[h1] = o[NM:2 * NM]
                        ox_s[cur, :, h0 * D:(h0 + 1) * D] = o[2 * NM:2 * NM + SEG]
                        ox_s[cur, :, h1 * D:(h1 + 1) * D] = o[2 * NM + SEG:]
                if 0 <= g - 3 < NG:
                    gg = g - 3
                    c0, c1 = gg * GB * D, (gg + 1) * GB * D
                    parts = [jnp.concatenate([om[h] for h in range(gg * GB, (gg + 1) * GB)], axis=1)]
                    parts += [ox_s[slot, r0:r1, c0:c1] for (slot, r0, r1) in ox_parts]
                    lo = jnp.concatenate(parts, axis=0).astype(bf16)
                    t = jnp.dot(lo, wob(gg), preferred_element_type=f32)
                    z = t if z is None else z + t
            mem_s[...] = z[:NM].astype(bf16).astype(f32)
            return z[NM:]

        def b_body(j, carry):
            s0 = (j % 2) * 2
            s1 = s0 + 1
            s2 = 2 - s0
            s3 = 3 - s0
            xn = _as_bf16(x_s[pl.ds(pl.multiple_of(j * SEG + XPAD + 16, 8), SEG), :]).astype(f32)
            g = gate(j)
            a0 = pl.multiple_of(j * 64, 64)
            z = b_step(xn[0:40], s0, [(NM, SEG, s1, 0), (NM + SEG, NM, s2, 0)],
                       [(s2, SEG - NM, SEG), (s3, 0, SEG)])
            finalize(pl.multiple_of(a0 + (APAD - 40), 8), 40, g[0:40], z)
            z = b_step(xn[40:64], s1, [(NM, SEG - NM, s2, NM)], [(s0, 0, SEG - NM)])
            finalize(pl.multiple_of(a0 + APAD, 8), 24, g[40:64], z)
            emit_window(j)

            @pl.when(j > 0)
            def _():
                out_copy(j).start()
            return carry

        jax.lax.fori_loop(0, NPAIR, b_body, 0)

        lo = jnp.concatenate([ox_s[2, SEG - NM:SEG, :], ox_s[3, :, :]], axis=0).astype(bf16)
        z = jnp.dot(lo, _as_bf16(wo_b[...]), preferred_element_type=f32)
        g = gate(NPAIR)
        finalize(NPAIR * 64 + APAD - 40, 40, g[0:40], z)
        emit_window(NPAIR)
        out_copy(NPAIR).start()
        for j in range(1, NPAIR + 1):
            out_copy(j).wait()

    scratch = [
        pltpu.VMEM((XPAD + S // 2 + XTAIL, M), u32),
        pltpu.VMEM((S // 2, M), u32),
        pltpu.VMEM((APAD + S, M), f32),
        pltpu.VMEM((S, D), bf16),
        pltpu.VMEM((S, D), bf16),
        pltpu.VMEM((S, D), bf16),
        pltpu.VMEM((2, 3, M, D), u32),
        pltpu.VMEM((2, 3, M, D), bf16),
        pltpu.VMEM((HD // 2, M), u32),
        pltpu.VMEM((2, 3, M, D), u32),
        pltpu.VMEM((3 * (H + 1), M, D), bf16),
        pltpu.VMEM((HD // 2, M), u32),
        pltpu.VMEM((NM, M), bf16),
        pltpu.VMEM((1, M), bf16),
        pltpu.VMEM((NM, M), f32),
        pltpu.VMEM((4, SEG, 3 * HD), f32),
        pltpu.VMEM((4, SEG, HD), f32),
        pltpu.VMEM((APAD + S, M), bf16),
        pltpu.SemaphoreType.DMA((6,)),
        pltpu.SemaphoreType.DMA((3,)),
        pltpu.SemaphoreType.DMA((3,)),
        pltpu.SemaphoreType.DMA((NPAIR,)),
    ]
    return kernel, scratch


@functools.partial(jax.jit, static_argnames=("B_seg_len",))
def pallas_gated_mix__compressed_kv_cla__memory_aug_recurrent_mem_tr__prompt_kernel(
    A_x: jax.Array,
    A_c_kv: jax.Array,
    A_w_q: jax.Array,
    A_w_uk: jax.Array,
    A_w_uv: jax.Array,
    A_w_o: jax.Array,
    B_x: jax.Array,
    B_mem0: jax.Array,
    B_Wq: jax.Array,
    B_Wk: jax.Array,
    B_Wv: jax.Array,
    B_Wo: jax.Array,
    B_seg_len: int,
    gate_w: jax.Array,
):
    _, S, M = A_x.shape
    _, H, D = A_w_q.shape
    NM = B_mem0.shape[1]
    kernel, scratch = _make_kernel(S, M, H, D, NM, int(B_seg_len))
    any_spec = pl.BlockSpec(memory_space=pl.ANY)
    out = pl.pallas_call(
        kernel,
        out_shape=jax.ShapeDtypeStruct((S, M), bf16),
        in_specs=[any_spec] * 12,
        out_specs=any_spec,
        scratch_shapes=scratch,
        compiler_params=pltpu.CompilerParams(vmem_limit_bytes=100 * 1024 * 1024),
    )(
        A_x.reshape(S, M), A_c_kv.reshape(S, M), A_w_q, A_w_uk, A_w_uv,
        A_w_o.reshape(H * D, M), B_mem0.reshape(NM, M),
        B_Wq, B_Wk, B_Wv, B_Wo.reshape(H * D, M), gate_w.reshape(1, M),
    )
    return out.reshape(1, S, M)
```

```python
import functools

import jax
import jax.numpy as jnp
import jax.experimental.pallas as pl
import jax.experimental.pallas.tpu as pltpu

bf16 = jnp.bfloat16
f32 = jnp.float32
u32 = jnp.uint32

LOG2E = 1.4426950408889634
NEG = -1e9 * LOG2E
NT = (((1,), (1,)), ((), ()))

BQ = 128
PCH = 512
GB = 4
XPAD = 24
XTAIL = 16
APAD = 64


def _as_bf16(words):
    return pltpu.bitcast(words, bf16)


def _recip(l):
    r = pl.reciprocal(l, approx=True)
    return r * (2.0 - l * r)


def _unpack_head(words, par):
    sh = ((1 - par) * 16).astype(u32)
    w = jnp.bitwise_and(jnp.left_shift(words, sh), jnp.uint32(0xFFFF0000))
    return pltpu.bitcast(w, f32).astype(bf16)


def _token(v):
    f = pltpu.bitcast(jnp.right_shift(pltpu.bitcast(v[0:8, 0:128], u32), jnp.uint32(2)), f32)
    return pltpu.bitcast(f - f, u32)


def _unpack_head_tok(words, par, tok):
    r, c = words.shape
    sh = ((1 - par) * 16).astype(u32) + tok
    mask = jnp.bitwise_or(tok, jnp.uint32(0xFFFF0000))
    w = jnp.bitwise_and(jnp.left_shift(words.reshape(r // 8, 8, c), sh[None]), mask[None])
    return pltpu.bitcast(w.reshape(r, c), f32).astype(bf16)


def _a_schedule(nq, bpc):
    assert nq == 16 and bpc == 4
    out = []
    fill = {0: ("Pk", 1, None), 1: ("Pq", 1, None), 2: ("Pv", 1, None),
            4: ("Pk", 2, 2), 5: ("Pq", 2, 3), 6: ("Pv", 2, 4),
            8: ("Pk", 3, 6), 9: ("Pq", 3, 7), 10: ("Pv", 3, 8)}
    for t in range(nq):
        out.append(("S", t, None))
        if t in fill:
            out.append(fill[t])
        if t == nq - 1:
            out.append(("Nk", 0, 13))
        if t >= 1:
            out.append(("O", t - 1, None))
        if t == nq - 1:
            out.append(("Nq", 0, 14))
        if t >= 2:
            out.append(("F", t - 2, None))
    out += [("F", nq - 2, None), ("O", nq - 1, None), ("Nv", 0, 15), ("F", nq - 1, None)]
    return out


def _make_kernel(S, M, H, D, NM, SEG):
    assert SEG == 32 and NM == 8 and D == 128 and S % PCH == 0 and H % 2 == 0 and H % GB == 0
    NQ = S // BQ
    NPAIR = S // (2 * SEG)
    NG = H // GB
    HD = H * D
    qscale = D ** -0.5 * LOG2E
    a_sched = _a_schedule(NQ, PCH // BQ)

    def kernel(x_hbm, c_hbm, wq_hbm, wk_hbm, wv_hbm, wo_hbm, mem0_hbm,
               bq_hbm, bk_hbm, bv_hbm, bo_hbm, gw_hbm, out_hbm,
               x_s, c_s, acc, q_s, k_s, v_s, st_a, wo_a, st_b, w_b, wo_b,
               mem0_s, gw_s, mem_s, qkv_s, ox_s, out_s,
               sem_in, sem_a, sem_b, sem_out):
        a_w_hbm = (wk_hbm, wq_hbm, wv_hbm)
        b_w_hbm = (bq_hbm, bk_hbm, bv_hbm)

        def pair_copy(src, stage, sems, t, p):
            return pltpu.make_async_copy(
                src.bitcast(u32).at[:, p, :], stage.at[p % 2, t], sems.at[t])

        def a_copies(p):
            return [pair_copy(a_w_hbm[t], st_a, sem_a, t, p) for t in range(3)]

        def b_copies(p):
            return [pair_copy(b_w_hbm[t], st_b, sem_b, t, p) for t in range(3)]

        cp_x = pltpu.make_async_copy(x_hbm.bitcast(u32), x_s.at[XPAD:XPAD + S // 2, :], sem_in.at[0])
        cp_c = pltpu.make_async_copy(c_hbm.bitcast(u32), c_s, sem_in.at[1])
        cp_woa0 = pltpu.make_async_copy(wo_hbm.bitcast(u32).at[0:D, :], wo_a.at[0:D, :], sem_in.at[2])
        cp_woa = pltpu.make_async_copy(wo_hbm.bitcast(u32).at[D:HD // 2, :], wo_a.at[D:HD // 2, :], sem_in.at[6])
        cp_wob = pltpu.make_async_copy(bo_hbm.bitcast(u32), wo_b, sem_in.at[3])
        cp_mem = pltpu.make_async_copy(mem0_hbm, mem0_s, sem_in.at[4])
        cp_gw = pltpu.make_async_copy(gw_hbm, gw_s, sem_in.at[5])

        first = a_copies(0) + b_copies(0)
        first[0].start()
        cp_c.start()
        first[1].start()
        cp_x.start()
        first[2].start()
        cp_woa0.start()
        for cp in first[3:]:
            cp.start()
        cp_woa.start()
        cp_mem.start()
        cp_gw.start()
        cp_wob.start()

        x_s[0:XPAD, :] = jnp.zeros((XPAD, M), u32)
        x_s[XPAD + S // 2:XPAD + S // 2 + XTAIL, :] = jnp.zeros((XTAIL, M), u32)
        acc[...] = jnp.zeros(acc.shape, f32)
        ox_s[...] = jnp.zeros(ox_s.shape, f32)

        def unpack_weights(hn):
            slot = (hn // 2) % 2
            par = hn % 2
            for t in range(3):
                w_b[t * (H + 1) + hn] = _unpack_head(st_b[slot, t], par)

        def unpack_b_piece(hn, t, c, tok):
            rows = pl.ds(c * (M // 4), M // 4)
            w_b[t * (H + 1) + hn, rows, :] = _unpack_head_tok(st_b[(hn // 2) % 2, t, rows, :], hn % 2, tok)

        for cp in first[3:]:
            cp.wait()
        unpack_weights(jnp.int32(0))
        for cp in first[:3]:
            cp.wait()
        cp_c.wait()
        cp_x.wait()
        for (srcr, off, t, dst, sc) in ((c_s, 0, 0, k_s, None), (x_s, XPAD, 1, q_s, qscale), (c_s, 0, 2, v_s, None)):
            y = jnp.dot(_as_bf16(srcr[off:off + PCH // 2, :]), _unpack_head(st_a[0, t], jnp.int32(0)),
                        preferred_element_type=f32)
            if sc is not None:
                y = y * sc
            dst[0:PCH, :] = y.astype(bf16)
        cp_woa0.wait()

        row = jax.lax.broadcasted_iota(jnp.int32, (BQ, BQ), 0)
        col = jax.lax.broadcasted_iota(jnp.int32, (BQ, BQ), 1)
        tri = col <= row

        def ldp(ref, r0, r1):
            return _as_bf16(ref.bitcast(u32)[r0 // 2:r1 // 2, :])

        def a_body(h, carry):
            @pl.when(jnp.logical_and(h % 2 == 0, h + 2 < H))
            def _():
                for cp in a_copies(h // 2 + 1) + b_copies(h // 2 + 1):
                    cp.start()

            @pl.when(jnp.logical_and(h % 2 == 1, h + 1 < H))
            def _():
                for cp in a_copies(h // 2 + 1) + b_copies(h // 2 + 1):
                    cp.wait()

            @pl.when(h == 1)
            def _():
                cp_woa.wait()

            st = {}
            toks = {}

            def proj(src, off, t, dst, sc, c, hh, tk):
                r = c * PCH
                words = st_a[(hh // 2) % 2, t]
                if tk is None:
                    w = _unpack_head(words, hh % 2)
                else:
                    w = _unpack_head_tok(words, hh % 2, toks[tk])
                y = jnp.dot(_as_bf16(src[off + r // 2:off + (r + PCH) // 2, :]), w,
                            preferred_element_type=f32)
                if sc is not None:
                    y = y * sc
                dst[r:r + PCH, :] = y.astype(bf16)

            def scores(i):
                r0 = i * BQ
                q = ldp(q_s, r0, r0 + BQ)
                ss = []
                mm = None
                for j in range(i + 1):
                    s = jax.lax.dot_general(q, ldp(k_s, j * BQ, (j + 1) * BQ), NT,
                                            preferred_element_type=f32)
                    if j == i:
                        s = jnp.where(tri, s, NEG)
                    mm = s if mm is None else jnp.maximum(mm, s)
                    ss.append(s)
                toks[i] = _token(mm)
                m = jnp.max(mm, axis=1, keepdims=True)
                ps = []
                l = None
                for s in ss:
                    p = jnp.exp2(s - m)
                    l = p if l is None else l + p
                    ps.append(p.astype(bf16))
                st[i] = (ps, _recip(jnp.sum(l, axis=1, keepdims=True)))

            def pv(i):
                ps, rl = st[i]
                o = None
                for j, p in enumerate(ps):
                    t = jnp.dot(p, ldp(v_s, j * BQ, (j + 1) * BQ), preferred_element_type=f32)
                    o = t if o is None else o + t
                st[i] = (o * rl).astype(bf16)

            def outproj(i):
                r0 = APAD + i * BQ
                w = _as_bf16(wo_a[pl.ds(pl.multiple_of(h * (D // 2), D // 2), D // 2), :])
                acc[r0:r0 + BQ, :] += jnp.dot(st[i], w, preferred_element_type=f32)

            for kind, i, tk in a_sched:
                hh = h if kind[0] == "P" else h + 1
                if kind in ("Pk", "Nk"):
                    proj(c_s, 0, 0, k_s, None, i, hh, tk)
                elif kind in ("Pq", "Nq"):
                    proj(x_s, XPAD, 1, q_s, qscale, i, hh, tk)
                elif kind in ("Pv", "Nv"):
                    proj(c_s, 0, 2, v_s, None, i, hh, tk)
                elif kind == "S":
                    scores(i)
                    if 1 <= i <= 12:
                        unpack_b_piece(h + 1, (i - 1) // 4, (i - 1) % 4, toks[i])
                elif kind == "O":
                    pv(i)
                else:
                    outproj(i)
            return carry

        jax.lax.fori_loop(0, H, a_body, 0)

        cp_mem.wait()
        cp_gw.wait()
        cp_wob.wait()

        def wb(t, h):
            return _as_bf16(w_b.bitcast(u32)[t * (H + 1) + h])

        def wob(g):
            return _as_bf16(wo_b[g * GB * D // 2:(g + 1) * GB * D // 2, :])

        mem_s[...] = mem0_s[...].astype(f32)
        gw = gw_s[...].astype(f32)

        x0 = _as_bf16(x_s[XPAD:XPAD + SEG // 2, :])
        for t in range(3):
            for h in range(H):
                y = jnp.dot(x0, wb(t, h), preferred_element_type=f32)
                if t == 0:
                    y = y * qscale
                qkv_s[0, :, (t * H + h) * D:(t * H + h + 1) * D] = y

        L = NM + SEG
        r80 = jax.lax.broadcasted_iota(jnp.int32, (2 * L, 2 * L), 0)
        c80 = jax.lax.broadcasted_iota(jnp.int32, (2 * L, 2 * L), 1)
        rhead = jnp.where(r80 < NM, 0, jnp.where(r80 < 2 * NM, 1, jnp.where(r80 < 2 * NM + SEG, 0, 1)))
        chead = jnp.where(c80 < L, 0, 1)
        rpos = jnp.where(r80 < 2 * NM, L - 1,
                         jnp.where(r80 < 2 * NM + SEG, r80 - 2 * NM + NM, r80 - 2 * NM - SEG + NM))
        cpos = jnp.where(c80 < L, c80, c80 - L)
        same = rhead == chead
        valid = jnp.logical_and(same, cpos <= rpos)
        fill = jnp.where(same, NEG, -3e38).astype(f32)

        def gate(j):
            xg = _as_bf16(x_s[pl.ds(pl.multiple_of(j * SEG, SEG), 40), :]).astype(f32)[8:72]
            return jax.nn.sigmoid(jnp.sum(xg * gw, axis=1, keepdims=True))

        def finalize(a0, n, g, z):
            a = acc[pl.ds(a0, n), :]
            acc[pl.ds(a0, n), :] = g * a + (1.0 - g) * z

        def emit_window(j):
            a0 = pl.multiple_of(j * 64, 64)
            out_s[pl.ds(a0, 64), :] = acc[pl.ds(a0, 64), :].astype(bf16)

        def out_copy(j):
            a0 = pl.multiple_of(j * 64, 64)
            return pltpu.make_async_copy(out_s.at[pl.ds(a0, 64), :],
                                         out_hbm.at[pl.ds(a0 - 64, 64), :], sem_out.at[j - 1])

        def b_step(xr, cur, stores, ox_parts, tie):
            lhs = jnp.concatenate([mem_s[...], xr], axis=0).astype(bf16)
            memp, ps, om = {}, {}, {}
            z = None
            for g in range(NG + 3):
                if g < NG:
                    for h in range(g * GB, (g + 1) * GB):
                        r = []
                        for t in range(3):
                            y = jnp.dot(lhs, wb(t, h), preferred_element_type=f32)
                            if t == 0:
                                y = y * qscale
                            c0 = (t * H + h) * D
                            for (y0, n, slot, d0) in stores:
                                qkv_s[slot, d0:d0 + n, c0:c0 + D] = y[y0:y0 + n]
                            r.append(y[:NM])
                        memp[h] = r
                if 0 <= g - 1 < NG:
                    for h0 in range((g - 1) * GB, g * GB, 2):
                        h1 = h0 + 1

                        def xs(t, h):
                            return qkv_s[cur, :, (t * H + h) * D:(t * H + h + 1) * D]
                        q2 = jnp.concatenate([memp[h0][0], memp[h1][0], xs(0, h0), xs(0, h1)], axis=0).astype(bf16)
                        k2 = jnp.concatenate([memp[h0][1], xs(1, h0), memp[h1][1], xs(1, h1)], axis=0).astype(bf16)
                        v2 = jnp.concatenate([memp[h0][2], xs(2, h0), memp[h1][2], xs(2, h1)], axis=0).astype(bf16)
                        sc = jax.lax.dot_general(q2, k2, NT, preferred_element_type=f32)
                        sc = jnp.where(valid, sc, fill)
                        m = jnp.max(sc, axis=1, keepdims=True)
                        p = jnp.exp2(sc - m)
                        l = jnp.sum(p, axis=1, keepdims=True)
                        ps[h0] = (p.astype(bf16), _recip(l), v2)
                if 0 <= g - 2 < NG:
                    for h0 in range((g - 2) * GB, (g - 1) * GB, 2):
                        h1 = h0 + 1
                        p, rl, v2 = ps.pop(h0)
                        o = jnp.dot(p, v2, preferred_element_type=f32) * rl
                        om[h0] = o[0:NM]
                        om[h1] = o[NM:2 * NM]
                        if tie and g - 2 < NG - 1:
                            ou = pltpu.bitcast(o[2 * NM:], u32).reshape(2 * SEG // 8, 8, D)
                            acc_or = ou[0]
                            for r in range(1, 2 * SEG // 8):
                                acc_or = jnp.bitwise_or(acc_or, ou[r])
                            f = pltpu.bitcast(jnp.right_shift(acc_or, jnp.uint32(2)), f32)
                            om[h0] = om[h0] + (f - f)
                        ox_s[cur, :, h0 * D:(h0 + 1) * D] = o[2 * NM:2 * NM + SEG]
                        ox_s[cur, :, h1 * D:(h1 + 1) * D] = o[2 * NM + SEG:]
                if 0 <= g - 3 < NG:
                    gg = g - 3
                    c0, c1 = gg * GB * D, (gg + 1) * GB * D
                    parts = [jnp.concatenate([om[h] for h in range(gg * GB, (gg + 1) * GB)], axis=1)]
                    parts += [ox_s[slot, r0:r1, c0:c1] for (slot, r0, r1) in ox_parts]
                    lo = jnp.concatenate(parts, axis=0).astype(bf16)
                    t = jnp.dot(lo, wob(gg), preferred_element_type=f32)
                    z = t if z is None else z + t
            mem_s[...] = z[:NM].astype(bf16).astype(f32)
            return z[NM:]

        def b_body(j, carry):
            s0 = (j % 2) * 2
            s1 = s0 + 1
            s2 = 2 - s0
            s3 = 3 - s0
            xn = _as_bf16(x_s[pl.ds(pl.multiple_of(j * SEG + XPAD + 16, 8), SEG), :]).astype(f32)
            g = gate(j)
            a0 = pl.multiple_of(j * 64, 64)
            z = b_step(xn[0:40], s0, [(NM, SEG, s1, 0), (NM + SEG, NM, s2, 0)],
                       [(s2, SEG - NM, SEG), (s3, 0, SEG)], False)
            finalize(pl.multiple_of(a0 + (APAD - 40), 8), 40, g[0:40], z)
            emit_window(j)
            z = b_step(xn[40:64], s1, [(NM, SEG - NM, s2, NM)], [(s0, 0, SEG - NM)], True)
            finalize(pl.multiple_of(a0 + APAD, 8), 24, g[40:64], z)

            @pl.when(j > 0)
            def _():
                out_copy(j).start()
            return carry

        jax.lax.fori_loop(0, NPAIR, b_body, 0)

        lo = jnp.concatenate([ox_s[2, SEG - NM:SEG, :], ox_s[3, :, :]], axis=0).astype(bf16)
        z = jnp.dot(lo, _as_bf16(wo_b[...]), preferred_element_type=f32)
        g = gate(NPAIR)
        finalize(NPAIR * 64 + APAD - 40, 40, g[0:40], z)
        emit_window(NPAIR)
        out_copy(NPAIR).start()
        for j in range(1, NPAIR + 1):
            out_copy(j).wait()

    scratch = [
        pltpu.VMEM((XPAD + S // 2 + XTAIL, M), u32),
        pltpu.VMEM((S // 2, M), u32),
        pltpu.VMEM((APAD + S, M), f32),
        pltpu.VMEM((S, D), bf16),
        pltpu.VMEM((S, D), bf16),
        pltpu.VMEM((S, D), bf16),
        pltpu.VMEM((2, 3, M, D), u32),
        pltpu.VMEM((HD // 2, M), u32),
        pltpu.VMEM((2, 3, M, D), u32),
        pltpu.VMEM((3 * (H + 1), M, D), bf16),
        pltpu.VMEM((HD // 2, M), u32),
        pltpu.VMEM((NM, M), bf16),
        pltpu.VMEM((1, M), bf16),
        pltpu.VMEM((NM, M), f32),
        pltpu.VMEM((4, SEG, 3 * HD), f32),
        pltpu.VMEM((4, SEG, HD), f32),
        pltpu.VMEM((APAD + S, M), bf16),
        pltpu.SemaphoreType.DMA((7,)),
        pltpu.SemaphoreType.DMA((3,)),
        pltpu.SemaphoreType.DMA((3,)),
        pltpu.SemaphoreType.DMA((NPAIR,)),
    ]
    return kernel, scratch


@functools.partial(jax.jit, static_argnames=("B_seg_len",))
def pallas_gated_mix__compressed_kv_cla__memory_aug_recurrent_mem_tr__prompt_kernel(
    A_x: jax.Array,
    A_c_kv: jax.Array,
    A_w_q: jax.Array,
    A_w_uk: jax.Array,
    A_w_uv: jax.Array,
    A_w_o: jax.Array,
    B_x: jax.Array,
    B_mem0: jax.Array,
    B_Wq: jax.Array,
    B_Wk: jax.Array,
    B_Wv: jax.Array,
    B_Wo: jax.Array,
    B_seg_len: int,
    gate_w: jax.Array,
):
    _, S, M = A_x.shape
    _, H, D = A_w_q.shape
    NM = B_mem0.shape[1]
    kernel, scratch = _make_kernel(S, M, H, D, NM, int(B_seg_len))
    any_spec = pl.BlockSpec(memory_space=pl.ANY)
    out = pl.pallas_call(
        kernel,
        out_shape=jax.ShapeDtypeStruct((S, M), bf16),
        in_specs=[any_spec] * 12,
        out_specs=any_spec,
        scratch_shapes=scratch,
        compiler_params=pltpu.CompilerParams(vmem_limit_bytes=100 * 1024 * 1024, disable_bounds_checks=True, disable_semaphore_checks=True),
    )(
        A_x.reshape(S, M), A_c_kv.reshape(S, M), A_w_q, A_w_uk, A_w_uv,
        A_w_o.reshape(H * D, M), B_mem0.reshape(NM, M),
        B_Wq, B_Wk, B_Wv, B_Wo.reshape(H * D, M), gate_w.reshape(1, M),
    )
    return out.reshape(1, S, M)
```

```python
import functools

import jax
import jax.numpy as jnp
import jax.experimental.pallas as pl
import jax.experimental.pallas.tpu as pltpu

bf16 = jnp.bfloat16
f32 = jnp.float32
u32 = jnp.uint32

LOG2E = 1.4426950408889634
NEG = -1e9 * LOG2E
NT = (((1,), (1,)), ((), ()))

BQ = 128
PCH = 512
GB = 4
XPAD = 24
XTAIL = 16
APAD = 64

JG = 4
JLA = 8
EXP_LEAD = 256
MAX_SLACK = 384
MAX_MIN = 4


def _as_bf16(words):
    return pltpu.bitcast(words, bf16)


def _recip(l):
    r = pl.reciprocal(l, approx=True)
    return r * (2.0 - l * r)


def _unpack_head(words, par):
    sh = ((1 - par) * 16).astype(u32)
    w = jnp.bitwise_and(jnp.left_shift(words, sh), jnp.uint32(0xFFFF0000))
    return pltpu.bitcast(w, f32).astype(bf16)


def _token(v):
    f = pltpu.bitcast(jnp.right_shift(pltpu.bitcast(v[0:8, 0:128], u32), jnp.uint32(2)), f32)
    return pltpu.bitcast(f - f, u32)


def _token_all(v):
    v3 = v.reshape(v.shape[0] // 8, 8, v.shape[1])
    n = v3.shape[0]
    parts = [v3[i] for i in range(n)]
    while len(parts) > 1:
        parts = [jnp.maximum(parts[i], parts[i + 1]) for i in range(0, len(parts), 2)]
    return _token(parts[0])


def _unpack_head_tok(words, par, tok):
    r, c = words.shape
    sh = ((1 - par) * 16).astype(u32) + tok
    mask = jnp.bitwise_or(tok, jnp.uint32(0xFFFF0000))
    w = jnp.bitwise_and(jnp.left_shift(words.reshape(r // 8, 8, c), sh[None]), mask[None])
    return pltpu.bitcast(w.reshape(r, c), f32).astype(bf16)


def _unpack_pair_tok(words, tok):
    r, c = words.shape
    w3 = words.reshape(r // 8, 8, c)
    lo = jnp.left_shift(w3, (tok + jnp.uint32(16))[None])
    hi = jnp.bitwise_and(w3, jnp.bitwise_or(tok, jnp.uint32(0xFFFF0000))[None])
    return (pltpu.bitcast(lo.reshape(r, c), f32).astype(bf16),
            pltpu.bitcast(hi.reshape(r, c), f32).astype(bf16))


def _a_schedule(nq, bpc):
    assert nq == 16 and bpc == 4
    out = []
    fill = {0: ("Pk", 1, None), 1: ("Pq", 1, None), 2: ("Pv", 1, None),
            4: ("Pk", 2, 2), 5: ("Pq", 2, 3), 6: ("Pv", 2, 4),
            8: ("Pk", 3, 6), 9: ("Pq", 3, 7), 10: ("Pv", 3, 8)}
    for t in range(nq):
        out.append(("S", t, None))
        if t in fill:
            out.append(fill[t])
        if t == nq - 1:
            out.append(("Nk", 0, 13))
        if t >= 1:
            out.append(("O", t - 1, None))
        if t == nq - 1:
            out.append(("Nq", 0, 14))
        if t >= 2:
            out.append(("F", t - 2, None))
    out += [("F", nq - 2, None), ("O", nq - 1, None), ("Nv", 0, 15), ("F", nq - 1, None)]
    return out


def _units(a_tasks):
    units = []
    for name, fn in a_tasks:
        if name[0] == "S":
            units.append([])
        units[-1].append((name, fn))
    return units


def _merge(a_tasks, b_tasks):
    units = _units(a_tasks)
    plan = {}
    mids = [[2, 5], [1, 3, 5], [1, 3, 5], [0, 2, 4, 6]]
    u = 0
    for step in range(4):
        for g in mids[step]:
            plan.setdefault((step, "end", g), []).extend(units[u])
            u += 1
        t = units[u]
        u += 1
        if step < 3:
            assert len(t) == 4
            plan[(step, "Sc", 7)] = [t[0]]
            plan[(step, "Pv", 7)] = [t[1]]
            plan[(step, "Op", 7)] = t[2:]
        else:
            plan[(step, "Sc", 7)] = t[0:2]
            plan[(step, "Pv", 7)] = t[2:5]
            plan[(step, "Op", 7)] = t[5:]
    assert u == len(units)
    out = []
    for name, fn in b_tasks:
        if fn is not None:
            out.append(fn)
        out += [f for _, f in plan.pop(name, [])]
    assert not plan, plan
    return out


def _make_kernel(S, M, H, D, NM, SEG):
    assert SEG == 32 and NM == 8 and D == 128 and S % PCH == 0 and H % 2 == 0 and H % GB == 0
    NQ = S // BQ
    NPAIR = S // (2 * SEG)
    NG = H // GB
    HD = H * D
    NCH = S // PCH
    H1 = H // 2
    NP2 = H // 2
    assert NPAIR == 2 * (H - H1) and NQ == H1 and NP2 == H1
    EMIT = NQ - 2
    qscale = D ** -0.5 * LOG2E
    a_sched = _a_schedule(NQ, PCH // BQ)

    def kernel(x_hbm, c_hbm, wq_hbm, wk_hbm, wv_hbm, wo_hbm, mem0_hbm,
               bq_hbm, bk_hbm, bv_hbm, bo_hbm, gw_hbm, out_hbm,
               x_s, c_s, acc1, acc, g_s, q_s, k_s, v_s, st_a, wo_a, st_b, w_b, wo_b,
               mem0_s, gw_s, mem_s, qkv_s, ox_s, out_s,
               sem_in, sem_a, sem_b, sem_out, sem_xc):
        a_w_hbm = (wk_hbm, wq_hbm, wv_hbm)
        b_w_hbm = (bq_hbm, bk_hbm, bv_hbm)

        def a_copies(p):
            return [pltpu.make_async_copy(a_w_hbm[t].bitcast(u32).at[:, p, :], st_a.at[p, t],
                                          sem_a.at[t, p % 2]) for t in range(3)]

        def b_copies(p):
            return [pltpu.make_async_copy(b_w_hbm[t].bitcast(u32).at[:, p, :], st_b.at[p % 2, t],
                                          sem_b.at[t, p % 2]) for t in range(3)]

        cp_x = [pltpu.make_async_copy(x_hbm.bitcast(u32).at[c * (PCH // 2):(c + 1) * (PCH // 2), :],
                                      x_s.at[XPAD + c * (PCH // 2):XPAD + (c + 1) * (PCH // 2), :], sem_xc.at[c])
                for c in range(NCH)]
        cp_c = [pltpu.make_async_copy(c_hbm.bitcast(u32).at[c * (PCH // 2):(c + 1) * (PCH // 2), :],
                                      c_s.at[c * (PCH // 2):(c + 1) * (PCH // 2), :], sem_xc.at[NCH + c])
                for c in range(NCH)]
        cp_woa0 = pltpu.make_async_copy(wo_hbm.bitcast(u32).at[0:D, :], wo_a.at[0:D, :], sem_in.at[2])
        cp_woa = pltpu.make_async_copy(wo_hbm.bitcast(u32).at[D:HD // 2, :], wo_a.at[D:HD // 2, :], sem_in.at[6])
        cp_wob = pltpu.make_async_copy(bo_hbm.bitcast(u32), wo_b, sem_in.at[3])
        cp_mem = pltpu.make_async_copy(mem0_hbm, mem0_s, sem_in.at[4])
        cp_gw = pltpu.make_async_copy(gw_hbm, gw_s, sem_in.at[5])

        first = a_copies(0)
        cp_gw.start()
        first[0].start()
        cp_c[0].start()
        first[1].start()
        cp_x[0].start()
        first[2].start()
        for c in range(1, NCH):
            cp_c[c].start()
            cp_x[c].start()
        cp_woa0.start()
        for cp in b_copies(0) + a_copies(1):
            cp.start()
        cp_woa.start()
        cp_mem.start()
        cp_wob.start()

        x_s[0:XPAD, :] = jnp.zeros((XPAD, M), u32)
        x_s[XPAD + S // 2:XPAD + S // 2 + XTAIL, :] = jnp.zeros((XTAIL, M), u32)
        acc1[...] = jnp.zeros(acc1.shape, f32)
        acc[0:APAD, :] = jnp.zeros((APAD, M), f32)
        g_s[0:APAD, :] = jnp.zeros((APAD, D), f32)
        ox_s[...] = jnp.zeros(ox_s.shape, f32)

        for (srcr, off, t, dst, sc, pre) in ((c_s, 0, 0, k_s, None, [first[0], cp_c[0]]),
                                             (x_s, XPAD, 1, q_s, qscale, [first[1], cp_x[0]]),
                                             (c_s, 0, 2, v_s, None, [first[2]])):
            for cp in pre:
                cp.wait()
            y = jnp.dot(_as_bf16(srcr[off:off + PCH // 2, :]), _unpack_head(st_a[0, t], jnp.int32(0)),
                        preferred_element_type=f32)
            if sc is not None:
                y = y * sc
            dst[0:PCH, :] = y.astype(bf16)
        for cp in cp_c[1:] + cp_x[1:]:
            cp.wait()
        cp_woa0.wait()
        cp_gw.wait()

        row = jax.lax.broadcasted_iota(jnp.int32, (BQ, BQ), 0)
        col = jax.lax.broadcasted_iota(jnp.int32, (BQ, BQ), 1)
        tri = col <= row

        def tie(words, tok, r=0):
            if tok is None:
                return words
            n, c = words.shape
            blk = words[r:r + 8]
            if c > 128:
                blk = jnp.concatenate([jnp.bitwise_or(blk[:, :128], tok), blk[:, 128:]], axis=1)
            else:
                blk = jnp.bitwise_or(blk, tok)
            parts = ([words[:r]] if r else []) + [blk] + ([words[r + 8:]] if r + 8 < n else [])
            return jnp.concatenate(parts, axis=0)

        def ldp(ref, r0, r1, tok=None):
            return _as_bf16(tie(ref.bitcast(u32)[r0 // 2:r1 // 2, :], tok))

        def a_tasks(h, fused, on_scores, on_emit=None):
            st = {}
            toks = {}
            marks = []
            clock = [0]
            due = []

            def take(time):
                tk = None
                for tm, v in [d for d in due if d[0] <= time]:
                    t = _token_all(v)
                    tk = t if tk is None else jnp.bitwise_or(tk, t)
                due[:] = [d for d in due if d[0] > time]
                return tk

            def anchor(time):
                best = None
                for tm, v in marks:
                    if tm <= time:
                        best = v
                return best

            def proj(src, off, t, dst, sc, c, hh, tk):
                r = c * PCH
                words = st_a[(hh // 2) % NP2, t]
                if tk is None:
                    w = _unpack_head(words, hh % 2)
                else:
                    w = _unpack_head_tok(words, hh % 2, toks[tk])
                lhs = src[off + r // 2:off + (r + PCH) // 2, :]
                for rr in range(0, PCH, BQ):
                    lhs = tie(lhs, take(clock[0] + rr), rr // 2)
                y = jnp.dot(_as_bf16(lhs), w, preferred_element_type=f32)
                for rr in range(64, PCH, 64):
                    marks.append((clock[0] + rr, y[rr:rr + 8]))
                clock[0] += PCH
                if sc is not None:
                    y = y * sc
                dst[r:r + PCH, :] = y.astype(bf16)

            def scores(i):
                r0 = i * BQ
                qw = q_s.bitcast(u32)[r0 // 2:(r0 + BQ) // 2, :]
                ss = []
                mm = None
                for j in range(i + 1):
                    tk = take(clock[0] + (j // 4) * BQ) if j % 4 == 0 else None
                    s = jax.lax.dot_general(_as_bf16(tie(qw, tk)), ldp(k_s, j * BQ, (j + 1) * BQ), NT,
                                            preferred_element_type=f32)
                    marks.append((clock[0] + min(BQ * (j // 4 + 1), (i + 1) * BQ // 4), s))
                    if j == i:
                        s = jnp.where(tri, s, NEG)
                    mm = s if mm is None else jnp.maximum(mm, s)
                    if fused and (j % 4 == 3 or j == i) and i >= MAX_MIN:
                        due.append((clock[0] + min(BQ * (j // 4 + 1), (i + 1) * BQ // 4) + MAX_SLACK, mm))
                    ss.append(s)
                clock[0] += (i + 1) * BQ // 4
                toks[i] = _token(mm)
                m = jnp.max(mm, axis=1, keepdims=True)
                st[i] = (ss, m)
                on_scores(i, toks[i])

            def pv(i):
                ss, m = st[i]
                m = jnp.broadcast_to(m, (BQ, BQ))
                o = None
                l = None
                ts = []
                for j, s in enumerate(ss):
                    if j % JG == 0:
                        if j >= JLA:
                            av = ts[j - JLA]
                        else:
                            av = anchor(clock[0] + (j // 4) * BQ - EXP_LEAD) if fused else None
                        if av is not None:
                            tok = pltpu.bitcast(_token(av), f32)
                            m = (m.reshape(BQ // 8, 8, BQ) + tok[None]).reshape(BQ, BQ)
                    p = jnp.exp2(s - m)
                    l = p if l is None else l + p
                    tk = take(clock[0] + (j // 4) * BQ) if j % 4 == 0 else None
                    pb = p.astype(bf16)
                    if tk is not None:
                        pb = _as_bf16(tie(pltpu.bitcast(pb, u32), tk))
                    t = jnp.dot(pb, ldp(v_s, j * BQ, (j + 1) * BQ), preferred_element_type=f32)
                    ts.append(t)
                    o = t if o is None else o + t
                for j, t in enumerate(ts):
                    marks.append((clock[0] + min(BQ * (j // 4 + 1), (i + 1) * BQ // 4), t))
                clock[0] += (i + 1) * BQ // 4
                o = o * _recip(jnp.sum(l, axis=1, keepdims=True))
                if fused:
                    o = o * g_s[APAD + i * BQ:APAD + (i + 1) * BQ, :]
                st[i] = o.astype(bf16)

            def outproj(i):
                r0 = APAD + i * BQ
                w = _as_bf16(wo_a[pl.ds(pl.multiple_of(h * (D // 2), D // 2), D // 2), :])
                dst = acc if fused else acc1
                lhs = st[i]
                tk = take(clock[0])
                if tk is not None:
                    lhs = _as_bf16(tie(pltpu.bitcast(lhs, u32), tk))
                d = jnp.dot(lhs, w, preferred_element_type=f32)
                marks.append((clock[0] + BQ // 2, d[BQ // 2:BQ // 2 + 8]))
                marks.append((clock[0] + BQ, d[BQ - 8:BQ]))
                clock[0] += BQ
                a = dst[r0:r0 + BQ, :] + d
                dst[r0:r0 + BQ, :] = a
                if fused and i < EMIT:
                    out_s[i * BQ:(i + 1) * BQ, :] = a.astype(bf16)
                    on_emit(i)

            out = []
            for kind, i, tk in a_sched:
                hh = h if kind[0] == "P" else h + 1
                if kind in ("Pk", "Nk"):
                    fn = functools.partial(proj, c_s, 0, 0, k_s, None, i, hh, tk)
                elif kind in ("Pq", "Nq"):
                    fn = functools.partial(proj, x_s, XPAD, 1, q_s, qscale, i, hh, tk)
                elif kind in ("Pv", "Nv"):
                    fn = functools.partial(proj, c_s, 0, 2, v_s, None, i, hh, tk)
                elif kind == "S":
                    fn = functools.partial(scores, i)
                elif kind == "O":
                    fn = functools.partial(pv, i)
                else:
                    fn = functools.partial(outproj, i)
                out.append(((kind, i), fn))
            return out

        gw = gw_s[...].astype(f32)

        def a_body(h, carry):
            for cp in b_copies(h):
                cp.wait()

            @pl.when(h + 1 < H1)
            def _():
                for cp in a_copies(h + 1):
                    cp.wait()
                for cp in b_copies(h + 1):
                    cp.start()

            @pl.when(h + 2 < H1)
            def _():
                for cp in a_copies(h + 2):
                    cp.start()

            @pl.when(h == 1)
            def _():
                cp_woa.wait()

            def on_scores(i, tok):
                if 1 <= i <= 12:
                    t, c = (i - 1) // 4, (i - 1) % 4
                    rows = pl.ds(c * (M // 4), M // 4)
                    lo, hi = _unpack_pair_tok(st_b[h % 2, t, rows, :], tok)
                    w_b[t * H + 2 * h, rows, :] = lo
                    w_b[t * H + 2 * h + 1, rows, :] = hi

            xg = _as_bf16(x_s[pl.ds(pl.multiple_of(XPAD + h * (BQ // 2), 8), BQ // 2), :]).astype(f32)
            g = jax.nn.sigmoid(jnp.sum(xg * gw, axis=1, keepdims=True))
            g_s[pl.ds(pl.multiple_of(APAD + h * BQ, 8), BQ), :] = jnp.broadcast_to(g, (BQ, D))
            acc[pl.ds(pl.multiple_of(APAD + h * BQ, 8), BQ), :] = jnp.zeros((BQ, M), f32)

            for _, fn in a_tasks(h, False, on_scores):
                fn()
            return carry

        jax.lax.fori_loop(0, H1, a_body, 0)

        cp_mem.wait()
        cp_wob.wait()

        def wb(t, h):
            return _as_bf16(w_b.bitcast(u32)[t * H + h])

        def wob(g):
            return _as_bf16(wo_b[g * GB * D // 2:(g + 1) * GB * D // 2, :])

        def tile4(g):
            return jnp.concatenate([g] * (M // D), axis=1)

        mem_s[...] = mem0_s[...].astype(f32)

        x0 = _as_bf16(x_s[XPAD:XPAD + SEG // 2, :])
        for t in range(3):
            for h in range(H):
                y = jnp.dot(x0, wb(t, h), preferred_element_type=f32)
                if t == 0:
                    y = y * qscale
                qkv_s[0, :, (t * H + h) * D:(t * H + h + 1) * D] = y

        L = NM + SEG
        r80 = jax.lax.broadcasted_iota(jnp.int32, (2 * L, 2 * L), 0)
        c80 = jax.lax.broadcasted_iota(jnp.int32, (2 * L, 2 * L), 1)
        rhead = jnp.where(r80 < NM, 0, jnp.where(r80 < 2 * NM, 1, jnp.where(r80 < 2 * NM + SEG, 0, 1)))
        chead = jnp.where(c80 < L, 0, 1)
        rpos = jnp.where(r80 < 2 * NM, L - 1,
                         jnp.where(r80 < 2 * NM + SEG, r80 - 2 * NM + NM, r80 - 2 * NM - SEG + NM))
        cpos = jnp.where(c80 < L, c80, c80 - L)
        same = rhead == chead
        valid = jnp.logical_and(same, cpos <= rpos)
        fill = jnp.where(same, NEG, -3e38).astype(f32)

        def finalize(a0, n, z):
            acc[pl.ds(a0, n), :] += z + tile4(g_s[pl.ds(a0, n), :]) * (acc1[pl.ds(a0, n), :] - z)

        def b_step(step, get_xr, cur, stores, ox_parts, finish):
            v = {"z": None}
            memp, ps, om = {}, {}, {}

            def proj(h):
                if "lhs" not in v:
                    v["lhs"] = jnp.concatenate([mem_s[...], get_xr()], axis=0).astype(bf16)
                r = []
                for t in range(3):
                    y = jnp.dot(v["lhs"], wb(t, h), preferred_element_type=f32)
                    if t == 0:
                        y = y * qscale
                    c0 = (t * H + h) * D
                    for (y0, n, slot, d0) in stores:
                        qkv_s[slot, d0:d0 + n, c0:c0 + D] = y[y0:y0 + n]
                    r.append(y[:NM])
                memp[h] = r

            def scores(gg):
                for h0 in range(gg * GB, (gg + 1) * GB, 2):
                    h1 = h0 + 1

                    def xs(t, h):
                        return qkv_s[cur, :, (t * H + h) * D:(t * H + h + 1) * D]
                    q2 = jnp.concatenate([memp[h0][0], memp[h1][0], xs(0, h0), xs(0, h1)], axis=0).astype(bf16)
                    k2 = jnp.concatenate([memp[h0][1], xs(1, h0), memp[h1][1], xs(1, h1)], axis=0).astype(bf16)
                    v2 = jnp.concatenate([memp[h0][2], xs(2, h0), memp[h1][2], xs(2, h1)], axis=0).astype(bf16)
                    sc = jax.lax.dot_general(q2, k2, NT, preferred_element_type=f32)
                    sc = jnp.where(valid, sc, fill)
                    m = jnp.max(sc, axis=1, keepdims=True)
                    p = jnp.exp2(sc - m)
                    l = jnp.sum(p, axis=1, keepdims=True)
                    ps[h0] = (p.astype(bf16), _recip(l), v2)

            def pv(gg):
                for h0 in range(gg * GB, (gg + 1) * GB, 2):
                    h1 = h0 + 1
                    p, rl, v2 = ps.pop(h0)
                    o = jnp.dot(p, v2, preferred_element_type=f32) * rl
                    om[h0] = o[0:NM]
                    om[h1] = o[NM:2 * NM]
                    ox_s[cur, :, h0 * D:(h0 + 1) * D] = o[2 * NM:2 * NM + SEG]
                    ox_s[cur, :, h1 * D:(h1 + 1) * D] = o[2 * NM + SEG:]

            def oproj(gg):
                c0, c1 = gg * GB * D, (gg + 1) * GB * D
                parts = [jnp.concatenate([om[h] for h in range(gg * GB, (gg + 1) * GB)], axis=1)]
                parts += [ox_s[slot, r0:r1, c0:c1] for (slot, r0, r1) in ox_parts]
                lo = jnp.concatenate(parts, axis=0).astype(bf16)
                t = jnp.dot(lo, wob(gg), preferred_element_type=f32)
                v["z"] = t if v["z"] is None else v["z"] + t
                if gg == NG - 1:
                    mem_s[...] = v["z"][:NM].astype(bf16).astype(f32)
                    finish(v["z"][NM:])

            tasks = []
            for g in range(NG + 3):
                if g < NG:
                    for h in range(g * GB, (g + 1) * GB):
                        tasks.append(((step, "P", h), functools.partial(proj, h)))
                if 0 <= g - 1 < NG:
                    tasks.append(((step, "Sc", g - 1), functools.partial(scores, g - 1)))
                if 0 <= g - 2 < NG:
                    tasks.append(((step, "Pv", g - 2), functools.partial(pv, g - 2)))
                if 0 <= g - 3 < NG:
                    tasks.append(((step, "Op", g - 3), functools.partial(oproj, g - 3)))
                tasks.append(((step, "end", g), None))
            return tasks

        def b_pair(j, par):
            s0 = par * 2
            s1 = s0 + 1
            s2 = 2 - s0
            s3 = 3 - s0
            a0 = pl.multiple_of(j * 64, 64)
            v = {}

            def xn():
                if "xn" not in v:
                    v["xn"] = _as_bf16(x_s[pl.ds(pl.multiple_of(j * SEG + XPAD + 16, 8), SEG), :]).astype(f32)
                return v["xn"]

            ev = b_step(2 * par, lambda: xn()[0:40], s0, [(NM, SEG, s1, 0), (NM + SEG, NM, s2, 0)],
                        [(s2, SEG - NM, SEG), (s3, 0, SEG)],
                        lambda z: finalize(pl.multiple_of(a0 + (APAD - 40), 8), 40, z))
            od = b_step(2 * par + 1, lambda: xn()[40:64], s1, [(NM, SEG - NM, s2, NM)], [(s0, 0, SEG - NM)],
                        lambda z: finalize(pl.multiple_of(a0 + APAD, 8), 24, z))
            return ev + od

        NI = H - H1
        out_main = pltpu.make_async_copy(out_s.at[0:EMIT * BQ, :], out_hbm.at[0:EMIT * BQ, :], sem_out.at[0])
        out_last = pltpu.make_async_copy(out_s.at[EMIT * BQ:S, :], out_hbm.at[EMIT * BQ:S, :], sem_out.at[1])

        def f_body(i, carry):
            def on_emit(t):
                if t == EMIT - 1:
                    @pl.when(i == NI - 1)
                    def _():
                        out_main.start()

            at = a_tasks(H1 + i, True, lambda t, tok: None, on_emit)
            bt = b_pair(2 * i, 0) + b_pair(2 * i + 1, 1)
            for fn in _merge(at, bt):
                fn()
            return carry

        jax.lax.fori_loop(0, NI, f_body, 0)

        lo = jnp.concatenate([ox_s[2, SEG - NM:SEG, :], ox_s[3, :, :]], axis=0).astype(bf16)
        z = jnp.dot(lo, _as_bf16(wo_b[...]), preferred_element_type=f32)
        finalize(NPAIR * 64 + APAD - 40, 40, z)
        out_s[EMIT * BQ:S, :] = acc[APAD + EMIT * BQ:APAD + S, :].astype(bf16)
        out_last.start()
        out_main.wait()
        out_last.wait()

    scratch = [
        pltpu.VMEM((XPAD + S // 2 + XTAIL, M), u32),
        pltpu.VMEM((S // 2, M), u32),
        pltpu.VMEM((APAD + S, M), f32),
        pltpu.VMEM((APAD + S, M), f32),
        pltpu.VMEM((APAD + S, D), f32),
        pltpu.VMEM((S, D), bf16),
        pltpu.VMEM((S, D), bf16),
        pltpu.VMEM((S, D), bf16),
        pltpu.VMEM((NP2, 3, M, D), u32),
        pltpu.VMEM((HD // 2, M), u32),
        pltpu.VMEM((2, 3, M, D), u32),
        pltpu.VMEM((3 * H, M, D), bf16),
        pltpu.VMEM((HD // 2, M), u32),
        pltpu.VMEM((NM, M), bf16),
        pltpu.VMEM((1, M), bf16),
        pltpu.VMEM((NM, M), f32),
        pltpu.VMEM((4, SEG, 3 * HD), f32),
        pltpu.VMEM((4, SEG, HD), f32),
        pltpu.VMEM((S, M), bf16),
        pltpu.SemaphoreType.DMA((7,)),
        pltpu.SemaphoreType.DMA((3, 2)),
        pltpu.SemaphoreType.DMA((3, 2)),
        pltpu.SemaphoreType.DMA((2,)),
        pltpu.SemaphoreType.DMA((2 * NCH,)),
    ]
    return kernel, scratch


@functools.partial(jax.jit, static_argnames=("B_seg_len",))
def pallas_gated_mix__compressed_kv_cla__memory_aug_recurrent_mem_tr__prompt_kernel(
    A_x: jax.Array,
    A_c_kv: jax.Array,
    A_w_q: jax.Array,
    A_w_uk: jax.Array,
    A_w_uv: jax.Array,
    A_w_o: jax.Array,
    B_x: jax.Array,
    B_mem0: jax.Array,
    B_Wq: jax.Array,
    B_Wk: jax.Array,
    B_Wv: jax.Array,
    B_Wo: jax.Array,
    B_seg_len: int,
    gate_w: jax.Array,
):
    _, S, M = A_x.shape
    _, H, D = A_w_q.shape
    NM = B_mem0.shape[1]
    kernel, scratch = _make_kernel(S, M, H, D, NM, int(B_seg_len))
    any_spec = pl.BlockSpec(memory_space=pl.ANY)
    out = pl.pallas_call(
        kernel,
        out_shape=jax.ShapeDtypeStruct((S, M), bf16),
        in_specs=[any_spec] * 12,
        out_specs=any_spec,
        scratch_shapes=scratch,
        compiler_params=pltpu.CompilerParams(vmem_limit_bytes=100 * 1024 * 1024, disable_bounds_checks=True, disable_semaphore_checks=True),
    )(
        A_x.reshape(S, M), A_c_kv.reshape(S, M), A_w_q, A_w_uk, A_w_uv,
        A_w_o.reshape(H * D, M), B_mem0.reshape(NM, M),
        B_Wq, B_Wk, B_Wv, B_Wo.reshape(H * D, M), gate_w.reshape(1, M),
    )
    return out.reshape(1, S, M)
```

```python
import functools

import jax
import jax.numpy as jnp
import jax.experimental.pallas as pl
import jax.experimental.pallas.tpu as pltpu

bf16 = jnp.bfloat16
f32 = jnp.float32
u32 = jnp.uint32

LOG2E = 1.4426950408889634
NEG = -1e9 * LOG2E
NT = (((1,), (1,)), ((), ()))

BQ = 128
PCH = 512
GB = 4

JG = 4
JLA = 8
LA1 = 100000
LA2 = 256
MD2 = 448
MMIN = 4
NPEEL = 3
START0 = 24
STARTPOS = 3
WOWAIT = 2
W0 = {("Pk", 1): ("c1",), ("Pq", 1): ("x1", "wo"), ("Pk", 2): ("c2",), ("Pq", 2): ("x2",),
      ("Pk", 3): ("c3", "x3")}
MIDS = ((2, 5), (1, 3, 5), (2, 4, 6), (0, 2, 4, 6))
TSPLIT = (2, 5)
OSPLIT = (9, 13, 14, 15)


def _mo(x, m):
    return x if isinstance(x, int) else pl.multiple_of(x, m)


def _as_bf16(words):
    return pltpu.bitcast(words, bf16)


def _recip(l):
    r = pl.reciprocal(l, approx=True)
    return r * (2.0 - l * r)


def _unpack_head(words, par):
    if isinstance(par, int):
        w = jnp.bitwise_and(words, jnp.uint32(0xFFFF0000)) if par else jnp.left_shift(words, jnp.uint32(16))
        return pltpu.bitcast(w, f32).astype(bf16)
    sh = ((1 - par) * 16).astype(u32)
    w = jnp.bitwise_and(jnp.left_shift(words, sh), jnp.uint32(0xFFFF0000))
    return pltpu.bitcast(w, f32).astype(bf16)


def _token(v):
    f = pltpu.bitcast(jnp.right_shift(pltpu.bitcast(v[0:8, 0:128], u32), jnp.uint32(2)), f32)
    return pltpu.bitcast(f - f, u32)


def _token_all(v):
    v3 = v.reshape(v.shape[0] // 8, 8, v.shape[1])
    n = v3.shape[0]
    parts = [v3[i] for i in range(n)]
    while len(parts) > 1:
        parts = [jnp.maximum(parts[i], parts[i + 1]) for i in range(0, len(parts), 2)]
    return _token(parts[0])


def _unpack_head_tok(words, par, tok):
    r, c = words.shape
    if isinstance(par, int):
        w3 = words.reshape(r // 8, 8, c)
        if par:
            w = jnp.bitwise_and(w3, jnp.bitwise_or(tok, jnp.uint32(0xFFFF0000))[None])
        else:
            w = jnp.left_shift(w3, (tok + jnp.uint32(16))[None])
        return pltpu.bitcast(w.reshape(r, c), f32).astype(bf16)
    sh = ((1 - par) * 16).astype(u32) + tok
    mask = jnp.bitwise_or(tok, jnp.uint32(0xFFFF0000))
    w = jnp.bitwise_and(jnp.left_shift(words.reshape(r // 8, 8, c), sh[None]), mask[None])
    return pltpu.bitcast(w.reshape(r, c), f32).astype(bf16)


def _unpack_pair_tok(words, tok):
    r, c = words.shape
    w3 = words.reshape(r // 8, 8, c)
    lo = jnp.left_shift(w3, (tok + jnp.uint32(16))[None])
    hi = jnp.bitwise_and(w3, jnp.bitwise_or(tok, jnp.uint32(0xFFFF0000))[None])
    return (pltpu.bitcast(lo.reshape(r, c), f32).astype(bf16),
            pltpu.bitcast(hi.reshape(r, c), f32).astype(bf16))


def _a_schedule(nq, bpc, fused):
    assert nq == 16 and bpc == 4
    out = []
    fill = {0: ("Pk", 1, None), 1: ("Pq", 1, None), 2: ("Pv", 1, None),
            4: ("Pk", 2, 2), 5: ("Pq", 2, 3), 6: ("Pv", 2, 4),
            8: ("Pk", 3, 6), 9: ("Pq", 3, 7), 10: ("Pv", 3, 8)}
    for t in range(nq - 1):
        out.append(("S", t, None))
        if t in fill:
            out.append(fill[t])
        if t >= 1:
            out.append(("O", t - 1, None))
        if t >= 2:
            out.append(("F", t - 2, None))
    if fused:
        out += [("S", 15, None), ("O", 14, None), ("F", 13, None), ("O", 15, None), ("F", 14, None),
                ("F", 15, None), ("Nk", 0, 13), ("Nq", 0, 14), ("Nv", 0, 15)]
    else:
        out += [("S", 15, None), ("Nk", 0, 13), ("O", 14, None), ("F", 13, None), ("Nq", 0, 14),
                ("O", 15, None), ("F", 14, None), ("Nv", 0, 15), ("F", 15, None)]
    return out


def _units(a_tasks):
    units = []
    for name, fn in a_tasks:
        if name[0] == "S":
            units.append([])
        units[-1].append((name, fn))
    return units


def _merge(a_tasks, b_tasks):
    units = _units(a_tasks)
    plan = {}
    u = 0
    for step in range(4):
        for g in MIDS[step]:
            plan.setdefault((step, "end", g), []).extend(units[u])
            u += 1
        t = units[u]
        u += 1
        a, b = (1, 2) if step < 3 else TSPLIT
        plan[(step, "Sc", 7)] = t[0:a]
        plan[(step, "Pv", 7)] = t[a:b]
        plan[(step, "Op", 7)] = t[b:]
    assert u == len(units)
    out = []
    for name, fn in b_tasks:
        if fn is not None:
            out.append(fn)
        out += [f for _, f in plan.pop(name, [])]
    assert not plan, plan
    return out


def _make_kernel(S, M, H, D, NM, SEG):
    assert SEG == 32 and NM == 8 and D == 128 and S % PCH == 0 and H % 2 == 0 and H % GB == 0
    NQ = S // BQ
    NPAIR = S // (2 * SEG)
    NG = H // GB
    HD = H * D
    NCH = S // PCH
    H1 = H // 2
    NP2 = H // 2
    assert NPAIR == 2 * (H - H1) and NQ == H1 and NP2 == H1
    qscale = D ** -0.5 * LOG2E
    a_sched1 = _a_schedule(NQ, PCH // BQ, False)
    a_sched2 = _a_schedule(NQ, PCH // BQ, True)

    def kernel(x_hbm, c_hbm, wq_hbm, wk_hbm, wv_hbm, wo_hbm, mem0_hbm,
               bq_hbm, bk_hbm, bv_hbm, bo_hbm, gw_hbm, out_hbm,
               x_s, c_s, acc1, acc, g_s, q_s, k_s, v_s, st_a, wo_a, st_b, w_b, wo_b,
               mem0_s, gw_s, mem_s, qkv_s, ox_s, out_s,
               sem_in, sem_a, sem_b, sem_out, sem_xc):
        a_w_hbm = (wk_hbm, wq_hbm, wv_hbm)
        b_w_hbm = (bq_hbm, bk_hbm, bv_hbm)

        def a_copies(p):
            return [pltpu.make_async_copy(a_w_hbm[t].bitcast(u32).at[:, p, :], st_a.at[p, t],
                                          sem_a.at[t]) for t in range(3)]

        def b_copies(p):
            return [pltpu.make_async_copy(b_w_hbm[t].bitcast(u32).at[:, p, :], st_b.at[p % 2, t],
                                          sem_b.at[t]) for t in range(3)]

        cp_x = [pltpu.make_async_copy(x_hbm.bitcast(u32).at[c * (PCH // 2):(c + 1) * (PCH // 2), :],
                                      x_s.at[c * (PCH // 2):(c + 1) * (PCH // 2), :], sem_xc.at[c])
                for c in range(NCH)]
        cp_c = [pltpu.make_async_copy(c_hbm.bitcast(u32).at[c * (PCH // 2):(c + 1) * (PCH // 2), :],
                                      c_s.at[c * (PCH // 2):(c + 1) * (PCH // 2), :], sem_xc.at[NCH + c])
                for c in range(NCH)]
        cp_woa0 = pltpu.make_async_copy(wo_hbm.bitcast(u32).at[pl.ds(0, D), :], wo_a.at[pl.ds(0, D), :], sem_a.at[3])
        cp_woa = pltpu.make_async_copy(wo_hbm.bitcast(u32).at[D:HD // 2, :], wo_a.at[D:HD // 2, :], sem_b.at[3])
        cp_wob = pltpu.make_async_copy(bo_hbm.bitcast(u32), wo_b, sem_in.at[2])
        cp_mem = pltpu.make_async_copy(mem0_hbm, mem0_s, sem_in.at[0])
        cp_gw = pltpu.make_async_copy(gw_hbm, gw_s, sem_in.at[1])

        first = a_copies(0)
        cp_gw.start()
        first[0].start()
        cp_c[0].start()
        first[1].start()
        cp_x[0].start()
        first[2].start()
        for c in range(1, NCH):
            cp_c[c].start()
            cp_x[c].start()
            if c == 1:
                cp_woa0.start()
        cp_mem.start()

        for (srcr, t, dst, sc, pre) in ((c_s, 0, k_s, None, [first[0], cp_c[0]]),
                                        (x_s, 1, q_s, qscale, [first[1], cp_x[0]]),
                                        (c_s, 2, v_s, None, [first[2]])):
            for cp in pre:
                cp.wait()
            y = jnp.dot(_as_bf16(srcr[0:PCH // 2, :]), _unpack_head(st_a[0, t], jnp.int32(0)),
                        preferred_element_type=f32)
            if sc is not None:
                y = y * sc
            dst[0:PCH, :] = y.astype(bf16)
        cp_gw.wait()

        row = jax.lax.broadcasted_iota(jnp.int32, (BQ, BQ), 0)
        col = jax.lax.broadcasted_iota(jnp.int32, (BQ, BQ), 1)
        tri = col <= row

        def tie(words, tok, r=0):
            if tok is None:
                return words
            n, c = words.shape
            blk = words[r:r + 8]
            if c > 128:
                blk = jnp.concatenate([jnp.bitwise_or(blk[:, :128], tok), blk[:, 128:]], axis=1)
            else:
                blk = jnp.bitwise_or(blk, tok)
            parts = ([words[:r]] if r else []) + [blk] + ([words[r + 8:]] if r + 8 < n else [])
            return jnp.concatenate(parts, axis=0)

        def ldp(ref, r0, r1, tok=None):
            return _as_bf16(tie(ref.bitcast(u32)[r0 // 2:r1 // 2, :], tok))

        def a_tasks(h, fused, on_scores, on_emit=None, spar=None, first_head=False):
            st = {}
            toks = {}
            marks, clock, due = [], [0], []

            def take(time):
                tk = None
                for tm, v in [d for d in due if d[0] <= time]:
                    t = _token_all(v)
                    tk = t if tk is None else jnp.bitwise_or(tk, t)
                due[:] = [d for d in due if d[0] > time]
                return tk

            def anchor(time):
                best = None
                for tm, v in marks:
                    if tm <= time:
                        best = v
                return best

            def proj(src, t, dst, sc, c, hh, tk):
                r = c * PCH
                hh, nxt = hh
                words = st_a[(hh // 2) % NP2, t]
                par = hh % 2 if spar is None else (spar + nxt) % 2
                if tk is None:
                    w = _unpack_head(words, par)
                else:
                    w = _unpack_head_tok(words, par, toks[tk])
                lhs = src[r // 2:(r + PCH) // 2, :]
                for rr in range(0, PCH, BQ):
                    lhs = tie(lhs, take(clock[0] + rr), rr // 2)
                y = jnp.dot(_as_bf16(lhs), w, preferred_element_type=f32)
                for rr in range(64, PCH, 64):
                    marks.append((clock[0] + rr, y[rr:rr + 8]))
                clock[0] += PCH
                if sc is not None:
                    y = y * sc
                dst[r:r + PCH, :] = y.astype(bf16)

            def scores(i):
                r0 = i * BQ
                qw = q_s.bitcast(u32)[r0 // 2:(r0 + BQ) // 2, :]
                ss = []
                mm = None
                for j in range(i + 1):
                    tk = take(clock[0] + (j // 4) * BQ) if j % 4 == 0 else None
                    s = jax.lax.dot_general(_as_bf16(tie(qw, tk)), ldp(k_s, j * BQ, (j + 1) * BQ), NT,
                                            preferred_element_type=f32)
                    marks.append((clock[0] + min(BQ * (j // 4 + 1), (i + 1) * BQ // 4), s))
                    if j == i:
                        s = jnp.where(tri, s, NEG)
                    mm = s if mm is None else jnp.maximum(mm, s)
                    if (j % 4 == 3 or j == i) and i >= MMIN and fused:
                        due.append((clock[0] + min(BQ * (j // 4 + 1), (i + 1) * BQ // 4) + MD2, mm))
                    ss.append(s)
                clock[0] += (i + 1) * BQ // 4
                toks[i] = _token(mm)
                m = jnp.max(mm, axis=1, keepdims=True)
                st[i] = (ss, m)
                on_scores(i, toks[i])

            def pv(i):
                ss, m = st[i]
                m = jnp.broadcast_to(m, (BQ, BQ))
                o = None
                l = None
                ts = []
                for j, s in enumerate(ss):
                    if j % JG == 0:
                        av = ts[j - JLA] if j >= JLA else anchor(clock[0] + (j // 4) * BQ - (LA2 if fused else LA1))
                        if av is not None:
                            tok = pltpu.bitcast(_token(av), f32)
                            m = (m.reshape(BQ // 8, 8, BQ) + tok[None]).reshape(BQ, BQ)
                    p = jnp.exp2(s - m)
                    l = p if l is None else l + p
                    tk = take(clock[0] + (j // 4) * BQ) if j % 4 == 0 else None
                    pb = p.astype(bf16)
                    if tk is not None:
                        pb = _as_bf16(tie(pltpu.bitcast(pb, u32), tk))
                    t = jnp.dot(pb, ldp(v_s, j * BQ, (j + 1) * BQ), preferred_element_type=f32)
                    ts.append(t)
                    o = t if o is None else o + t
                for j, t in enumerate(ts):
                    marks.append((clock[0] + min(BQ * (j // 4 + 1), (i + 1) * BQ // 4), t))
                clock[0] += (i + 1) * BQ // 4
                o = o * _recip(jnp.sum(l, axis=1, keepdims=True))
                if fused:
                    o = o * g_s[i * BQ:(i + 1) * BQ, :]
                st[i] = o.astype(bf16)

            def outproj(i):
                r0 = i * BQ
                w = _as_bf16(wo_a[pl.ds(_mo(h * (D // 2), D // 2), D // 2), :])
                dst = acc if fused else acc1
                lhs = st[i]
                tk = take(clock[0])
                if tk is not None:
                    lhs = _as_bf16(tie(pltpu.bitcast(lhs, u32), tk))
                d = jnp.dot(lhs, w, preferred_element_type=f32)
                marks.append((clock[0] + BQ // 2, d[BQ // 2:BQ // 2 + 8]))
                marks.append((clock[0] + BQ, d[BQ - 8:BQ]))
                clock[0] += BQ
                a = d if first_head else dst[r0:r0 + BQ, :] + d
                dst[r0:r0 + BQ, :] = a
                if fused:
                    out_s[i * BQ:(i + 1) * BQ, :] = a.astype(bf16)
                    on_emit(i)

            out = []
            for kind, i, tk in (a_sched2 if fused else a_sched1):
                hh = (h, 0) if kind[0] == "P" else (h + 1, 1)
                if kind in ("Pk", "Nk"):
                    fn = functools.partial(proj, c_s, 0, k_s, None, i, hh, tk)
                elif kind in ("Pq", "Nq"):
                    fn = functools.partial(proj, x_s, 1, q_s, qscale, i, hh, tk)
                elif kind in ("Pv", "Nv"):
                    fn = functools.partial(proj, c_s, 2, v_s, None, i, hh, tk)
                elif kind == "S":
                    fn = functools.partial(scores, i)
                elif kind == "O":
                    fn = functools.partial(pv, i)
                else:
                    fn = functools.partial(outproj, i)
                out.append(((kind, i), fn))
            return out

        def unpack_b(p, t, c, tok):
            rows = pl.ds(c * (M // 4), M // 4)
            lo, hi = _unpack_pair_tok(st_b[p % 2, t, rows, :], tok)
            w_b[t * H + 2 * p, rows, :] = lo
            w_b[t * H + 2 * p + 1, rows, :] = hi

        gw = gw_s[...].astype(f32).reshape(1, M)

        def a_head(h, first_head):
            if not first_head:
                for cp in a_copies(h) + b_copies(h - 1):
                    cp.wait()

            nxt = a_copies((h + 1) % NP2) + b_copies(h)
            if isinstance(h, int) and h == WOWAIT:
                cp_woa.wait()

            def on_scores(i, tok):
                if 1 <= i <= 12 and not first_head:
                    unpack_b(h - 1, (i - 1) // 4, (i - 1) % 4, tok)

            xg = _as_bf16(x_s[pl.ds(_mo(h * (BQ // 2), 8), BQ // 2), :]).astype(f32)
            g = jax.nn.sigmoid(jnp.sum(xg * gw, axis=1, keepdims=True))
            g_s[pl.ds(_mo(h * BQ, 8), BQ), :] = jnp.broadcast_to(g, (BQ, D))
            acc[pl.ds(_mo(h * BQ, 8), BQ), :] = jnp.zeros((BQ, M), f32)

            waits = {}
            if first_head:
                waits = {task: [cp_woa0 if cp == "wo" else (cp_c if cp[0] == "c" else cp_x)[int(cp[1])]
                                for cp in cps] for task, cps in W0.items()}

            for n, (name, fn) in enumerate(a_tasks(h, False, on_scores, spar=h % 2 if isinstance(h, int) else None,
                                                   first_head=first_head)):
                for cp in waits.pop(name, []):
                    cp.wait()
                fn()
                if n == (START0 if first_head else STARTPOS):
                    for cp in nxt + ([cp_woa, cp_wob] if first_head else []):
                        cp.start()
            assert not waits

        def a_body(h, carry):
            a_head(h, False)
            return carry

        a_head(0, True)
        for hp in range(1, NPEEL):
            a_head(hp, False)
        jax.lax.fori_loop(NPEEL, H1, a_body, 0)

        cp_mem.wait()
        cp_wob.wait()

        def wb(t, h):
            return _as_bf16(w_b.bitcast(u32)[t * H + h])

        def wob(g):
            return _as_bf16(wo_b[g * GB * D // 2:(g + 1) * GB * D // 2, :])

        def tile4(g):
            return jnp.concatenate([g] * (M // D), axis=1)

        mem_s[...] = mem0_s[...].astype(f32)

        for cp in a_copies(0) + b_copies(H1 - 1):
            cp.wait()
        ztok = jnp.zeros((8, D), u32)
        for n in range(12):
            unpack_b(NP2 - 1, n // 4, n % 4, ztok)

        L = NM + SEG
        r80 = jax.lax.broadcasted_iota(jnp.int32, (2 * L, 2 * L), 0)
        c80 = jax.lax.broadcasted_iota(jnp.int32, (2 * L, 2 * L), 1)
        rhead = jnp.where(r80 < NM, 0, jnp.where(r80 < 2 * NM, 1, jnp.where(r80 < 2 * NM + SEG, 0, 1)))
        chead = jnp.where(c80 < L, 0, 1)
        rpos = jnp.where(r80 < 2 * NM, L - 1,
                         jnp.where(r80 < 2 * NM + SEG, r80 - 2 * NM + NM, r80 - 2 * NM - SEG + NM))
        cpos = jnp.where(c80 < L, c80, c80 - L)
        same = rhead == chead
        valid = jnp.logical_and(same, cpos <= rpos)
        fill = jnp.where(same, NEG, -3e38).astype(f32)

        def finalize(a0, n, z):
            acc[pl.ds(a0, n), :] += z + tile4(g_s[pl.ds(a0, n), :]) * (acc1[pl.ds(a0, n), :] - z)

        def b_step(step, get_xr, cur, stores, ox_parts, finish):
            v = {"z": None}
            memp, ps, om = {}, {}, {}

            def proj(h):
                if "lhs" not in v:
                    v["lhs"] = jnp.concatenate([mem_s[...], get_xr()], axis=0).astype(bf16)
                r = []
                for t in range(3):
                    y = jnp.dot(v["lhs"], wb(t, h), preferred_element_type=f32)
                    if t == 0:
                        y = y * qscale
                    c0 = (t * H + h) * D
                    for (y0, n, slot, d0) in stores:
                        qkv_s[slot, d0:d0 + n, c0:c0 + D] = y[y0:y0 + n]
                    r.append(y[:NM])
                memp[h] = r

            def scores(gg):
                for h0 in range(gg * GB, (gg + 1) * GB, 2):
                    h1 = h0 + 1

                    def xs(t, h):
                        return qkv_s[cur, :, (t * H + h) * D:(t * H + h + 1) * D]
                    q2 = jnp.concatenate([memp[h0][0], memp[h1][0], xs(0, h0), xs(0, h1)], axis=0).astype(bf16)
                    k2 = jnp.concatenate([memp[h0][1], xs(1, h0), memp[h1][1], xs(1, h1)], axis=0).astype(bf16)
                    v2 = jnp.concatenate([memp[h0][2], xs(2, h0), memp[h1][2], xs(2, h1)], axis=0).astype(bf16)
                    sc = jax.lax.dot_general(q2, k2, NT, preferred_element_type=f32)
                    sc = jnp.where(valid, sc, fill)
                    m = jnp.max(sc, axis=1, keepdims=True)
                    p = jnp.exp2(sc - m)
                    l = jnp.sum(p, axis=1, keepdims=True)
                    ps[h0] = (p.astype(bf16), _recip(l), v2)

            def pv(gg):
                for h0 in range(gg * GB, (gg + 1) * GB, 2):
                    h1 = h0 + 1
                    p, rl, v2 = ps.pop(h0)
                    o = jnp.dot(p, v2, preferred_element_type=f32) * rl
                    om[h0] = o[0:NM]
                    om[h1] = o[NM:2 * NM]
                    ox_s[cur, :, h0 * D:(h0 + 1) * D] = o[2 * NM:2 * NM + SEG]
                    ox_s[cur, :, h1 * D:(h1 + 1) * D] = o[2 * NM + SEG:]

            def oproj(gg):
                c0, c1 = gg * GB * D, (gg + 1) * GB * D
                parts = [jnp.concatenate([om[h] for h in range(gg * GB, (gg + 1) * GB)], axis=1)]
                parts += [ox_s[slot, r0:r1, c0:c1] for (slot, r0, r1) in ox_parts]
                lo = jnp.concatenate(parts, axis=0).astype(bf16)
                t = jnp.dot(lo, wob(gg), preferred_element_type=f32)
                v["z"] = t if v["z"] is None else v["z"] + t
                if gg == NG - 1:
                    mem_s[...] = v["z"][:NM].astype(bf16).astype(f32)
                    finish(v["z"][NM:])

            tasks = []
            for g in range(NG + 3):
                if g < NG:
                    for h in range(g * GB, (g + 1) * GB):
                        tasks.append(((step, "P", h), functools.partial(proj, h)))
                if 0 <= g - 1 < NG:
                    tasks.append(((step, "Sc", g - 1), functools.partial(scores, g - 1)))
                if 0 <= g - 2 < NG:
                    tasks.append(((step, "Pv", g - 2), functools.partial(pv, g - 2)))
                if 0 <= g - 3 < NG:
                    tasks.append(((step, "Op", g - 3), functools.partial(oproj, g - 3)))
                tasks.append(((step, "end", g), None))
            return tasks

        def b_pair(j, par):
            s0 = par * 2
            s1 = s0 + 1
            a0 = pl.multiple_of(j * 64, 64)
            v = {}

            def xn():
                if "xn" not in v:
                    v["xn"] = _as_bf16(x_s[pl.ds(pl.multiple_of(j * SEG, 8), SEG), :]).astype(f32)
                return v["xn"]

            ev = b_step(2 * par, lambda: xn()[0:40], s0, [(NM, SEG, s0, 0), (NM + SEG, NM, s1, 0)],
                        [(s0, 0, SEG - NM)],
                        lambda z: finalize(a0, 24, z))
            od = b_step(2 * par + 1, lambda: xn()[40:64], s1, [(NM, SEG - NM, s1, NM)],
                        [(s0, SEG - NM, SEG), (s1, 0, SEG)],
                        lambda z: finalize(pl.multiple_of(a0 + 24, 8), 40, z))
            return ev + od

        NI = H - H1
        bounds = [0] + [t + 1 for t in OSPLIT]
        assert bounds[-1] == NQ
        out_cp = [pltpu.make_async_copy(out_s.at[bounds[n] * BQ:bounds[n + 1] * BQ, :],
                                        out_hbm.at[bounds[n] * BQ:bounds[n + 1] * BQ, :], sem_out.at[n])
                  for n in range(len(bounds) - 1)]

        def f_body(i, carry):
            def on_emit(t):
                if t in OSPLIT:
                    @pl.when(i == NI - 1)
                    def _():
                        out_cp[OSPLIT.index(t)].start()

            at = a_tasks(H1 + i, True, lambda t, tok: None, on_emit)
            bt = b_pair(2 * i, 0) + b_pair(2 * i + 1, 1)
            for fn in _merge(at, bt):
                fn()
            return carry

        jax.lax.fori_loop(0, NI, f_body, 0)

        for cp in out_cp:
            cp.wait()

    scratch = [
        pltpu.VMEM((S // 2, M), u32),
        pltpu.VMEM((S // 2, M), u32),
        pltpu.VMEM((S, M), f32),
        pltpu.VMEM((S, M), f32),
        pltpu.VMEM((S, D), f32),
        pltpu.VMEM((S, D), bf16),
        pltpu.VMEM((S, D), bf16),
        pltpu.VMEM((S, D), bf16),
        pltpu.VMEM((NP2, 3, M, D), u32),
        pltpu.VMEM((HD // 2, M), u32),
        pltpu.VMEM((2, 3, M, D), u32),
        pltpu.VMEM((3 * H, M, D), bf16),
        pltpu.VMEM((HD // 2, M), u32),
        pltpu.VMEM((NM, M), bf16),
        pltpu.VMEM((M,), bf16),
        pltpu.VMEM((NM, M), f32),
        pltpu.VMEM((4, SEG, 3 * HD), f32),
        pltpu.VMEM((4, SEG, HD), f32),
        pltpu.VMEM((S, M), bf16),
        pltpu.SemaphoreType.DMA((3,)),
        pltpu.SemaphoreType.DMA((4,)),
        pltpu.SemaphoreType.DMA((4,)),
        pltpu.SemaphoreType.DMA((len(OSPLIT),)),
        pltpu.SemaphoreType.DMA((2 * NCH,)),
    ]
    return kernel, scratch


@functools.partial(jax.jit, static_argnames=("B_seg_len",))
def pallas_gated_mix__compressed_kv_cla__memory_aug_recurrent_mem_tr__prompt_kernel(
    A_x: jax.Array,
    A_c_kv: jax.Array,
    A_w_q: jax.Array,
    A_w_uk: jax.Array,
    A_w_uv: jax.Array,
    A_w_o: jax.Array,
    B_x: jax.Array,
    B_mem0: jax.Array,
    B_Wq: jax.Array,
    B_Wk: jax.Array,
    B_Wv: jax.Array,
    B_Wo: jax.Array,
    B_seg_len: int,
    gate_w: jax.Array,
):
    _, S, M = A_x.shape
    _, H, D = A_w_q.shape
    NM = B_mem0.shape[1]
    kernel, scratch = _make_kernel(S, M, H, D, NM, int(B_seg_len))
    any_spec = pl.BlockSpec(memory_space=pl.ANY)
    out = pl.pallas_call(
        kernel,
        out_shape=jax.ShapeDtypeStruct((S, M), bf16),
        in_specs=[any_spec] * 12,
        out_specs=any_spec,
        scratch_shapes=scratch,
        compiler_params=pltpu.CompilerParams(vmem_limit_bytes=100 * 1024 * 1024, disable_bounds_checks=True,
                                             disable_semaphore_checks=True),
    )(
        A_x.reshape(S, M), A_c_kv.reshape(S, M), A_w_q, A_w_uk, A_w_uv,
        A_w_o.reshape(H * D, M), B_mem0.reshape(NM, M),
        B_Wq, B_Wk, B_Wv, B_Wo.reshape(H * D, M), gate_w,
    )
    return out.reshape(1, S, M)
```

```python
import functools

import jax
import jax.numpy as jnp
import jax.experimental.pallas as pl
import jax.experimental.pallas.tpu as pltpu

bf16 = jnp.bfloat16
f32 = jnp.float32
u32 = jnp.uint32

LOG2E = 1.4426950408889634
NEG = -1e9 * LOG2E
NT = (((1,), (1,)), ((), ()))

BQ = 128
PCH = 512
GB = 4

JG = 4
JLA = 8
LA1 = 100000
LA2 = 256
MD2 = 448
MMIN = 4
HALF = 256
SPLIT1 = 3
STARTPOS = 3
DORD = "gw wk c0a c0b wv wq x0 c1 x1 wo c2 x2 c3 x3 mem".split()
H0 = ("w:wk+c0a Pk0a Tk0a w:c0b+wv Pk0b Tk0b Pv0 Tv0 w:wq+x0+gw Pq0 G0 Tq0 S0 S1 O0 S2 O1 S3 O2 O3 "
      "w:c1 Pk1 Pv1 w:x1+wo Pq1 F0 F1 S4 F2 S5 O4 F3 S6 O5 F4 w:c2+x2 Pk2 S7 O6 F5 Pq2 O7 F6 Pv2 F7 S8 "
      "w:c3+x3 Pk3").split()
MIDS = ((2, 5), (1, 3, 5), (2, 4, 6), (0, 2, 4, 6))
TSPLIT = (2, 5)
OSPLIT = (9, 13, 14, 15)


def _mo(x, m):
    return x if isinstance(x, int) else pl.multiple_of(x, m)


def _as_bf16(words):
    return pltpu.bitcast(words, bf16)


def _recip(l):
    r = pl.reciprocal(l, approx=True)
    return r * (2.0 - l * r)


def _unpack_head(words, par):
    if isinstance(par, int):
        w = jnp.bitwise_and(words, jnp.uint32(0xFFFF0000)) if par else jnp.left_shift(words, jnp.uint32(16))
        return pltpu.bitcast(w, f32).astype(bf16)
    sh = ((1 - par) * 16).astype(u32)
    w = jnp.bitwise_and(jnp.left_shift(words, sh), jnp.uint32(0xFFFF0000))
    return pltpu.bitcast(w, f32).astype(bf16)


def _token(v):
    f = pltpu.bitcast(jnp.right_shift(pltpu.bitcast(v[0:8, 0:128], u32), jnp.uint32(2)), f32)
    return pltpu.bitcast(f - f, u32)


def _token_all(v):
    v3 = v.reshape(v.shape[0] // 8, 8, v.shape[1])
    n = v3.shape[0]
    parts = [v3[i] for i in range(n)]
    while len(parts) > 1:
        parts = [jnp.maximum(parts[i], parts[i + 1]) for i in range(0, len(parts), 2)]
    return _token(parts[0])


def _unpack_head_tok(words, par, tok):
    r, c = words.shape
    if isinstance(par, int):
        w3 = words.reshape(r // 8, 8, c)
        if par:
            w = jnp.bitwise_and(w3, jnp.bitwise_or(tok, jnp.uint32(0xFFFF0000))[None])
        else:
            w = jnp.left_shift(w3, (tok + jnp.uint32(16))[None])
        return pltpu.bitcast(w.reshape(r, c), f32).astype(bf16)
    sh = ((1 - par) * 16).astype(u32) + tok
    mask = jnp.bitwise_or(tok, jnp.uint32(0xFFFF0000))
    w = jnp.bitwise_and(jnp.left_shift(words.reshape(r // 8, 8, c), sh[None]), mask[None])
    return pltpu.bitcast(w.reshape(r, c), f32).astype(bf16)


def _unpack_pair_tok(words, tok):
    r, c = words.shape
    w3 = words.reshape(r // 8, 8, c)
    lo = jnp.left_shift(w3, (tok + jnp.uint32(16))[None])
    hi = jnp.bitwise_and(w3, jnp.bitwise_or(tok, jnp.uint32(0xFFFF0000))[None])
    return (pltpu.bitcast(lo.reshape(r, c), f32).astype(bf16),
            pltpu.bitcast(hi.reshape(r, c), f32).astype(bf16))


def _first_schedule(base):
    tk = {(k, i): t for k, i, t in base}
    head = []
    for s in H0:
        if s.startswith("w:"):
            head.append(("w", tuple(s[2:].split("+")), None))
        else:
            nm = (s[:-1], int(s[-1])) if s[0] in "SOFG" else (s[:2], int(s[2]) if len(s) == 3 else s[2:])
            head.append(nm + (tk.get(nm),))
    used = {(k, i) for k, i, _ in head}
    rest = [(k, i, t) for k, i, t in base if (k, i) not in used]
    rest = [("C" + k[1], i, t) if k[0] == "N" else (k, i, t) for k, i, t in rest]
    return head + rest


def _a_schedule(nq, bpc, fused):
    assert nq == 16 and bpc == 4
    out = []
    fill = {0: ("Pk", 1, None), 1: ("Pq", 1, None), 2: ("Pv", 1, None),
            4: ("Pk", 2, 2), 5: ("Pq", 2, 3), 6: ("Pv", 2, 4),
            8: ("Pk", 3, 6), 9: ("Pq", 3, 7), 10: ("Pv", 3, 8)}
    for t in range(nq - 1):
        out.append(("S", t, None))
        if t in fill:
            out.append(fill[t])
        if t >= 1:
            out.append(("O", t - 1, None))
        if t >= 2:
            out.append(("F", t - 2, None))
    if fused:
        out += [("S", 15, None), ("O", 14, None), ("F", 13, None), ("O", 15, None), ("F", 14, None),
                ("F", 15, None), ("Nk", 0, 13), ("Nq", 0, 14), ("Nv", 0, 15)]
    else:
        out += [("S", 15, None), ("Nk", 0, 13), ("O", 14, None), ("F", 13, None), ("Nq", 0, 14),
                ("O", 15, None), ("F", 14, None), ("Nv", 0, 15), ("F", 15, None)]
    return out


def _units(a_tasks):
    units = []
    for name, fn in a_tasks:
        if name[0] == "S":
            units.append([])
        units[-1].append((name, fn))
    return units


def _merge(a_tasks, b_tasks):
    units = _units(a_tasks)
    plan = {}
    u = 0
    for step in range(4):
        for g in MIDS[step]:
            plan.setdefault((step, "end", g), []).extend(units[u])
            u += 1
        t = units[u]
        u += 1
        a, b = (1, 2) if step < 3 else TSPLIT
        plan[(step, "Sc", 7)] = t[0:a]
        plan[(step, "Pv", 7)] = t[a:b]
        plan[(step, "Op", 7)] = t[b:]
    assert u == len(units)
    out = []
    for name, fn in b_tasks:
        if fn is not None:
            out.append(fn)
        out += [f for _, f in plan.pop(name, [])]
    assert not plan, plan
    return out


def _make_kernel(S, M, H, D, NM, SEG):
    assert SEG == 32 and NM == 8 and D == 128 and S % PCH == 0 and H % 2 == 0 and H % GB == 0
    NQ = S // BQ
    NPAIR = S // (2 * SEG)
    NG = H // GB
    HD = H * D
    NCH = S // PCH
    H1 = H // 2
    NP2 = H // 2
    assert NPAIR == 2 * (H - H1) and NQ == H1 and NP2 == H1
    qscale = D ** -0.5 * LOG2E
    a_sched1 = _a_schedule(NQ, PCH // BQ, False)
    a_sched2 = _a_schedule(NQ, PCH // BQ, True)
    a_sched0 = _first_schedule(a_sched1)

    def kernel(x_hbm, c_hbm, wq_hbm, wk_hbm, wv_hbm, wo_hbm, mem0_hbm,
               bq_hbm, bk_hbm, bv_hbm, bo_hbm, gw_hbm, out_hbm,
               x_s, c_s, acc1, acc, g_s, q_s, k_s, v_s, st_a, wo_a, st_b, w_b, wo_b,
               mem0_s, gw_s, mem_s, qkv_s, ox_s, out_s, tmp_s,
               sem_in, sem_a, sem_b, sem_out, sem_xc, sem_f):
        a_w_hbm = (wk_hbm, wq_hbm, wv_hbm)
        b_w_hbm = (bq_hbm, bk_hbm, bv_hbm)

        def a_copies(p, sem=sem_a):
            return [pltpu.make_async_copy(a_w_hbm[t].bitcast(u32).at[:, p, :], st_a.at[p, t],
                                          sem.at[t]) for t in range(3)]

        def b_copies(p):
            return [pltpu.make_async_copy(b_w_hbm[t].bitcast(u32).at[:, p, :], st_b.at[p % 2, t],
                                          sem_b.at[t]) for t in range(3)]

        cp_x = [pltpu.make_async_copy(x_hbm.bitcast(u32).at[c * (PCH // 2):(c + 1) * (PCH // 2), :],
                                      x_s.at[c * (PCH // 2):(c + 1) * (PCH // 2), :], sem_xc.at[c])
                for c in range(NCH)]
        cp_c = {c: pltpu.make_async_copy(c_hbm.bitcast(u32).at[c * (PCH // 2):(c + 1) * (PCH // 2), :],
                                         c_s.at[c * (PCH // 2):(c + 1) * (PCH // 2), :], sem_xc.at[NCH + c])
                for c in range(1, NCH)}
        cp_woa0 = pltpu.make_async_copy(wo_hbm.bitcast(u32).at[pl.ds(0, D), :], wo_a.at[pl.ds(0, D), :], sem_a.at[3])
        cp_woa1 = pltpu.make_async_copy(wo_hbm.bitcast(u32).at[D:2 * D, :], wo_a.at[D:2 * D, :], sem_in.at[3])
        cp_woa = pltpu.make_async_copy(wo_hbm.bitcast(u32).at[2 * D:HD // 2, :], wo_a.at[2 * D:HD // 2, :], sem_b.at[3])
        cp_wob = pltpu.make_async_copy(bo_hbm.bitcast(u32), wo_b, sem_in.at[2])
        cp_mem = pltpu.make_async_copy(mem0_hbm, mem0_s, sem_in.at[0])
        cp_gw = pltpu.make_async_copy(gw_hbm, gw_s, sem_in.at[1])

        first = a_copies(0, sem_f)
        named = {"gw": cp_gw, "wk": first[0], "wq": first[1], "wv": first[2], "wo": cp_woa0, "mem": cp_mem}
        named.update({"c%d" % c: cp_c[c] for c in range(1, NCH)})
        named.update({"x%d" % c: cp_x[c] for c in range(NCH)})
        named["c0a"] = pltpu.make_async_copy(c_hbm.bitcast(u32).at[0:HALF // 2, :], c_s.at[0:HALF // 2, :], sem_xc.at[NCH])
        named["c0b"] = pltpu.make_async_copy(c_hbm.bitcast(u32).at[HALF // 2:PCH // 2, :], c_s.at[HALF // 2:PCH // 2, :],
                                             sem_xc.at[2 * NCH])
        for nm in DORD:
            named[nm].start()
        for cp in a_copies(1) + b_copies(0) + [cp_woa1]:
            cp.start()
        acc[...] = jnp.zeros(acc.shape, f32)

        row = jax.lax.broadcasted_iota(jnp.int32, (BQ, BQ), 0)
        col = jax.lax.broadcasted_iota(jnp.int32, (BQ, BQ), 1)
        tri = col <= row

        def tie(words, tok, r=0):
            if tok is None:
                return words
            n, c = words.shape
            blk = words[r:r + 8]
            if c > 128:
                blk = jnp.concatenate([jnp.bitwise_or(blk[:, :128], tok), blk[:, 128:]], axis=1)
            else:
                blk = jnp.bitwise_or(blk, tok)
            parts = ([words[:r]] if r else []) + [blk] + ([words[r + 8:]] if r + 8 < n else [])
            return jnp.concatenate(parts, axis=0)

        def ldp(ref, r0, r1, tok=None):
            return _as_bf16(tie(ref.bitcast(u32)[r0 // 2:r1 // 2, :], tok))

        def a_tasks(h, fused, on_scores, on_emit=None, spar=None, first_head=False):
            st = {}
            toks = {}
            marks, clock, due = [], [0], []

            def take(time):
                tk = None
                for tm, v in [d for d in due if d[0] <= time]:
                    t = _token_all(v)
                    tk = t if tk is None else jnp.bitwise_or(tk, t)
                due[:] = [d for d in due if d[0] > time]
                return tk

            def anchor(time):
                best = None
                for tm, v in marks:
                    if tm <= time:
                        best = v
                return best

            def proj(src, t, dst, sc, c, hh, tk):
                if isinstance(c, str):
                    r, n = (0, HALF) if c[1] == "a" else (HALF, PCH - HALF)
                else:
                    r, n = c * PCH, PCH
                hh, nxt = hh
                words = st_a[(hh // 2) % NP2, t]
                par = hh % 2 if spar is None else (spar + nxt) % 2
                if tk is None:
                    w = _unpack_head(words, par)
                else:
                    w = _unpack_head_tok(words, par, toks[tk])
                lhs = src[r // 2:(r + n) // 2, :]
                for rr in range(0, n, BQ):
                    lhs = tie(lhs, take(clock[0] + rr), rr // 2)
                y = jnp.dot(_as_bf16(lhs), w, preferred_element_type=f32)
                for rr in range(64, n, 64):
                    marks.append((clock[0] + rr, y[rr:rr + 8]))
                clock[0] += n
                if sc is not None:
                    y = y * sc
                dst[r:r + n, :] = y.astype(bf16)

            def move(dst, t):
                dst[0:PCH, :] = tmp_s[t]

            def scores(i):
                r0 = i * BQ
                qw = q_s.bitcast(u32)[r0 // 2:(r0 + BQ) // 2, :]
                ss = []
                mm = None
                for j in range(i + 1):
                    tk = take(clock[0] + (j // 4) * BQ) if j % 4 == 0 else None
                    s = jax.lax.dot_general(_as_bf16(tie(qw, tk)), ldp(k_s, j * BQ, (j + 1) * BQ), NT,
                                            preferred_element_type=f32)
                    marks.append((clock[0] + min(BQ * (j // 4 + 1), (i + 1) * BQ // 4), s))
                    if j == i:
                        s = jnp.where(tri, s, NEG)
                    mm = s if mm is None else jnp.maximum(mm, s)
                    if (j % 4 == 3 or j == i) and i >= MMIN and fused:
                        due.append((clock[0] + min(BQ * (j // 4 + 1), (i + 1) * BQ // 4) + MD2, mm))
                    ss.append(s)
                clock[0] += (i + 1) * BQ // 4
                toks[i] = _token(mm)
                m = jnp.max(mm, axis=1, keepdims=True)
                st[i] = (ss, m)
                on_scores(i, toks[i])

            def pv(i):
                ss, m = st[i]
                m = jnp.broadcast_to(m, (BQ, BQ))
                o = None
                l = None
                ts = []
                for j, s in enumerate(ss):
                    if j % JG == 0:
                        av = ts[j - JLA] if j >= JLA else anchor(clock[0] + (j // 4) * BQ - (LA2 if fused else LA1))
                        if av is not None:
                            tok = pltpu.bitcast(_token(av), f32)
                            m = (m.reshape(BQ // 8, 8, BQ) + tok[None]).reshape(BQ, BQ)
                    p = jnp.exp2(s - m)
                    l = p if l is None else l + p
                    tk = take(clock[0] + (j // 4) * BQ) if j % 4 == 0 else None
                    pb = p.astype(bf16)
                    if tk is not None:
                        pb = _as_bf16(tie(pltpu.bitcast(pb, u32), tk))
                    t = jnp.dot(pb, ldp(v_s, j * BQ, (j + 1) * BQ), preferred_element_type=f32)
                    ts.append(t)
                    o = t if o is None else o + t
                for j, t in enumerate(ts):
                    marks.append((clock[0] + min(BQ * (j // 4 + 1), (i + 1) * BQ // 4), t))
                clock[0] += (i + 1) * BQ // 4
                o = o * _recip(jnp.sum(l, axis=1, keepdims=True))
                if fused:
                    o = o * g_s[i * BQ:(i + 1) * BQ, :]
                st[i] = o.astype(bf16)

            def outproj(i):
                r0 = i * BQ
                w = _as_bf16(wo_a[pl.ds(_mo(h * (D // 2), D // 2), D // 2), :])
                dst = acc if fused else acc1
                lhs = st[i]
                tk = take(clock[0])
                if tk is not None:
                    lhs = _as_bf16(tie(pltpu.bitcast(lhs, u32), tk))
                d = jnp.dot(lhs, w, preferred_element_type=f32)
                marks.append((clock[0] + BQ // 2, d[BQ // 2:BQ // 2 + 8]))
                marks.append((clock[0] + BQ, d[BQ - 8:BQ]))
                clock[0] += BQ
                a = d if first_head else dst[r0:r0 + BQ, :] + d
                dst[r0:r0 + BQ, :] = a
                if fused:
                    out_s[i * BQ:(i + 1) * BQ, :] = a.astype(bf16)
                    on_emit(i)

            out = []
            for kind, i, tk in (a_sched2 if fused else a_sched0 if first_head else a_sched1):
                hh = (h, 0) if kind[0] == "P" else (h + 1, 1)
                if kind in ("w", "G"):
                    fn = None
                elif kind[0] == "T":
                    t = "kqv".index(kind[1])
                    fn = functools.partial(proj, x_s if t == 1 else c_s, t, tmp_s.at[t], qscale if t == 1 else None,
                                           i, hh, tk)
                elif kind[0] == "C":
                    t = "kqv".index(kind[1])
                    fn = functools.partial(move, (k_s, q_s, v_s)[t], t)
                elif kind in ("Pk", "Nk"):
                    fn = functools.partial(proj, c_s, 0, k_s, None, i, hh, tk)
                elif kind in ("Pq", "Nq"):
                    fn = functools.partial(proj, x_s, 1, q_s, qscale, i, hh, tk)
                elif kind in ("Pv", "Nv"):
                    fn = functools.partial(proj, c_s, 2, v_s, None, i, hh, tk)
                elif kind == "S":
                    fn = functools.partial(scores, i)
                elif kind == "O":
                    fn = functools.partial(pv, i)
                else:
                    fn = functools.partial(outproj, i)
                out.append(((kind, i), fn))
            return out

        def unpack_b(p, t, c, tok):
            rows = pl.ds(c * (M // 4), M // 4)
            lo, hi = _unpack_pair_tok(st_b[p % 2, t, rows, :], tok)
            w_b[t * H + 2 * p, rows, :] = lo
            w_b[t * H + 2 * p + 1, rows, :] = hi

        gwv = {}

        def gate(h):
            if "gw" not in gwv:
                gwv["gw"] = gw_s[...].astype(f32).reshape(1, M)
            xg = _as_bf16(x_s[pl.ds(_mo(h * (BQ // 2), 8), BQ // 2), :]).astype(f32)
            g = jax.nn.sigmoid(jnp.sum(xg * gwv["gw"], axis=1, keepdims=True))
            gb = jnp.broadcast_to(g, (BQ, D))
            g_s[pl.ds(_mo(h * BQ, 8), BQ), :] = gb

        def a_head(h, first_head):
            if not isinstance(h, int):
                for cp in a_copies(h) + b_copies(h - 1):
                    cp.wait()

            nxt = [] if isinstance(h, int) else a_copies((h + 1) % NP2) + b_copies(h)

            def on_scores(i, tok):
                if 1 <= i <= 12 and not first_head:
                    unpack_b(h - 1, (i - 1) // 4, (i - 1) % 4, tok)

            if not first_head:
                gate(h)

            for n, (name, fn) in enumerate(a_tasks(h, False, on_scores, spar=h % 2 if isinstance(h, int) else None,
                                                   first_head=first_head)):
                if name[0] == "w":
                    for cp in name[1]:
                        named[cp].wait()
                elif name[0] == "G":
                    gate(h)
                else:
                    fn()
                if n == STARTPOS:
                    for cp in nxt:
                        cp.start()

        def a_body(h, carry):
            a_head(h, False)
            return carry

        a_head(0, True)
        cp_woa1.wait()
        cp_woa.start()
        jax.lax.fori_loop(1, SPLIT1, a_body, 0)
        cp_woa.wait()
        cp_wob.start()
        jax.lax.fori_loop(SPLIT1, H1, a_body, 0)

        cp_mem.wait()
        cp_wob.wait()

        def wb(t, h):
            return _as_bf16(w_b.bitcast(u32)[t * H + h])

        def wob(g):
            return _as_bf16(wo_b[g * GB * D // 2:(g + 1) * GB * D // 2, :])

        def tile4(g):
            return jnp.concatenate([g] * (M // D), axis=1)

        mem_s[...] = mem0_s[...].astype(f32)

        for cp in a_copies(0) + b_copies(H1 - 1):
            cp.wait()
        ztok = jnp.zeros((8, D), u32)
        for n in range(12):
            unpack_b(NP2 - 1, n // 4, n % 4, ztok)

        L = NM + SEG
        r80 = jax.lax.broadcasted_iota(jnp.int32, (2 * L, 2 * L), 0)
        c80 = jax.lax.broadcasted_iota(jnp.int32, (2 * L, 2 * L), 1)
        rhead = jnp.where(r80 < NM, 0, jnp.where(r80 < 2 * NM, 1, jnp.where(r80 < 2 * NM + SEG, 0, 1)))
        chead = jnp.where(c80 < L, 0, 1)
        rpos = jnp.where(r80 < 2 * NM, L - 1,
                         jnp.where(r80 < 2 * NM + SEG, r80 - 2 * NM + NM, r80 - 2 * NM - SEG + NM))
        cpos = jnp.where(c80 < L, c80, c80 - L)
        same = rhead == chead
        valid = jnp.logical_and(same, cpos <= rpos)
        fill = jnp.where(same, NEG, -3e38).astype(f32)

        def finalize(a0, n, z):
            acc[pl.ds(a0, n), :] += z + tile4(g_s[pl.ds(a0, n), :]) * (acc1[pl.ds(a0, n), :] - z)

        def b_step(step, get_xr, cur, stores, ox_parts, finish):
            v = {"z": None}
            memp, ps, om = {}, {}, {}

            def proj(h):
                if "lhs" not in v:
                    v["lhs"] = jnp.concatenate([mem_s[...], get_xr()], axis=0).astype(bf16)
                r = []
                for t in range(3):
                    y = jnp.dot(v["lhs"], wb(t, h), preferred_element_type=f32)
                    if t == 0:
                        y = y * qscale
                    c0 = (t * H + h) * D
                    for (y0, n, slot, d0) in stores:
                        qkv_s[slot, d0:d0 + n, c0:c0 + D] = y[y0:y0 + n]
                    r.append(y[:NM])
                memp[h] = r

            def scores(gg):
                for h0 in range(gg * GB, (gg + 1) * GB, 2):
                    h1 = h0 + 1

                    def xs(t, h):
                        return qkv_s[cur, :, (t * H + h) * D:(t * H + h + 1) * D]
                    q2 = jnp.concatenate([memp[h0][0], memp[h1][0], xs(0, h0), xs(0, h1)], axis=0).astype(bf16)
                    k2 = jnp.concatenate([memp[h0][1], xs(1, h0), memp[h1][1], xs(1, h1)], axis=0).astype(bf16)
                    v2 = jnp.concatenate([memp[h0][2], xs(2, h0), memp[h1][2], xs(2, h1)], axis=0).astype(bf16)
                    sc = jax.lax.dot_general(q2, k2, NT, preferred_element_type=f32)
                    sc = jnp.where(valid, sc, fill)
                    m = jnp.max(sc, axis=1, keepdims=True)
                    p = jnp.exp2(sc - m)
                    l = jnp.sum(p, axis=1, keepdims=True)
                    ps[h0] = (p.astype(bf16), _recip(l), v2)

            def pv(gg):
                for h0 in range(gg * GB, (gg + 1) * GB, 2):
                    h1 = h0 + 1
                    p, rl, v2 = ps.pop(h0)
                    o = jnp.dot(p, v2, preferred_element_type=f32) * rl
                    om[h0] = o[0:NM]
                    om[h1] = o[NM:2 * NM]
                    ox_s[cur, :, h0 * D:(h0 + 1) * D] = o[2 * NM:2 * NM + SEG]
                    ox_s[cur, :, h1 * D:(h1 + 1) * D] = o[2 * NM + SEG:]

            def oproj(gg):
                c0, c1 = gg * GB * D, (gg + 1) * GB * D
                parts = [jnp.concatenate([om[h] for h in range(gg * GB, (gg + 1) * GB)], axis=1)]
                parts += [ox_s[slot, r0:r1, c0:c1] for (slot, r0, r1) in ox_parts]
                lo = jnp.concatenate(parts, axis=0).astype(bf16)
                t = jnp.dot(lo, wob(gg), preferred_element_type=f32)
                v["z"] = t if v["z"] is None else v["z"] + t
                if gg == NG - 1:
                    mem_s[...] = v["z"][:NM].astype(bf16).astype(f32)
                    finish(v["z"][NM:])

            tasks = []
            for g in range(NG + 3):
                if g < NG:
                    for h in range(g * GB, (g + 1) * GB):
                        tasks.append(((step, "P", h), functools.partial(proj, h)))
                if 0 <= g - 1 < NG:
                    tasks.append(((step, "Sc", g - 1), functools.partial(scores, g - 1)))
                if 0 <= g - 2 < NG:
                    tasks.append(((step, "Pv", g - 2), functools.partial(pv, g - 2)))
                if 0 <= g - 3 < NG:
                    tasks.append(((step, "Op", g - 3), functools.partial(oproj, g - 3)))
                tasks.append(((step, "end", g), None))
            return tasks

        def b_pair(j, par):
            s0 = par * 2
            s1 = s0 + 1
            a0 = pl.multiple_of(j * 64, 64)
            v = {}

            def xn():
                if "xn" not in v:
                    v["xn"] = _as_bf16(x_s[pl.ds(pl.multiple_of(j * SEG, 8), SEG), :]).astype(f32)
                return v["xn"]

            ev = b_step(2 * par, lambda: xn()[0:40], s0, [(NM, SEG, s0, 0), (NM + SEG, NM, s1, 0)],
                        [(s0, 0, SEG - NM)],
                        lambda z: finalize(a0, 24, z))
            od = b_step(2 * par + 1, lambda: xn()[40:64], s1, [(NM, SEG - NM, s1, NM)],
                        [(s0, SEG - NM, SEG), (s1, 0, SEG)],
                        lambda z: finalize(pl.multiple_of(a0 + 24, 8), 40, z))
            return ev + od

        NI = H - H1
        bounds = [0] + [t + 1 for t in OSPLIT]
        assert bounds[-1] == NQ
        out_cp = [pltpu.make_async_copy(out_s.at[bounds[n] * BQ:bounds[n + 1] * BQ, :],
                                        out_hbm.at[bounds[n] * BQ:bounds[n + 1] * BQ, :], sem_out.at[n])
                  for n in range(len(bounds) - 1)]

        def f_body(i, carry):
            def on_emit(t):
                if t in OSPLIT:
                    @pl.when(i == NI - 1)
                    def _():
                        out_cp[OSPLIT.index(t)].start()

            at = a_tasks(H1 + i, True, lambda t, tok: None, on_emit)
            bt = b_pair(2 * i, 0) + b_pair(2 * i + 1, 1)
            for fn in _merge(at, bt):
                fn()
            return carry

        jax.lax.fori_loop(0, NI, f_body, 0)

        for cp in out_cp:
            cp.wait()

    scratch = [
        pltpu.VMEM((S // 2, M), u32),
        pltpu.VMEM((S // 2, M), u32),
        pltpu.VMEM((S, M), f32),
        pltpu.VMEM((S, M), f32),
        pltpu.VMEM((S, D), f32),
        pltpu.VMEM((S, D), bf16),
        pltpu.VMEM((S, D), bf16),
        pltpu.VMEM((S, D), bf16),
        pltpu.VMEM((NP2, 3, M, D), u32),
        pltpu.VMEM((HD // 2, M), u32),
        pltpu.VMEM((2, 3, M, D), u32),
        pltpu.VMEM((3 * H, M, D), bf16),
        pltpu.VMEM((HD // 2, M), u32),
        pltpu.VMEM((NM, M), bf16),
        pltpu.VMEM((M,), bf16),
        pltpu.VMEM((NM, M), f32),
        pltpu.VMEM((4, SEG, 3 * HD), f32),
        pltpu.VMEM((4, SEG, HD), f32),
        pltpu.VMEM((S, M), bf16),
        pltpu.VMEM((3, PCH, D), bf16),
        pltpu.SemaphoreType.DMA((4,)),
        pltpu.SemaphoreType.DMA((4,)),
        pltpu.SemaphoreType.DMA((4,)),
        pltpu.SemaphoreType.DMA((len(OSPLIT),)),
        pltpu.SemaphoreType.DMA((2 * NCH + 1,)),
        pltpu.SemaphoreType.DMA((3,)),
    ]
    return kernel, scratch


@functools.partial(jax.jit, static_argnames=("B_seg_len",))
def pallas_gated_mix__compressed_kv_cla__memory_aug_recurrent_mem_tr__prompt_kernel(
    A_x: jax.Array,
    A_c_kv: jax.Array,
    A_w_q: jax.Array,
    A_w_uk: jax.Array,
    A_w_uv: jax.Array,
    A_w_o: jax.Array,
    B_x: jax.Array,
    B_mem0: jax.Array,
    B_Wq: jax.Array,
    B_Wk: jax.Array,
    B_Wv: jax.Array,
    B_Wo: jax.Array,
    B_seg_len: int,
    gate_w: jax.Array,
):
    _, S, M = A_x.shape
    _, H, D = A_w_q.shape
    NM = B_mem0.shape[1]
    kernel, scratch = _make_kernel(S, M, H, D, NM, int(B_seg_len))
    any_spec = pl.BlockSpec(memory_space=pl.ANY)
    out = pl.pallas_call(
        kernel,
        out_shape=jax.ShapeDtypeStruct((S, M), bf16),
        in_specs=[any_spec] * 12,
        out_specs=any_spec,
        scratch_shapes=scratch,
        compiler_params=pltpu.CompilerParams(vmem_limit_bytes=100 * 1024 * 1024, disable_bounds_checks=True,
                                             disable_semaphore_checks=True),
    )(
        A_x.reshape(S, M), A_c_kv.reshape(S, M), A_w_q, A_w_uk, A_w_uv,
        A_w_o.reshape(H * D, M), B_mem0.reshape(NM, M),
        B_Wq, B_Wk, B_Wv, B_Wo.reshape(H * D, M), gate_w,
    )
    return out.reshape(1, S, M)
```

```python
import functools

import jax
import jax.numpy as jnp
import jax.experimental.pallas as pl
import jax.experimental.pallas.tpu as pltpu

bf16 = jnp.bfloat16
f32 = jnp.float32
u32 = jnp.uint32

LOG2E = 1.4426950408889634
NEG = -1e9 * LOG2E
NT = (((1,), (1,)), ((), ()))

BQ = 128
PCH = 512
GB = 4

JG = 4
JLA = 8
LA1 = 100000
LA2 = 256
MD2 = 448
MMIN = 4
HALF = 256
SPLIT1 = 3
STARTPOS = 3
DORD = "gw wk c0a c0b wv wq x0 c1 x1 wo c2 x2 c3 x3 mem".split()
H0 = ("w:wk+c0a Pk0a Tk0a w:c0b+wv Pk0b Tk0b Pv0 Tv0 w:wq+x0+gw Pq0 G0 Tq0 S0 S1 O0 S2 O1 S3 O2 O3 "
      "w:c1 Pk1 Pv1 w:x1+wo Pq1 F0 F1 S4 F2 S5 O4 F3 S6 O5 F4 w:c2+x2 Pk2 S7 O6 F5 Pq2 O7 F6 Pv2 F7 S8 "
      "w:c3+x3 Pk3").split()
_MIDDLE = ("S3 O2 F1 S4 Pk2:2 O3 F2 S5 Pq2:3 O4 F3 S6 Pv2:4 O5 F4 S7 O6 F5 S8 Pk3:6 O7 F6 S9 Pq3:7 O8 F7 "
           "S10 Pv3:8 O9 F8 S11 O10 F9 S12 O11 F10 S13 O12 F11 S14 O13 F12 Nq0:14 S15 O14 F13 ")
A_ONLY = "Pk1 S0 Pq1 S1 O0 S2 Pv1 O1 F0 " + _MIDDLE + "Nk0:13 O15 F14 Nv0:15 F15"
A_FUSED = "S0 Pk1 S1 O0 Pq1 S2 O1 F0 Pv1 " + _MIDDLE + "O15 F14 F15 Nk0:13 Nv0:15"
MIDS = ((2, 5), (1, 3, 5), (2, 4, 6), (0, 2, 4, 6))
TSPLIT = (2, 5)
OSPLIT = (9, 13, 14, 15)


def _mo(x, m):
    return x if isinstance(x, int) else pl.multiple_of(x, m)


def _mod(x, n):
    assert n & (n - 1) == 0
    return x % n if isinstance(x, int) else jnp.bitwise_and(x, n - 1)


def _half(x):
    return x // 2 if isinstance(x, int) else jax.lax.shift_right_logical(x, 1)


def _as_bf16(words):
    return pltpu.bitcast(words, bf16)


def _recip(l):
    r = pl.reciprocal(l, approx=True)
    return r * (2.0 - l * r)


def _unpack_head(words, par):
    if isinstance(par, int):
        w = jnp.bitwise_and(words, jnp.uint32(0xFFFF0000)) if par else jnp.left_shift(words, jnp.uint32(16))
        return pltpu.bitcast(w, f32).astype(bf16)
    sh = ((1 - par) * 16).astype(u32)
    w = jnp.bitwise_and(jnp.left_shift(words, sh), jnp.uint32(0xFFFF0000))
    return pltpu.bitcast(w, f32).astype(bf16)


def _token(v):
    f = pltpu.bitcast(jnp.right_shift(pltpu.bitcast(v[0:8, 0:128], u32), jnp.uint32(2)), f32)
    return pltpu.bitcast(f - f, u32)


def _token_all(v):
    v3 = v.reshape(v.shape[0] // 8, 8, v.shape[1])
    n = v3.shape[0]
    parts = [v3[i] for i in range(n)]
    while len(parts) > 1:
        parts = [jnp.maximum(parts[i], parts[i + 1]) for i in range(0, len(parts), 2)]
    return _token(parts[0])


def _unpack_head_tok(words, par, tok):
    r, c = words.shape
    if isinstance(par, int):
        w3 = words.reshape(r // 8, 8, c)
        if par:
            w = jnp.bitwise_and(w3, jnp.bitwise_or(tok, jnp.uint32(0xFFFF0000))[None])
        else:
            w = jnp.left_shift(w3, (tok + jnp.uint32(16))[None])
        return pltpu.bitcast(w.reshape(r, c), f32).astype(bf16)
    sh = ((1 - par) * 16).astype(u32) + tok
    mask = jnp.bitwise_or(tok, jnp.uint32(0xFFFF0000))
    w = jnp.bitwise_and(jnp.left_shift(words.reshape(r // 8, 8, c), sh[None]), mask[None])
    return pltpu.bitcast(w.reshape(r, c), f32).astype(bf16)


def _unpack_pair_tok(words, tok):
    r, c = words.shape
    w3 = words.reshape(r // 8, 8, c)
    lo = jnp.left_shift(w3, (tok + jnp.uint32(16))[None])
    hi = jnp.bitwise_and(w3, jnp.bitwise_or(tok, jnp.uint32(0xFFFF0000))[None])
    return (pltpu.bitcast(lo.reshape(r, c), f32).astype(bf16),
            pltpu.bitcast(hi.reshape(r, c), f32).astype(bf16))


def _first_schedule(base):
    tk = {(k, i): t for k, i, t in base}
    head = []
    for s in H0:
        if s.startswith("w:"):
            head.append(("w", tuple(s[2:].split("+")), None))
        else:
            nm = (s[:-1], int(s[-1])) if s[0] in "SOFG" else (s[:2], int(s[2]) if len(s) == 3 else s[2:])
            head.append(nm + (tk.get(nm),))
    used = {(k, i) for k, i, _ in head}
    rest = [(k, i, t) for k, i, t in base if (k, i) not in used]
    rest = [("C" + k[1], i, t) if k[0] == "N" else (k, i, t) for k, i, t in rest]
    return head + rest


def _a_schedule(nq, bpc, fused):
    assert nq == 16 and bpc == 4
    out = []
    for s in (A_FUSED if fused else A_ONLY).split():
        name, _, tok = s.partition(":")
        n = 1 if name[0] in "SOF" else 2
        out.append((name[:n], int(name[n:]), int(tok) if tok else None))
    return out


def _units(a_tasks):
    units = []
    for name, fn in a_tasks:
        if name[0] == "S":
            units.append([])
        units[-1].append((name, fn))
    return units


def _merge(a_tasks, b_tasks):
    units = _units(a_tasks)
    plan = {}
    u = 0
    for step in range(4):
        for g in MIDS[step]:
            plan.setdefault((step, "end", g), []).extend(units[u])
            u += 1
        t = units[u]
        u += 1
        a, b = (1, 2) if step < 3 else TSPLIT
        plan[(step, "Sc", 7)] = t[0:a]
        plan[(step, "Pv", 7)] = t[a:b]
        plan[(step, "Op", 7)] = t[b:]
    assert u == len(units)
    out = []
    for name, fn in b_tasks:
        if fn is not None:
            out.append(fn)
        out += [f for _, f in plan.pop(name, [])]
    assert not plan, plan
    return out


def _make_kernel(S, M, H, D, NM, SEG):
    assert SEG == 32 and NM == 8 and D == 128 and S % PCH == 0 and H % 2 == 0 and H % GB == 0
    NQ = S // BQ
    NPAIR = S // (2 * SEG)
    NG = H // GB
    HD = H * D
    NCH = S // PCH
    H1 = H // 2
    NP2 = H // 2
    assert NPAIR == 2 * (H - H1) and NQ == H1 and NP2 == H1
    qscale = D ** -0.5 * LOG2E
    a_sched1 = _a_schedule(NQ, PCH // BQ, False)
    a_sched2 = _a_schedule(NQ, PCH // BQ, True)
    a_sched0 = _first_schedule(a_sched1)

    def kernel(x_hbm, c_hbm, wq_hbm, wk_hbm, wv_hbm, wo_hbm, mem0_hbm,
               bq_hbm, bk_hbm, bv_hbm, bo_hbm, gw_hbm, out_hbm,
               x_s, c_s, acc1, acc, g_s, q_s, k_s, v_s, st_a, wo_a, st_b, w_b, wo_b,
               mem0_s, gw_s, mem_s, qkv_s, ox_s, out_s, tmp_s,
               sem_in, sem_a, sem_b, sem_out, sem_xc, sem_f):
        a_w_hbm = (wk_hbm, wq_hbm, wv_hbm)
        b_w_hbm = (bq_hbm, bk_hbm, bv_hbm)

        def a_copies(p, sem=sem_a):
            return [pltpu.make_async_copy(a_w_hbm[t].bitcast(u32).at[:, p, :], st_a.at[p, t],
                                          sem.at[t]) for t in range(3)]

        def b_copies(p):
            return [pltpu.make_async_copy(b_w_hbm[t].bitcast(u32).at[:, p, :], st_b.at[_mod(p, 2), t],
                                          sem_b.at[t]) for t in range(3)]

        cp_x = [pltpu.make_async_copy(x_hbm.bitcast(u32).at[c * (PCH // 2):(c + 1) * (PCH // 2), :],
                                      x_s.at[c * (PCH // 2):(c + 1) * (PCH // 2), :], sem_xc.at[c])
                for c in range(NCH)]
        cp_c = {c: pltpu.make_async_copy(c_hbm.bitcast(u32).at[c * (PCH // 2):(c + 1) * (PCH // 2), :],
                                         c_s.at[c * (PCH // 2):(c + 1) * (PCH // 2), :], sem_xc.at[NCH + c])
                for c in range(1, NCH)}
        cp_woa0 = pltpu.make_async_copy(wo_hbm.bitcast(u32).at[pl.ds(0, D), :], wo_a.at[pl.ds(0, D), :], sem_a.at[3])
        cp_woa1 = pltpu.make_async_copy(wo_hbm.bitcast(u32).at[D:2 * D, :], wo_a.at[D:2 * D, :], sem_in.at[3])
        cp_woa = pltpu.make_async_copy(wo_hbm.bitcast(u32).at[2 * D:HD // 2, :], wo_a.at[2 * D:HD // 2, :], sem_b.at[3])
        cp_wob = pltpu.make_async_copy(bo_hbm.bitcast(u32), wo_b, sem_in.at[2])
        cp_mem = pltpu.make_async_copy(mem0_hbm, mem0_s, sem_in.at[0])
        cp_gw = pltpu.make_async_copy(gw_hbm, gw_s, sem_in.at[1])

        first = a_copies(0, sem_f)
        named = {"gw": cp_gw, "wk": first[0], "wq": first[1], "wv": first[2], "wo": cp_woa0, "mem": cp_mem}
        named.update({"c%d" % c: cp_c[c] for c in range(1, NCH)})
        named.update({"x%d" % c: cp_x[c] for c in range(NCH)})
        named["c0a"] = pltpu.make_async_copy(c_hbm.bitcast(u32).at[0:HALF // 2, :], c_s.at[0:HALF // 2, :], sem_xc.at[NCH])
        named["c0b"] = pltpu.make_async_copy(c_hbm.bitcast(u32).at[HALF // 2:PCH // 2, :], c_s.at[HALF // 2:PCH // 2, :],
                                             sem_xc.at[2 * NCH])
        for nm in DORD:
            named[nm].start()
        for cp in a_copies(1) + b_copies(0) + [cp_woa1]:
            cp.start()
        acc[...] = jnp.zeros(acc.shape, f32)

        row = jax.lax.broadcasted_iota(jnp.int32, (BQ, BQ), 0)
        col = jax.lax.broadcasted_iota(jnp.int32, (BQ, BQ), 1)
        tri = col <= row

        def tie(words, tok, r=0):
            if tok is None:
                return words
            n, c = words.shape
            blk = words[r:r + 8]
            if c > 128:
                blk = jnp.concatenate([jnp.bitwise_or(blk[:, :128], tok), blk[:, 128:]], axis=1)
            else:
                blk = jnp.bitwise_or(blk, tok)
            parts = ([words[:r]] if r else []) + [blk] + ([words[r + 8:]] if r + 8 < n else [])
            return jnp.concatenate(parts, axis=0)

        def ldp(ref, r0, r1, tok=None):
            return _as_bf16(tie(ref.bitcast(u32)[r0 // 2:r1 // 2, :], tok))

        def a_tasks(h, fused, on_scores, on_emit=None, spar=None, first_head=False):
            st = {}
            toks = {}
            marks, clock, due = [], [0], []

            def take(time):
                tk = None
                for tm, v in [d for d in due if d[0] <= time]:
                    t = _token_all(v)
                    tk = t if tk is None else jnp.bitwise_or(tk, t)
                due[:] = [d for d in due if d[0] > time]
                return tk

            def anchor(time):
                best = None
                for tm, v in marks:
                    if tm <= time:
                        best = v
                return best

            def proj(src, t, dst, sc, c, hh, tk):
                if isinstance(c, str):
                    r, n = (0, HALF) if c[1] == "a" else (HALF, PCH - HALF)
                else:
                    r, n = c * PCH, PCH
                hh, nxt = hh
                words = st_a[_mod(_half(hh), NP2), t]
                par = _mod(hh, 2) if spar is None else (spar + nxt) % 2
                if tk is None:
                    w = _unpack_head(words, par)
                else:
                    w = _unpack_head_tok(words, par, toks[tk])
                lhs = src[r // 2:(r + n) // 2, :]
                for rr in range(0, n, BQ):
                    lhs = tie(lhs, take(clock[0] + rr), rr // 2)
                y = jnp.dot(_as_bf16(lhs), w, preferred_element_type=f32)
                for rr in range(64, n, 64):
                    marks.append((clock[0] + rr, y[rr:rr + 8]))
                clock[0] += n
                if sc is not None:
                    y = y * sc
                dst[r:r + n, :] = y.astype(bf16)

            def move(dst, t):
                dst[0:PCH, :] = tmp_s[t]

            def scores(i):
                r0 = i * BQ
                qw = q_s.bitcast(u32)[r0 // 2:(r0 + BQ) // 2, :]
                ss = []
                mm = None
                for j in range(i + 1):
                    tk = take(clock[0] + (j // 4) * BQ) if j % 4 == 0 else None
                    s = jax.lax.dot_general(_as_bf16(tie(qw, tk)), ldp(k_s, j * BQ, (j + 1) * BQ), NT,
                                            preferred_element_type=f32)
                    marks.append((clock[0] + min(BQ * (j // 4 + 1), (i + 1) * BQ // 4), s))
                    if j == i:
                        s = jnp.where(tri, s, NEG)
                    mm = s if mm is None else jnp.maximum(mm, s)
                    if (j % 4 == 3 or j == i) and i >= MMIN and fused:
                        due.append((clock[0] + min(BQ * (j // 4 + 1), (i + 1) * BQ // 4) + MD2, mm))
                    ss.append(s)
                clock[0] += (i + 1) * BQ // 4
                toks[i] = _token(mm)
                m = jnp.max(mm, axis=1, keepdims=True)
                st[i] = (ss, m)
                on_scores(i, toks[i])

            def pv(i):
                ss, m = st[i]
                m = jnp.broadcast_to(m, (BQ, BQ))
                o = None
                l = None
                ts = []
                for j, s in enumerate(ss):
                    if j % JG == 0:
                        av = ts[j - JLA] if j >= JLA else anchor(clock[0] + (j // 4) * BQ - (LA2 if fused else LA1))
                        if av is not None:
                            tok = pltpu.bitcast(_token(av), f32)
                            m = (m.reshape(BQ // 8, 8, BQ) + tok[None]).reshape(BQ, BQ)
                    p = jnp.exp2(s - m)
                    l = p if l is None else l + p
                    tk = take(clock[0] + (j // 4) * BQ) if j % 4 == 0 else None
                    pb = p.astype(bf16)
                    if tk is not None:
                        pb = _as_bf16(tie(pltpu.bitcast(pb, u32), tk))
                    t = jnp.dot(pb, ldp(v_s, j * BQ, (j + 1) * BQ), preferred_element_type=f32)
                    ts.append(t)
                    o = t if o is None else o + t
                for j, t in enumerate(ts):
                    marks.append((clock[0] + min(BQ * (j // 4 + 1), (i + 1) * BQ // 4), t))
                clock[0] += (i + 1) * BQ // 4
                o = o * _recip(jnp.sum(l, axis=1, keepdims=True))
                if fused:
                    o = o * g_s[i * BQ:(i + 1) * BQ, :]
                st[i] = o.astype(bf16)

            def outproj(i):
                r0 = i * BQ
                w = _as_bf16(wo_a[pl.ds(_mo(h * (D // 2), D // 2), D // 2), :])
                dst = acc if fused else acc1
                lhs = st[i]
                tk = take(clock[0])
                if tk is not None:
                    lhs = _as_bf16(tie(pltpu.bitcast(lhs, u32), tk))
                d = jnp.dot(lhs, w, preferred_element_type=f32)
                marks.append((clock[0] + BQ // 2, d[BQ // 2:BQ // 2 + 8]))
                marks.append((clock[0] + BQ, d[BQ - 8:BQ]))
                clock[0] += BQ
                a = d if first_head else dst[r0:r0 + BQ, :] + d
                dst[r0:r0 + BQ, :] = a
                if fused:
                    out_s[i * BQ:(i + 1) * BQ, :] = a.astype(bf16)
                    on_emit(i)

            out = []
            for kind, i, tk in (a_sched2 if fused else a_sched0 if first_head else a_sched1):
                hh = (h, 0) if kind[0] == "P" else (h + 1, 1)
                if kind in ("w", "G"):
                    fn = None
                elif kind[0] == "T":
                    t = "kqv".index(kind[1])
                    fn = functools.partial(proj, x_s if t == 1 else c_s, t, tmp_s.at[t], qscale if t == 1 else None,
                                           i, hh, tk)
                elif kind[0] == "C":
                    t = "kqv".index(kind[1])
                    fn = functools.partial(move, (k_s, q_s, v_s)[t], t)
                elif kind in ("Pk", "Nk"):
                    fn = functools.partial(proj, c_s, 0, k_s, None, i, hh, tk)
                elif kind in ("Pq", "Nq"):
                    fn = functools.partial(proj, x_s, 1, q_s, qscale, i, hh, tk)
                elif kind in ("Pv", "Nv"):
                    fn = functools.partial(proj, c_s, 2, v_s, None, i, hh, tk)
                elif kind == "S":
                    fn = functools.partial(scores, i)
                elif kind == "O":
                    fn = functools.partial(pv, i)
                else:
                    fn = functools.partial(outproj, i)
                out.append(((kind, i), fn))
            return out

        def unpack_b(p, t, c, tok):
            rows = pl.ds(c * (M // 4), M // 4)
            lo, hi = _unpack_pair_tok(st_b[_mod(p, 2), t, rows, :], tok)
            w_b[t * H + 2 * p, rows, :] = lo
            w_b[t * H + 2 * p + 1, rows, :] = hi

        gwv = {}

        def gate(h):
            if "gw" not in gwv:
                gwv["gw"] = gw_s[...].astype(f32).reshape(1, M)
            xg = _as_bf16(x_s[pl.ds(_mo(h * (BQ // 2), 8), BQ // 2), :]).astype(f32)
            g = jax.nn.sigmoid(jnp.sum(xg * gwv["gw"], axis=1, keepdims=True))
            gb = jnp.broadcast_to(g, (BQ, D))
            g_s[pl.ds(_mo(h * BQ, 8), BQ), :] = gb

        def a_head(h, first_head):
            if not isinstance(h, int):
                for cp in a_copies(h) + b_copies(h - 1):
                    cp.wait()

            nxt = [] if isinstance(h, int) else a_copies(_mod(h + 1, NP2)) + b_copies(h)

            def on_scores(i, tok):
                if 1 <= i <= 12 and not first_head:
                    unpack_b(h - 1, (i - 1) // 4, (i - 1) % 4, tok)

            if not first_head:
                gate(h)

            for n, (name, fn) in enumerate(a_tasks(h, False, on_scores, spar=h % 2 if isinstance(h, int) else None,
                                                   first_head=first_head)):
                if name[0] == "w":
                    for cp in name[1]:
                        named[cp].wait()
                elif name[0] == "G":
                    gate(h)
                else:
                    fn()
                if n == STARTPOS:
                    for cp in nxt:
                        cp.start()

        def a_body(h, carry):
            a_head(h, False)
            return carry

        a_head(0, True)
        cp_woa1.wait()
        cp_woa.start()
        jax.lax.fori_loop(1, SPLIT1, a_body, 0)
        cp_woa.wait()
        cp_wob.start()
        jax.lax.fori_loop(SPLIT1, H1, a_body, 0)

        cp_mem.wait()
        cp_wob.wait()

        def wb(t, h):
            return _as_bf16(w_b.bitcast(u32)[t * H + h])

        def wob(g):
            return _as_bf16(wo_b[g * GB * D // 2:(g + 1) * GB * D // 2, :])

        def tile4(g):
            return jnp.concatenate([g] * (M // D), axis=1)

        mem_s[...] = mem0_s[...].astype(f32)

        for cp in a_copies(0) + b_copies(H1 - 1):
            cp.wait()
        ztok = jnp.zeros((8, D), u32)
        for n in range(12):
            unpack_b(NP2 - 1, n // 4, n % 4, ztok)

        L = NM + SEG
        r80 = jax.lax.broadcasted_iota(jnp.int32, (2 * L, 2 * L), 0)
        c80 = jax.lax.broadcasted_iota(jnp.int32, (2 * L, 2 * L), 1)
        rhead = jnp.where(r80 < NM, 0, jnp.where(r80 < 2 * NM, 1, jnp.where(r80 < 2 * NM + SEG, 0, 1)))
        chead = jnp.where(c80 < L, 0, 1)
        rpos = jnp.where(r80 < 2 * NM, L - 1,
                         jnp.where(r80 < 2 * NM + SEG, r80 - 2 * NM + NM, r80 - 2 * NM - SEG + NM))
        cpos = jnp.where(c80 < L, c80, c80 - L)
        same = rhead == chead
        valid = jnp.logical_and(same, cpos <= rpos)
        fill = jnp.where(same, NEG, -3e38).astype(f32)

        def finalize(a0, n, z):
            acc[pl.ds(a0, n), :] += z + tile4(g_s[pl.ds(a0, n), :]) * (acc1[pl.ds(a0, n), :] - z)

        def b_step(step, get_xr, cur, stores, ox_parts, finish):
            v = {"z": None}
            memp, ps, om = {}, {}, {}

            def proj(h):
                if "lhs" not in v:
                    v["lhs"] = jnp.concatenate([mem_s[...], get_xr()], axis=0).astype(bf16)
                r = []
                for t in range(3):
                    y = jnp.dot(v["lhs"], wb(t, h), preferred_element_type=f32)
                    if t == 0:
                        y = y * qscale
                    c0 = (t * H + h) * D
                    for (y0, n, slot, d0) in stores:
                        qkv_s[slot, d0:d0 + n, c0:c0 + D] = y[y0:y0 + n]
                    r.append(y[:NM])
                memp[h] = r

            def scores(gg):
                for h0 in range(gg * GB, (gg + 1) * GB, 2):
                    h1 = h0 + 1

                    def xs(t, h):
                        return qkv_s[cur, :, (t * H + h) * D:(t * H + h + 1) * D]
                    q2 = jnp.concatenate([memp[h0][0], memp[h1][0], xs(0, h0), xs(0, h1)], axis=0).astype(bf16)
                    k2 = jnp.concatenate([memp[h0][1], xs(1, h0), memp[h1][1], xs(1, h1)], axis=0).astype(bf16)
                    v2 = jnp.concatenate([memp[h0][2], xs(2, h0), memp[h1][2], xs(2, h1)], axis=0).astype(bf16)
                    sc = jax.lax.dot_general(q2, k2, NT, preferred_element_type=f32)
                    sc = jnp.where(valid, sc, fill)
                    m = jnp.max(sc, axis=1, keepdims=True)
                    p = jnp.exp2(sc - m)
                    l = jnp.sum(p, axis=1, keepdims=True)
                    ps[h0] = (p.astype(bf16), _recip(l), v2)

            def pv(gg):
                for h0 in range(gg * GB, (gg + 1) * GB, 2):
                    h1 = h0 + 1
                    p, rl, v2 = ps.pop(h0)
                    o = jnp.dot(p, v2, preferred_element_type=f32) * rl
                    om[h0] = o[0:NM]
                    om[h1] = o[NM:2 * NM]
                    ox_s[cur, :, h0 * D:(h0 + 1) * D] = o[2 * NM:2 * NM + SEG]
                    ox_s[cur, :, h1 * D:(h1 + 1) * D] = o[2 * NM + SEG:]

            def oproj(gg):
                c0, c1 = gg * GB * D, (gg + 1) * GB * D
                parts = [jnp.concatenate([om[h] for h in range(gg * GB, (gg + 1) * GB)], axis=1)]
                parts += [ox_s[slot, r0:r1, c0:c1] for (slot, r0, r1) in ox_parts]
                lo = jnp.concatenate(parts, axis=0).astype(bf16)
                t = jnp.dot(lo, wob(gg), preferred_element_type=f32)
                v["z"] = t if v["z"] is None else v["z"] + t
                if gg == NG - 1:
                    mem_s[...] = v["z"][:NM].astype(bf16).astype(f32)
                    finish(v["z"][NM:])

            tasks = []
            for g in range(NG + 3):
                if g < NG:
                    for h in range(g * GB, (g + 1) * GB):
                        tasks.append(((step, "P", h), functools.partial(proj, h)))
                if 0 <= g - 1 < NG:
                    tasks.append(((step, "Sc", g - 1), functools.partial(scores, g - 1)))
                if 0 <= g - 2 < NG:
                    tasks.append(((step, "Pv", g - 2), functools.partial(pv, g - 2)))
                if 0 <= g - 3 < NG:
                    tasks.append(((step, "Op", g - 3), functools.partial(oproj, g - 3)))
                tasks.append(((step, "end", g), None))
            return tasks

        def b_pair(j, par):
            s0 = par * 2
            s1 = s0 + 1
            a0 = pl.multiple_of(j * 64, 64)
            v = {}

            def xn():
                if "xn" not in v:
                    v["xn"] = _as_bf16(x_s[pl.ds(pl.multiple_of(j * SEG, 8), SEG), :]).astype(f32)
                return v["xn"]

            ev = b_step(2 * par, lambda: xn()[0:40], s0, [(NM, SEG, s0, 0), (NM + SEG, NM, s1, 0)],
                        [(s0, 0, SEG - NM)],
                        lambda z: finalize(a0, 24, z))
            od = b_step(2 * par + 1, lambda: xn()[40:64], s1, [(NM, SEG - NM, s1, NM)],
                        [(s0, SEG - NM, SEG), (s1, 0, SEG)],
                        lambda z: finalize(pl.multiple_of(a0 + 24, 8), 40, z))
            return ev + od

        NI = H - H1
        bounds = [0] + [t + 1 for t in OSPLIT]
        assert bounds[-1] == NQ
        out_cp = [pltpu.make_async_copy(out_s.at[bounds[n] * BQ:bounds[n + 1] * BQ, :],
                                        out_hbm.at[bounds[n] * BQ:bounds[n + 1] * BQ, :], sem_out.at[n])
                  for n in range(len(bounds) - 1)]

        def f_body(i, carry):
            def on_emit(t):
                if t in OSPLIT:
                    @pl.when(i == NI - 1)
                    def _():
                        out_cp[OSPLIT.index(t)].start()

            at = a_tasks(H1 + i, True, lambda t, tok: None, on_emit)
            bt = b_pair(2 * i, 0) + b_pair(2 * i + 1, 1)
            for fn in _merge(at, bt):
                fn()
            return carry

        jax.lax.fori_loop(0, NI, f_body, 0)

        for cp in out_cp:
            cp.wait()

    scratch = [
        pltpu.VMEM((S // 2, M), u32),
        pltpu.VMEM((S // 2, M), u32),
        pltpu.VMEM((S, M), f32),
        pltpu.VMEM((S, M), f32),
        pltpu.VMEM((S, D), f32),
        pltpu.VMEM((S, D), bf16),
        pltpu.VMEM((S, D), bf16),
        pltpu.VMEM((S, D), bf16),
        pltpu.VMEM((NP2, 3, M, D), u32),
        pltpu.VMEM((HD // 2, M), u32),
        pltpu.VMEM((2, 3, M, D), u32),
        pltpu.VMEM((3 * H, M, D), bf16),
        pltpu.VMEM((HD // 2, M), u32),
        pltpu.VMEM((NM, M), bf16),
        pltpu.VMEM((M,), bf16),
        pltpu.VMEM((NM, M), f32),
        pltpu.VMEM((4, SEG, 3 * HD), f32),
        pltpu.VMEM((4, SEG, HD), f32),
        pltpu.VMEM((S, M), bf16),
        pltpu.VMEM((3, PCH, D), bf16),
        pltpu.SemaphoreType.DMA((4,)),
        pltpu.SemaphoreType.DMA((4,)),
        pltpu.SemaphoreType.DMA((4,)),
        pltpu.SemaphoreType.DMA((len(OSPLIT),)),
        pltpu.SemaphoreType.DMA((2 * NCH + 1,)),
        pltpu.SemaphoreType.DMA((3,)),
    ]
    return kernel, scratch


@functools.partial(jax.jit, static_argnames=("B_seg_len",))
def pallas_gated_mix__compressed_kv_cla__memory_aug_recurrent_mem_tr__prompt_kernel(
    A_x: jax.Array,
    A_c_kv: jax.Array,
    A_w_q: jax.Array,
    A_w_uk: jax.Array,
    A_w_uv: jax.Array,
    A_w_o: jax.Array,
    B_x: jax.Array,
    B_mem0: jax.Array,
    B_Wq: jax.Array,
    B_Wk: jax.Array,
    B_Wv: jax.Array,
    B_Wo: jax.Array,
    B_seg_len: int,
    gate_w: jax.Array,
):
    _, S, M = A_x.shape
    _, H, D = A_w_q.shape
    NM = B_mem0.shape[1]
    kernel, scratch = _make_kernel(S, M, H, D, NM, int(B_seg_len))
    any_spec = pl.BlockSpec(memory_space=pl.ANY)
    out = pl.pallas_call(
        kernel,
        out_shape=jax.ShapeDtypeStruct((S, M), bf16),
        in_specs=[any_spec] * 12,
        out_specs=any_spec,
        scratch_shapes=scratch,
        compiler_params=pltpu.CompilerParams(vmem_limit_bytes=100 * 1024 * 1024, disable_bounds_checks=True,
                                             disable_semaphore_checks=True),
    )(
        A_x.reshape(S, M), A_c_kv.reshape(S, M), A_w_q, A_w_uk, A_w_uv,
        A_w_o.reshape(H * D, M), B_mem0.reshape(NM, M),
        B_Wq, B_Wk, B_Wv, B_Wo.reshape(H * D, M), gate_w,
    )
    return out.reshape(1, S, M)
```

```python
import functools

import jax
import jax.numpy as jnp
import jax.experimental.pallas as pl
import jax.experimental.pallas.tpu as pltpu

bf16 = jnp.bfloat16
f32 = jnp.float32
u32 = jnp.uint32

LOG2E = 1.4426950408889634
NEG = -1e9 * LOG2E
NT = (((1,), (1,)), ((), ()))

BQ = 128
PCH = 512
GB = 4

JG = 4
JLA = 8
LA1 = 100000
LA2 = 256
MD2 = 448
JLA_ONLY = {14: 9, 15: 9}
LA2_LAST = {15: 576}
MMIN = 4
HALF = 256
SPLIT1 = 3
STARTPOS = 3
DORD = "gw wk c0a c0b wv wq x0 c1 x1 wo c2 x2 c3 x3 mem".split()
H0 = ("w:wk+c0a Pk0a Tk0a w:c0b+wv Pk0b Tk0b Pv0 Tv0 w:wq+x0+gw Pq0 G0 Tq0 S0 S1 O0 S2 O1 S3 O2 O3 "
      "w:c1 Pk1 Pv1 w:x1+wo Pq1 F0 F1 S4 F2 S5 O4 F3 S6 O5 F4 w:c2+x2 Pk2 S7 O6 F5 Pq2 O7 F6 Pv2 F7 S8 "
      "w:c3+x3 Pk3").split()
_MIDDLE = ("S3 O2 F1 S4 Pk2:2 O3 F2 S5 Pq2:3 O4 F3 S6 Pv2:4 O5 F4 S7 O6 F5 S8 Pk3:6 O7 F6 S9 Pq3:7 O8 F7 "
           "S10 Pv3:8 O9 F8 S11 O10 F9 S12 O11 F10 S13 O12 F11 S14 O13 F12 Nq0:14 S15 O14 F13 ")
A_ONLY = "Pk1 S0 S1 Pq1 O0 S2 Pv1 O1 F0 " + _MIDDLE + "Nk0:13 O15 F14 Nv0:15 F15"
A_FUSED = "S0 Pk1 S1 O0 Pq1 S2 O1 F0 Pv1 " + _MIDDLE + "O15 F14 F15 Nk0:13 Nv0:15"
MIDS = ((2, 5), (1, 3, 5), (2, 4, 6), (0, 2, 4, 6))
TSPLIT = (2, 5)
OSPLIT = (9, 13, 14, 15)


def _mo(x, m):
    return x if isinstance(x, int) else pl.multiple_of(x, m)


def _mod(x, n):
    assert n & (n - 1) == 0
    return x % n if isinstance(x, int) else jnp.bitwise_and(x, n - 1)


def _half(x):
    return x // 2 if isinstance(x, int) else jax.lax.shift_right_logical(x, 1)


def _as_bf16(words):
    return pltpu.bitcast(words, bf16)


def _recip(l):
    r = pl.reciprocal(l, approx=True)
    return r * (2.0 - l * r)


def _unpack_head(words, par):
    if isinstance(par, int):
        w = jnp.bitwise_and(words, jnp.uint32(0xFFFF0000)) if par else jnp.left_shift(words, jnp.uint32(16))
        return pltpu.bitcast(w, f32).astype(bf16)
    sh = ((1 - par) * 16).astype(u32)
    w = jnp.bitwise_and(jnp.left_shift(words, sh), jnp.uint32(0xFFFF0000))
    return pltpu.bitcast(w, f32).astype(bf16)


def _token(v):
    f = pltpu.bitcast(jnp.right_shift(pltpu.bitcast(v[0:8, 0:128], u32), jnp.uint32(2)), f32)
    return pltpu.bitcast(f - f, u32)


def _token_all(v):
    v3 = v.reshape(v.shape[0] // 8, 8, v.shape[1])
    n = v3.shape[0]
    parts = [v3[i] for i in range(n)]
    while len(parts) > 1:
        parts = [jnp.maximum(parts[i], parts[i + 1]) for i in range(0, len(parts), 2)]
    return _token(parts[0])


def _unpack_head_tok(words, par, tok):
    r, c = words.shape
    if isinstance(par, int):
        w3 = words.reshape(r // 8, 8, c)
        if par:
            w = jnp.bitwise_and(w3, jnp.bitwise_or(tok, jnp.uint32(0xFFFF0000))[None])
        else:
            w = jnp.left_shift(w3, (tok + jnp.uint32(16))[None])
        return pltpu.bitcast(w.reshape(r, c), f32).astype(bf16)
    sh = ((1 - par) * 16).astype(u32) + tok
    mask = jnp.bitwise_or(tok, jnp.uint32(0xFFFF0000))
    w = jnp.bitwise_and(jnp.left_shift(words.reshape(r // 8, 8, c), sh[None]), mask[None])
    return pltpu.bitcast(w.reshape(r, c), f32).astype(bf16)


def _unpack_pair_tok(words, tok):
    r, c = words.shape
    w3 = words.reshape(r // 8, 8, c)
    lo = jnp.left_shift(w3, (tok + jnp.uint32(16))[None])
    hi = jnp.bitwise_and(w3, jnp.bitwise_or(tok, jnp.uint32(0xFFFF0000))[None])
    return (pltpu.bitcast(lo.reshape(r, c), f32).astype(bf16),
            pltpu.bitcast(hi.reshape(r, c), f32).astype(bf16))


def _first_schedule(base):
    tk = {(k, i): t for k, i, t in base}
    head = []
    for s in H0:
        if s.startswith("w:"):
            head.append(("w", tuple(s[2:].split("+")), None))
        else:
            nm = (s[:-1], int(s[-1])) if s[0] in "SOFG" else (s[:2], int(s[2]) if len(s) == 3 else s[2:])
            head.append(nm + (tk.get(nm),))
    used = {(k, i) for k, i, _ in head}
    rest = [(k, i, t) for k, i, t in base if (k, i) not in used]
    rest = [("C" + k[1], i, t) if k[0] == "N" else (k, i, t) for k, i, t in rest]
    return head + rest


def _a_schedule(nq, bpc, fused):
    assert nq == 16 and bpc == 4
    out = []
    for s in (A_FUSED if fused else A_ONLY).split():
        name, _, tok = s.partition(":")
        n = 1 if name[0] in "SOF" else 2
        out.append((name[:n], int(name[n:]), int(tok) if tok else None))
    return out


def _units(a_tasks):
    units = []
    for name, fn in a_tasks:
        if name[0] == "S":
            units.append([])
        units[-1].append((name, fn))
    return units


def _merge(a_tasks, b_tasks):
    units = _units(a_tasks)
    plan = {}
    u = 0
    for step in range(4):
        for g in MIDS[step]:
            plan.setdefault((step, "end", g), []).extend(units[u])
            u += 1
        t = units[u]
        u += 1
        a, b = (1, 2) if step < 3 else TSPLIT
        plan[(step, "Sc", 7)] = t[0:a]
        plan[(step, "Pv", 7)] = t[a:b]
        plan[(step, "Op", 7)] = t[b:]
    assert u == len(units)
    out = []
    for name, fn in b_tasks:
        if fn is not None:
            out.append(fn)
        out += [f for _, f in plan.pop(name, [])]
    assert not plan, plan
    return out


def _make_kernel(S, M, H, D, NM, SEG):
    assert SEG == 32 and NM == 8 and D == 128 and S % PCH == 0 and H % 2 == 0 and H % GB == 0
    NQ = S // BQ
    NPAIR = S // (2 * SEG)
    NG = H // GB
    HD = H * D
    NCH = S // PCH
    H1 = H // 2
    NP2 = H // 2
    assert NPAIR == 2 * (H - H1) and NQ == H1 and NP2 == H1
    qscale = D ** -0.5 * LOG2E
    a_sched1 = _a_schedule(NQ, PCH // BQ, False)
    a_sched2 = _a_schedule(NQ, PCH // BQ, True)
    a_sched0 = _first_schedule(a_sched1)

    def kernel(x_hbm, c_hbm, wq_hbm, wk_hbm, wv_hbm, wo_hbm, mem0_hbm,
               bq_hbm, bk_hbm, bv_hbm, bo_hbm, gw_hbm, out_hbm,
               x_s, c_s, acc1, acc, g_s, q_s, k_s, v_s, st_a, wo_a, st_b, w_b, wo_b,
               mem0_s, gw_s, mem_s, qkv_s, ox_s, out_s, tmp_s, wu_s,
               sem_in, sem_a, sem_b, sem_out, sem_xc, sem_f):
        a_w_hbm = (wk_hbm, wq_hbm, wv_hbm)
        b_w_hbm = (bq_hbm, bk_hbm, bv_hbm)

        def a_copies(p, sem=sem_a):
            return [pltpu.make_async_copy(a_w_hbm[t].bitcast(u32).at[:, p, :], st_a.at[p, t],
                                          sem.at[t]) for t in range(3)]

        def b_copies(p):
            return [pltpu.make_async_copy(b_w_hbm[t].bitcast(u32).at[:, p, :], st_b.at[_mod(p, 2), t],
                                          sem_b.at[t]) for t in range(3)]

        cp_x = [pltpu.make_async_copy(x_hbm.bitcast(u32).at[c * (PCH // 2):(c + 1) * (PCH // 2), :],
                                      x_s.at[c * (PCH // 2):(c + 1) * (PCH // 2), :], sem_xc.at[c])
                for c in range(NCH)]
        cp_c = {c: pltpu.make_async_copy(c_hbm.bitcast(u32).at[c * (PCH // 2):(c + 1) * (PCH // 2), :],
                                         c_s.at[c * (PCH // 2):(c + 1) * (PCH // 2), :], sem_xc.at[NCH + c])
                for c in range(1, NCH)}
        cp_woa0 = pltpu.make_async_copy(wo_hbm.bitcast(u32).at[pl.ds(0, D), :], wo_a.at[pl.ds(0, D), :], sem_a.at[3])
        cp_woa1 = pltpu.make_async_copy(wo_hbm.bitcast(u32).at[D:2 * D, :], wo_a.at[D:2 * D, :], sem_in.at[3])
        cp_woa = pltpu.make_async_copy(wo_hbm.bitcast(u32).at[2 * D:HD // 2, :], wo_a.at[2 * D:HD // 2, :], sem_b.at[3])
        cp_wob = pltpu.make_async_copy(bo_hbm.bitcast(u32), wo_b, sem_in.at[2])
        cp_mem = pltpu.make_async_copy(mem0_hbm, mem0_s, sem_in.at[0])
        cp_gw = pltpu.make_async_copy(gw_hbm, gw_s, sem_in.at[1])

        first = a_copies(0, sem_f)
        named = {"gw": cp_gw, "wk": first[0], "wq": first[1], "wv": first[2], "wo": cp_woa0, "mem": cp_mem}
        named.update({"c%d" % c: cp_c[c] for c in range(1, NCH)})
        named.update({"x%d" % c: cp_x[c] for c in range(NCH)})
        named["c0a"] = pltpu.make_async_copy(c_hbm.bitcast(u32).at[0:HALF // 2, :], c_s.at[0:HALF // 2, :], sem_xc.at[NCH])
        named["c0b"] = pltpu.make_async_copy(c_hbm.bitcast(u32).at[HALF // 2:PCH // 2, :], c_s.at[HALF // 2:PCH // 2, :],
                                             sem_xc.at[2 * NCH])
        for nm in DORD:
            named[nm].start()
        for cp in a_copies(1) + b_copies(0) + [cp_woa1]:
            cp.start()
        acc[...] = jnp.zeros(acc.shape, f32)

        row = jax.lax.broadcasted_iota(jnp.int32, (BQ, BQ), 0)
        col = jax.lax.broadcasted_iota(jnp.int32, (BQ, BQ), 1)
        tri = col <= row

        def tie(words, tok, r=0):
            if tok is None:
                return words
            n, c = words.shape
            blk = words[r:r + 8]
            if c > 128:
                blk = jnp.concatenate([jnp.bitwise_or(blk[:, :128], tok), blk[:, 128:]], axis=1)
            else:
                blk = jnp.bitwise_or(blk, tok)
            parts = ([words[:r]] if r else []) + [blk] + ([words[r + 8:]] if r + 8 < n else [])
            return jnp.concatenate(parts, axis=0)

        def ldp(ref, r0, r1, tok=None):
            return _as_bf16(tie(ref.bitcast(u32)[r0 // 2:r1 // 2, :], tok))

        def a_tasks(h, fused, on_scores, on_emit=None, spar=None, first_head=False):
            st = {}
            toks = {}
            marks, clock, due = [], [0], []

            def take(time):
                tk = None
                for tm, v in [d for d in due if d[0] <= time]:
                    t = _token_all(v)
                    tk = t if tk is None else jnp.bitwise_or(tk, t)
                due[:] = [d for d in due if d[0] > time]
                return tk

            def anchor(time):
                best = None
                for tm, v in marks:
                    if tm <= time:
                        best = v
                return best

            def weight(t, hh, tk, keep):
                hh, nxt = hh
                if not fused and not first_head and not nxt:
                    return _as_bf16(wu_s[t])
                words = st_a[_mod(_half(hh), NP2), t]
                par = _mod(hh, 2) if spar is None else (spar + nxt) % 2
                if tk is None:
                    w = _unpack_head(words, par)
                else:
                    w = _unpack_head_tok(words, par, toks[tk])
                if nxt and keep and not fused:
                    wu_s[t] = pltpu.bitcast(w, u32)
                return w

            def proj(src, t, dst, sc, c, hh, tk):
                if isinstance(c, str):
                    r, n = (0, HALF) if c[1] == "a" else (HALF, PCH - HALF)
                else:
                    r, n = c * PCH, PCH
                w = weight(t, hh, tk, c != "0b")
                lhs = src[r // 2:(r + n) // 2, :]
                for rr in range(0, n, BQ):
                    lhs = tie(lhs, take(clock[0] + rr), rr // 2)
                y = jnp.dot(_as_bf16(lhs), w, preferred_element_type=f32)
                for rr in range(64, n, 64):
                    marks.append((clock[0] + rr, y[rr:rr + 8]))
                clock[0] += n
                if sc is not None:
                    y = y * sc
                dst[r:r + n, :] = y.astype(bf16)

            def move(dst, t):
                dst[0:PCH, :] = tmp_s[t]

            def scores(i):
                r0 = i * BQ
                qw = q_s.bitcast(u32)[r0 // 2:(r0 + BQ) // 2, :]
                ss = []
                mm = None
                for j in range(i + 1):
                    tk = take(clock[0] + (j // 4) * BQ) if j % 4 == 0 else None
                    s = jax.lax.dot_general(_as_bf16(tie(qw, tk)), ldp(k_s, j * BQ, (j + 1) * BQ), NT,
                                            preferred_element_type=f32)
                    marks.append((clock[0] + min(BQ * (j // 4 + 1), (i + 1) * BQ // 4), s))
                    if j == i:
                        s = jnp.where(tri, s, NEG)
                    mm = s if mm is None else jnp.maximum(mm, s)
                    if (j % 4 == 3 or j == i) and i >= MMIN and fused:
                        due.append((clock[0] + min(BQ * (j // 4 + 1), (i + 1) * BQ // 4) + MD2, mm))
                    ss.append(s)
                clock[0] += (i + 1) * BQ // 4
                toks[i] = _token(mm)
                m = jnp.max(mm, axis=1, keepdims=True)
                st[i] = (ss, m)
                on_scores(i, toks[i])

            def pv(i):
                ss, m = st[i]
                m = jnp.broadcast_to(m, (BQ, BQ))
                o = None
                l = None
                ts = []
                jla = JLA if fused else JLA_ONLY.get(i, JLA)
                la = LA2_LAST.get(i, LA2) if fused else LA1
                for j, s in enumerate(ss):
                    if j % JG == 0:
                        av = ts[j - jla] if j >= jla else anchor(clock[0] + (j // 4) * BQ - la)
                        if av is not None:
                            tok = pltpu.bitcast(_token(av), f32)
                            m = (m.reshape(BQ // 8, 8, BQ) + tok[None]).reshape(BQ, BQ)
                    p = jnp.exp2(s - m)
                    l = p if l is None else l + p
                    tk = take(clock[0] + (j // 4) * BQ) if j % 4 == 0 else None
                    pb = p.astype(bf16)
                    if tk is not None:
                        pb = _as_bf16(tie(pltpu.bitcast(pb, u32), tk))
                    t = jnp.dot(pb, ldp(v_s, j * BQ, (j + 1) * BQ), preferred_element_type=f32)
                    ts.append(t)
                    o = t if o is None else o + t
                for j, t in enumerate(ts):
                    marks.append((clock[0] + min(BQ * (j // 4 + 1), (i + 1) * BQ // 4), t))
                clock[0] += (i + 1) * BQ // 4
                o = o * _recip(jnp.sum(l, axis=1, keepdims=True))
                if fused:
                    o = o * g_s[i * BQ:(i + 1) * BQ, :]
                st[i] = o.astype(bf16)

            def outproj(i):
                r0 = i * BQ
                w = _as_bf16(wo_a[pl.ds(_mo(h * (D // 2), D // 2), D // 2), :])
                dst = acc if fused else acc1
                lhs = st[i]
                tk = take(clock[0])
                if tk is not None:
                    lhs = _as_bf16(tie(pltpu.bitcast(lhs, u32), tk))
                d = jnp.dot(lhs, w, preferred_element_type=f32)
                marks.append((clock[0] + BQ // 2, d[BQ // 2:BQ // 2 + 8]))
                marks.append((clock[0] + BQ, d[BQ - 8:BQ]))
                clock[0] += BQ
                a = d if first_head else dst[r0:r0 + BQ, :] + d
                dst[r0:r0 + BQ, :] = a
                if fused:
                    out_s[i * BQ:(i + 1) * BQ, :] = a.astype(bf16)
                    on_emit(i)

            out = []
            for kind, i, tk in (a_sched2 if fused else a_sched0 if first_head else a_sched1):
                hh = (h, 0) if kind[0] == "P" else (h + 1, 1)
                if kind in ("w", "G"):
                    fn = None
                elif kind[0] == "T":
                    t = "kqv".index(kind[1])
                    fn = functools.partial(proj, x_s if t == 1 else c_s, t, tmp_s.at[t], qscale if t == 1 else None,
                                           i, hh, tk)
                elif kind[0] == "C":
                    t = "kqv".index(kind[1])
                    fn = functools.partial(move, (k_s, q_s, v_s)[t], t)
                elif kind in ("Pk", "Nk"):
                    fn = functools.partial(proj, c_s, 0, k_s, None, i, hh, tk)
                elif kind in ("Pq", "Nq"):
                    fn = functools.partial(proj, x_s, 1, q_s, qscale, i, hh, tk)
                elif kind in ("Pv", "Nv"):
                    fn = functools.partial(proj, c_s, 2, v_s, None, i, hh, tk)
                elif kind == "S":
                    fn = functools.partial(scores, i)
                elif kind == "O":
                    fn = functools.partial(pv, i)
                else:
                    fn = functools.partial(outproj, i)
                out.append(((kind, i), fn))
            return out

        def unpack_b(p, t, c, tok):
            rows = pl.ds(c * (M // 4), M // 4)
            lo, hi = _unpack_pair_tok(st_b[_mod(p, 2), t, rows, :], tok)
            w_b[t * H + 2 * p, rows, :] = lo
            w_b[t * H + 2 * p + 1, rows, :] = hi

        gwv = {}

        def gate(h):
            if "gw" not in gwv:
                gwv["gw"] = gw_s[...].astype(f32).reshape(1, M)
            xg = _as_bf16(x_s[pl.ds(_mo(h * (BQ // 2), 8), BQ // 2), :]).astype(f32)
            g = jax.nn.sigmoid(jnp.sum(xg * gwv["gw"], axis=1, keepdims=True))
            gb = jnp.broadcast_to(g, (BQ, D))
            g_s[pl.ds(_mo(h * BQ, 8), BQ), :] = gb

        def a_head(h, first_head):
            if not isinstance(h, int):
                for cp in a_copies(h) + b_copies(h - 1):
                    cp.wait()

            nxt = [] if isinstance(h, int) else a_copies(_mod(h + 1, NP2)) + b_copies(h)

            def on_scores(i, tok):
                if 1 <= i <= 12 and not first_head:
                    unpack_b(h - 1, (i - 1) // 4, (i - 1) % 4, tok)

            if not first_head:
                gate(h)

            for n, (name, fn) in enumerate(a_tasks(h, False, on_scores, spar=h % 2 if isinstance(h, int) else None,
                                                   first_head=first_head)):
                if name[0] == "w":
                    for cp in name[1]:
                        named[cp].wait()
                elif name[0] == "G":
                    gate(h)
                else:
                    fn()
                if n == STARTPOS:
                    for cp in nxt:
                        cp.start()

        def a_body(h, carry):
            a_head(h, False)
            return carry

        a_head(0, True)
        cp_woa1.wait()
        cp_woa.start()
        jax.lax.fori_loop(1, SPLIT1, a_body, 0)
        cp_woa.wait()
        cp_wob.start()
        jax.lax.fori_loop(SPLIT1, H1, a_body, 0)

        cp_mem.wait()
        cp_wob.wait()

        def wb(t, h):
            return _as_bf16(w_b.bitcast(u32)[t * H + h])

        def wob(g):
            return _as_bf16(wo_b[g * GB * D // 2:(g + 1) * GB * D // 2, :])

        def tile4(g):
            return jnp.concatenate([g] * (M // D), axis=1)

        mem_s[...] = mem0_s[...].astype(f32)

        for cp in a_copies(0) + b_copies(H1 - 1):
            cp.wait()
        ztok = jnp.zeros((8, D), u32)
        for n in range(12):
            unpack_b(NP2 - 1, n // 4, n % 4, ztok)

        L = NM + SEG
        r80 = jax.lax.broadcasted_iota(jnp.int32, (2 * L, 2 * L), 0)
        c80 = jax.lax.broadcasted_iota(jnp.int32, (2 * L, 2 * L), 1)
        rhead = jnp.where(r80 < NM, 0, jnp.where(r80 < 2 * NM, 1, jnp.where(r80 < 2 * NM + SEG, 0, 1)))
        chead = jnp.where(c80 < L, 0, 1)
        rpos = jnp.where(r80 < 2 * NM, L - 1,
                         jnp.where(r80 < 2 * NM + SEG, r80 - 2 * NM + NM, r80 - 2 * NM - SEG + NM))
        cpos = jnp.where(c80 < L, c80, c80 - L)
        same = rhead == chead
        valid = jnp.logical_and(same, cpos <= rpos)
        fill = jnp.where(same, NEG, -3e38).astype(f32)

        def finalize(a0, n, z):
            acc[pl.ds(a0, n), :] += z + tile4(g_s[pl.ds(a0, n), :]) * (acc1[pl.ds(a0, n), :] - z)

        def b_step(step, get_xr, cur, stores, ox_parts, finish):
            v = {"z": None}
            memp, ps, om = {}, {}, {}

            def proj(h):
                if "lhs" not in v:
                    v["lhs"] = jnp.concatenate([mem_s[...], get_xr()], axis=0).astype(bf16)
                r = []
                for t in range(3):
                    y = jnp.dot(v["lhs"], wb(t, h), preferred_element_type=f32)
                    if t == 0:
                        y = y * qscale
                    c0 = (t * H + h) * D
                    for (y0, n, slot, d0) in stores:
                        qkv_s[slot, d0:d0 + n, c0:c0 + D] = y[y0:y0 + n]
                    r.append(y[:NM])
                memp[h] = r

            def scores(gg):
                for h0 in range(gg * GB, (gg + 1) * GB, 2):
                    h1 = h0 + 1

                    def xs(t, h):
                        return qkv_s[cur, :, (t * H + h) * D:(t * H + h + 1) * D]
                    q2 = jnp.concatenate([memp[h0][0], memp[h1][0], xs(0, h0), xs(0, h1)], axis=0).astype(bf16)
                    k2 = jnp.concatenate([memp[h0][1], xs(1, h0), memp[h1][1], xs(1, h1)], axis=0).astype(bf16)
                    v2 = jnp.concatenate([memp[h0][2], xs(2, h0), memp[h1][2], xs(2, h1)], axis=0).astype(bf16)
                    sc = jax.lax.dot_general(q2, k2, NT, preferred_element_type=f32)
                    sc = jnp.where(valid, sc, fill)
                    m = jnp.max(sc, axis=1, keepdims=True)
                    p = jnp.exp2(sc - m)
                    l = jnp.sum(p, axis=1, keepdims=True)
                    ps[h0] = (p.astype(bf16), _recip(l), v2)

            def pv(gg):
                for h0 in range(gg * GB, (gg + 1) * GB, 2):
                    h1 = h0 + 1
                    p, rl, v2 = ps.pop(h0)
                    o = jnp.dot(p, v2, preferred_element_type=f32) * rl
                    om[h0] = o[0:NM]
                    om[h1] = o[NM:2 * NM]
                    ox_s[cur, :, h0 * D:(h0 + 1) * D] = o[2 * NM:2 * NM + SEG]
                    ox_s[cur, :, h1 * D:(h1 + 1) * D] = o[2 * NM + SEG:]

            def oproj(gg):
                c0, c1 = gg * GB * D, (gg + 1) * GB * D
                parts = [jnp.concatenate([om[h] for h in range(gg * GB, (gg + 1) * GB)], axis=1)]
                parts += [ox_s[slot, r0:r1, c0:c1] for (slot, r0, r1) in ox_parts]
                lo = jnp.concatenate(parts, axis=0).astype(bf16)
                t = jnp.dot(lo, wob(gg), preferred_element_type=f32)
                v["z"] = t if v["z"] is None else v["z"] + t
                if gg == NG - 1:
                    mem_s[...] = v["z"][:NM].astype(bf16).astype(f32)
                    finish(v["z"][NM:])

            tasks = []
            for g in range(NG + 3):
                if g < NG:
                    for h in range(g * GB, (g + 1) * GB):
                        tasks.append(((step, "P", h), functools.partial(proj, h)))
                if 0 <= g - 1 < NG:
                    tasks.append(((step, "Sc", g - 1), functools.partial(scores, g - 1)))
                if 0 <= g - 2 < NG:
                    tasks.append(((step, "Pv", g - 2), functools.partial(pv, g - 2)))
                if 0 <= g - 3 < NG:
                    tasks.append(((step, "Op", g - 3), functools.partial(oproj, g - 3)))
                tasks.append(((step, "end", g), None))
            return tasks

        def b_pair(j, par):
            s0 = par * 2
            s1 = s0 + 1
            a0 = pl.multiple_of(j * 64, 64)
            v = {}

            def xn():
                if "xn" not in v:
                    v["xn"] = _as_bf16(x_s[pl.ds(pl.multiple_of(j * SEG, 8), SEG), :]).astype(f32)
                return v["xn"]

            ev = b_step(2 * par, lambda: xn()[0:40], s0, [(NM, SEG, s0, 0), (NM + SEG, NM, s1, 0)],
                        [(s0, 0, SEG - NM)],
                        lambda z: finalize(a0, 24, z))
            od = b_step(2 * par + 1, lambda: xn()[40:64], s1, [(NM, SEG - NM, s1, NM)],
                        [(s0, SEG - NM, SEG), (s1, 0, SEG)],
                        lambda z: finalize(pl.multiple_of(a0 + 24, 8), 40, z))
            return ev + od

        NI = H - H1
        bounds = [0] + [t + 1 for t in OSPLIT]
        assert bounds[-1] == NQ
        out_cp = [pltpu.make_async_copy(out_s.at[bounds[n] * BQ:bounds[n + 1] * BQ, :],
                                        out_hbm.at[bounds[n] * BQ:bounds[n + 1] * BQ, :], sem_out.at[n])
                  for n in range(len(bounds) - 1)]

        def f_body(i, carry):
            def on_emit(t):
                if t in OSPLIT:
                    @pl.when(i == NI - 1)
                    def _():
                        out_cp[OSPLIT.index(t)].start()

            at = a_tasks(H1 + i, True, lambda t, tok: None, on_emit)
            bt = b_pair(2 * i, 0) + b_pair(2 * i + 1, 1)
            for fn in _merge(at, bt):
                fn()
            return carry

        jax.lax.fori_loop(0, NI, f_body, 0)

        for cp in out_cp:
            cp.wait()

    scratch = [
        pltpu.VMEM((S // 2, M), u32),
        pltpu.VMEM((S // 2, M), u32),
        pltpu.VMEM((S, M), f32),
        pltpu.VMEM((S, M), f32),
        pltpu.VMEM((S, D), f32),
        pltpu.VMEM((S, D), bf16),
        pltpu.VMEM((S, D), bf16),
        pltpu.VMEM((S, D), bf16),
        pltpu.VMEM((NP2, 3, M, D), u32),
        pltpu.VMEM((HD // 2, M), u32),
        pltpu.VMEM((2, 3, M, D), u32),
        pltpu.VMEM((3 * H, M, D), bf16),
        pltpu.VMEM((HD // 2, M), u32),
        pltpu.VMEM((NM, M), bf16),
        pltpu.VMEM((M,), bf16),
        pltpu.VMEM((NM, M), f32),
        pltpu.VMEM((4, SEG, 3 * HD), f32),
        pltpu.VMEM((4, SEG, HD), f32),
        pltpu.VMEM((S, M), bf16),
        pltpu.VMEM((3, PCH, D), bf16),
        pltpu.VMEM((3, M // 2, D), u32),
        pltpu.SemaphoreType.DMA((4,)),
        pltpu.SemaphoreType.DMA((4,)),
        pltpu.SemaphoreType.DMA((4,)),
        pltpu.SemaphoreType.DMA((len(OSPLIT),)),
        pltpu.SemaphoreType.DMA((2 * NCH + 1,)),
        pltpu.SemaphoreType.DMA((3,)),
    ]
    return kernel, scratch


@functools.partial(jax.jit, static_argnames=("B_seg_len",))
def pallas_gated_mix__compressed_kv_cla__memory_aug_recurrent_mem_tr__prompt_kernel(
    A_x: jax.Array,
    A_c_kv: jax.Array,
    A_w_q: jax.Array,
    A_w_uk: jax.Array,
    A_w_uv: jax.Array,
    A_w_o: jax.Array,
    B_x: jax.Array,
    B_mem0: jax.Array,
    B_Wq: jax.Array,
    B_Wk: jax.Array,
    B_Wv: jax.Array,
    B_Wo: jax.Array,
    B_seg_len: int,
    gate_w: jax.Array,
):
    _, S, M = A_x.shape
    _, H, D = A_w_q.shape
    NM = B_mem0.shape[1]
    kernel, scratch = _make_kernel(S, M, H, D, NM, int(B_seg_len))
    any_spec = pl.BlockSpec(memory_space=pl.ANY)
    out = pl.pallas_call(
        kernel,
        out_shape=jax.ShapeDtypeStruct((S, M), bf16),
        in_specs=[any_spec] * 12,
        out_specs=any_spec,
        scratch_shapes=scratch,
        compiler_params=pltpu.CompilerParams(vmem_limit_bytes=100 * 1024 * 1024, disable_bounds_checks=True,
                                             disable_semaphore_checks=True),
    )(
        A_x.reshape(S, M), A_c_kv.reshape(S, M), A_w_q, A_w_uk, A_w_uv,
        A_w_o.reshape(H * D, M), B_mem0.reshape(NM, M),
        B_Wq, B_Wk, B_Wv, B_Wo.reshape(H * D, M), gate_w,
    )
    return out.reshape(1, S, M)
```

```python
import functools

import jax
import jax.numpy as jnp
import jax.experimental.pallas as pl
import jax.experimental.pallas.tpu as pltpu

bf16 = jnp.bfloat16
f32 = jnp.float32
u32 = jnp.uint32

LOG2E = 1.4426950408889634
NEG = -1e9 * LOG2E
NT = (((1,), (1,)), ((), ()))

BQ = 128
PCH = 512
GB = 4

JG = 4
JLA = 8
LA1 = 100000
LA2 = 256
MD2 = 448
JLA_A, LA_A, HALVED_A = {8: 11, 9: 7, 14: 12, 15: 12}, {11: 1024}, (14, 15)
JLA_F, LA_F, HALVED_F = {10: 7, 15: 10}, {14: 384, 15: 576}, (15,)
MMIN = 4
HALF = 256
SPLIT1 = 3
STARTPOS = 3
DORD = "gw wk c0a c0b wv wq x0 c1 x1 wo c2 x2 c3 x3 mem".split()
H0 = ("w:wk+c0a Pk0a Tk0a w:c0b+wv Pk0b Tk0b Pv0 Tv0 w:wq+x0+gw Pq0 G0 Tq0 S0 S1 O0 S2 O1 S3 O2 O3 "
      "w:c1 Pk1 Pv1 w:x1+wo Pq1 F0 F1 S4 F2 S5 O4 F3 S6 O5 F4 w:c2+x2 Pk2 S7 O6 F5 Pq2 O7 F6 Pv2 F7 S8 "
      "w:c3+x3 Pk3").split()
_MIDDLE = ("S3 O2 F1 S4 Pk2:2 O3 F2 S5 Pq2:3 O4 F3 S6 Pv2:4 O5 F4 S7 O6 F5 S8 Pk3:6 O7 F6 S9 Pq3:7 O8 F7 "
           "S10 Pv3:8 O9 F8 S11 O10 F9 S12 O11 F10 S13 O12 F11 S14 O13 F12 Nq0:14 S15 O14 F13 ")
A_ONLY = "Pk1 S0 S1 Pq1 O0 S2 Pv1 O1 F0 " + _MIDDLE + "Nk0:13 O15 F14 Nv0:15 F15"
A_FUSED = "S0 Pk1 S1 O0 Pq1 S2 O1 F0 Pv1 " + _MIDDLE + "O15 F14 F15 Nk0:13 Nv0:15"
MIDS = ((2, 5), (1, 3, 5), (2, 4, 6), (0, 2, 4, 6))
TSPLIT = (2, 5)
OSPLIT = (9, 13, 14, 15)


def _mo(x, m):
    return x if isinstance(x, int) else pl.multiple_of(x, m)


def _mod(x, n):
    assert n & (n - 1) == 0
    return x % n if isinstance(x, int) else jnp.bitwise_and(x, n - 1)


def _half(x):
    return x // 2 if isinstance(x, int) else jax.lax.shift_right_logical(x, 1)


def _as_bf16(words):
    return pltpu.bitcast(words, bf16)


def _recip(l):
    r = pl.reciprocal(l, approx=True)
    return r * (2.0 - l * r)


def _unpack_head(words, par):
    if isinstance(par, int):
        w = jnp.bitwise_and(words, jnp.uint32(0xFFFF0000)) if par else jnp.left_shift(words, jnp.uint32(16))
        return pltpu.bitcast(w, f32).astype(bf16)
    sh = ((1 - par) * 16).astype(u32)
    w = jnp.bitwise_and(jnp.left_shift(words, sh), jnp.uint32(0xFFFF0000))
    return pltpu.bitcast(w, f32).astype(bf16)


def _token(v):
    f = pltpu.bitcast(jnp.right_shift(pltpu.bitcast(v[0:8, 0:128], u32), jnp.uint32(2)), f32)
    return pltpu.bitcast(f - f, u32)


def _token_all(v):
    v3 = v.reshape(v.shape[0] // 8, 8, v.shape[1])
    n = v3.shape[0]
    parts = [v3[i] for i in range(n)]
    while len(parts) > 1:
        parts = [jnp.maximum(parts[i], parts[i + 1]) for i in range(0, len(parts), 2)]
    return _token(parts[0])


def _unpack_head_tok(words, par, tok):
    r, c = words.shape
    if isinstance(par, int):
        w3 = words.reshape(r // 8, 8, c)
        if par:
            w = jnp.bitwise_and(w3, jnp.bitwise_or(tok, jnp.uint32(0xFFFF0000))[None])
        else:
            w = jnp.left_shift(w3, (tok + jnp.uint32(16))[None])
        return pltpu.bitcast(w.reshape(r, c), f32).astype(bf16)
    sh = ((1 - par) * 16).astype(u32) + tok
    mask = jnp.bitwise_or(tok, jnp.uint32(0xFFFF0000))
    w = jnp.bitwise_and(jnp.left_shift(words.reshape(r // 8, 8, c), sh[None]), mask[None])
    return pltpu.bitcast(w.reshape(r, c), f32).astype(bf16)


def _unpack_pair_tok(words, tok):
    r, c = words.shape
    w3 = words.reshape(r // 8, 8, c)
    lo = jnp.left_shift(w3, (tok + jnp.uint32(16))[None])
    hi = jnp.bitwise_and(w3, jnp.bitwise_or(tok, jnp.uint32(0xFFFF0000))[None])
    return (pltpu.bitcast(lo.reshape(r, c), f32).astype(bf16),
            pltpu.bitcast(hi.reshape(r, c), f32).astype(bf16))


def _first_schedule(base):
    tk = {(k, i): t for k, i, t in base}
    head = []
    for s in H0:
        if s.startswith("w:"):
            head.append(("w", tuple(s[2:].split("+")), None))
        else:
            nm = (s[:-1], int(s[-1])) if s[0] in "SOFG" else (s[:2], int(s[2]) if len(s) == 3 else s[2:])
            head.append(nm + (tk.get(nm),))
    used = {(k, i) for k, i, _ in head}
    rest = [(k, i, t) for k, i, t in base if (k, i) not in used]
    rest = [("C" + k[1], i, t) if k[0] == "N" else (k, i, t) for k, i, t in rest]
    return head + rest


def _a_schedule(nq, bpc, fused):
    assert nq == 16 and bpc == 4
    out = []
    for s in (A_FUSED if fused else A_ONLY).split():
        name, _, tok = s.partition(":")
        n = 1 if name[0] in "SOF" else 2
        out.append((name[:n], int(name[n:]), int(tok) if tok else None))
    return out


def _units(a_tasks):
    units = []
    for name, fn in a_tasks:
        if name[0] == "S":
            units.append([])
        units[-1].append((name, fn))
    return units


def _merge(a_tasks, b_tasks):
    units = _units(a_tasks)
    plan = {}
    u = 0
    for step in range(4):
        for g in MIDS[step]:
            plan.setdefault((step, "end", g), []).extend(units[u])
            u += 1
        t = units[u]
        u += 1
        a, b = (1, 2) if step < 3 else TSPLIT
        plan[(step, "Sc", 7)] = t[0:a]
        plan[(step, "Pv", 7)] = t[a:b]
        plan[(step, "Op", 7)] = t[b:]
    assert u == len(units)
    out = []
    for name, fn in b_tasks:
        if fn is not None:
            out.append(fn)
        out += [f for _, f in plan.pop(name, [])]
    assert not plan, plan
    return out


def _make_kernel(S, M, H, D, NM, SEG):
    assert SEG == 32 and NM == 8 and D == 128 and S % PCH == 0 and H % 2 == 0 and H % GB == 0
    NQ = S // BQ
    NPAIR = S // (2 * SEG)
    NG = H // GB
    HD = H * D
    NCH = S // PCH
    H1 = H // 2
    NP2 = H // 2
    assert NPAIR == 2 * (H - H1) and NQ == H1 and NP2 == H1
    qscale = D ** -0.5 * LOG2E
    a_sched1 = _a_schedule(NQ, PCH // BQ, False)
    a_sched2 = _a_schedule(NQ, PCH // BQ, True)
    a_sched0 = _first_schedule(a_sched1)

    def kernel(x_hbm, c_hbm, wq_hbm, wk_hbm, wv_hbm, wo_hbm, mem0_hbm,
               bq_hbm, bk_hbm, bv_hbm, bo_hbm, gw_hbm, out_hbm,
               x_s, c_s, acc1, acc, g_s, q_s, k_s, v_s, st_a, wo_a, st_b, w_b, wo_b,
               mem0_s, gw_s, mem_s, qkv_s, ox_s, out_s, tmp_s, wu_s,
               sem_in, sem_a, sem_b, sem_out, sem_xc, sem_f):
        a_w_hbm = (wk_hbm, wq_hbm, wv_hbm)
        b_w_hbm = (bq_hbm, bk_hbm, bv_hbm)

        def a_copies(p, sem=sem_a):
            return [pltpu.make_async_copy(a_w_hbm[t].bitcast(u32).at[:, p, :], st_a.at[p, t],
                                          sem.at[t]) for t in range(3)]

        def b_copies(p):
            return [pltpu.make_async_copy(b_w_hbm[t].bitcast(u32).at[:, p, :], st_b.at[_mod(p, 2), t],
                                          sem_b.at[t]) for t in range(3)]

        cp_x = [pltpu.make_async_copy(x_hbm.bitcast(u32).at[c * (PCH // 2):(c + 1) * (PCH // 2), :],
                                      x_s.at[c * (PCH // 2):(c + 1) * (PCH // 2), :], sem_xc.at[c])
                for c in range(NCH)]
        cp_c = {c: pltpu.make_async_copy(c_hbm.bitcast(u32).at[c * (PCH // 2):(c + 1) * (PCH // 2), :],
                                         c_s.at[c * (PCH // 2):(c + 1) * (PCH // 2), :], sem_xc.at[NCH + c])
                for c in range(1, NCH)}
        cp_woa0 = pltpu.make_async_copy(wo_hbm.bitcast(u32).at[pl.ds(0, D), :], wo_a.at[pl.ds(0, D), :], sem_a.at[3])
        cp_woa1 = pltpu.make_async_copy(wo_hbm.bitcast(u32).at[D:2 * D, :], wo_a.at[D:2 * D, :], sem_in.at[3])
        cp_woa = pltpu.make_async_copy(wo_hbm.bitcast(u32).at[2 * D:HD // 2, :], wo_a.at[2 * D:HD // 2, :], sem_b.at[3])
        cp_wob = pltpu.make_async_copy(bo_hbm.bitcast(u32), wo_b, sem_in.at[2])
        cp_mem = pltpu.make_async_copy(mem0_hbm, mem0_s, sem_in.at[0])
        cp_gw = pltpu.make_async_copy(gw_hbm, gw_s, sem_in.at[1])

        first = a_copies(0, sem_f)
        named = {"gw": cp_gw, "wk": first[0], "wq": first[1], "wv": first[2], "wo": cp_woa0, "mem": cp_mem}
        named.update({"c%d" % c: cp_c[c] for c in range(1, NCH)})
        named.update({"x%d" % c: cp_x[c] for c in range(NCH)})
        named["c0a"] = pltpu.make_async_copy(c_hbm.bitcast(u32).at[0:HALF // 2, :], c_s.at[0:HALF // 2, :], sem_xc.at[NCH])
        named["c0b"] = pltpu.make_async_copy(c_hbm.bitcast(u32).at[HALF // 2:PCH // 2, :], c_s.at[HALF // 2:PCH // 2, :],
                                             sem_xc.at[2 * NCH])
        for nm in DORD:
            named[nm].start()
        for cp in a_copies(1) + b_copies(0) + [cp_woa1]:
            cp.start()
        acc[...] = jnp.zeros(acc.shape, f32)

        row = jax.lax.broadcasted_iota(jnp.int32, (BQ, BQ), 0)
        col = jax.lax.broadcasted_iota(jnp.int32, (BQ, BQ), 1)
        tri = col <= row

        def tie(words, tok, r=0):
            if tok is None:
                return words
            n, c = words.shape
            blk = words[r:r + 8]
            if c > 128:
                blk = jnp.concatenate([jnp.bitwise_or(blk[:, :128], tok), blk[:, 128:]], axis=1)
            else:
                blk = jnp.bitwise_or(blk, tok)
            parts = ([words[:r]] if r else []) + [blk] + ([words[r + 8:]] if r + 8 < n else [])
            return jnp.concatenate(parts, axis=0)

        def ldp(ref, r0, r1, tok=None):
            return _as_bf16(tie(ref.bitcast(u32)[r0 // 2:r1 // 2, :], tok))

        def a_tasks(h, fused, on_scores, on_emit=None, spar=None, first_head=False):
            st = {}
            toks = {}
            marks, clock, due = [], [0], []

            def take(time):
                tk = None
                for tm, v in [d for d in due if d[0] <= time]:
                    t = _token_all(v)
                    tk = t if tk is None else jnp.bitwise_or(tk, t)
                due[:] = [d for d in due if d[0] > time]
                return tk

            def anchor(time):
                best = None
                for tm, v in marks:
                    if tm <= time:
                        best = v
                return best

            def weight(t, hh, tk, keep):
                hh, nxt = hh
                if not fused and not first_head and not nxt:
                    return _as_bf16(wu_s[t])
                words = st_a[_mod(_half(hh), NP2), t]
                par = _mod(hh, 2) if spar is None else (spar + nxt) % 2
                if tk is None:
                    w = _unpack_head(words, par)
                else:
                    w = _unpack_head_tok(words, par, toks[tk])
                if nxt and keep and not fused:
                    wu_s[t] = pltpu.bitcast(w, u32)
                return w

            def proj(src, t, dst, sc, c, hh, tk):
                if isinstance(c, str):
                    r, n = (0, HALF) if c[1] == "a" else (HALF, PCH - HALF)
                else:
                    r, n = c * PCH, PCH
                w = weight(t, hh, tk, c != "0b")
                lhs = src[r // 2:(r + n) // 2, :]
                for rr in range(0, n, BQ):
                    lhs = tie(lhs, take(clock[0] + rr), rr // 2)
                y = jnp.dot(_as_bf16(lhs), w, preferred_element_type=f32)
                for rr in range(64, n, 64):
                    marks.append((clock[0] + rr, y[rr:rr + 8]))
                clock[0] += n
                if sc is not None:
                    y = y * sc
                dst[r:r + n, :] = y.astype(bf16)

            def move(dst, t):
                dst[0:PCH, :] = tmp_s[t]

            def scores(i):
                r0 = i * BQ
                qw = q_s.bitcast(u32)[r0 // 2:(r0 + BQ) // 2, :]
                ss = []
                mm = None
                for j in range(i + 1):
                    tk = take(clock[0] + (j // 4) * BQ) if j % 4 == 0 else None
                    s = jax.lax.dot_general(_as_bf16(tie(qw, tk)), ldp(k_s, j * BQ, (j + 1) * BQ), NT,
                                            preferred_element_type=f32)
                    marks.append((clock[0] + min(BQ * (j // 4 + 1), (i + 1) * BQ // 4), s))
                    if j == i:
                        s = jnp.where(tri, s, NEG)
                    mm = s if mm is None else jnp.maximum(mm, s)
                    if (j % 4 == 3 or j == i) and i >= MMIN and fused:
                        due.append((clock[0] + min(BQ * (j // 4 + 1), (i + 1) * BQ // 4) + MD2, mm))
                    ss.append(s)
                clock[0] += (i + 1) * BQ // 4
                toks[i] = _token(mm)
                m = jnp.max(mm, axis=1, keepdims=True)
                st[i] = (ss, m)
                on_scores(i, toks[i])

            def pv(i):
                ss, m = st[i]
                jla = (JLA_F if fused else JLA_A).get(i, JLA)
                la = LA_F.get(i, LA2) if fused else LA_A.get(i, LA1)
                n = BQ // 2 if i in (HALVED_F if fused else HALVED_A) else BQ
                outs = []
                for r0 in range(0, BQ, n):
                    c0 = clock[0] + (r0 // n) * ((i + 1) * n // 4)
                    mh = jnp.broadcast_to(m[r0:r0 + n], (n, BQ))
                    o = None
                    l = None
                    ts = []
                    for j, s in enumerate(ss):
                        tj = c0 + (j // 4) * n
                        if j % JG == 0:
                            av = ts[j - jla] if j >= jla else anchor(tj - la)
                            if av is not None:
                                tok = pltpu.bitcast(_token(av), f32)
                                mh = (mh.reshape(n // 8, 8, BQ) + tok[None]).reshape(n, BQ)
                        p = jnp.exp2(s[r0:r0 + n] - mh)
                        l = p if l is None else l + p
                        tk = take(tj) if j % 4 == 0 else None
                        pb = p.astype(bf16)
                        if tk is not None:
                            pb = _as_bf16(tie(pltpu.bitcast(pb, u32), tk))
                        t = jnp.dot(pb, ldp(v_s, j * BQ, (j + 1) * BQ), preferred_element_type=f32)
                        ts.append(t)
                        o = t if o is None else o + t
                    for j, t in enumerate(ts):
                        marks.append((c0 + min(n * (j // 4 + 1), (i + 1) * n // 4), t))
                    o = o * _recip(jnp.sum(l, axis=1, keepdims=True))
                    if fused:
                        o = o * g_s[i * BQ + r0:i * BQ + r0 + n, :]
                    outs.append(o.astype(bf16))
                clock[0] += (i + 1) * BQ // 4
                st[i] = outs[0] if n == BQ else jnp.concatenate(outs, axis=0)

            def outproj(i):
                r0 = i * BQ
                w = _as_bf16(wo_a[pl.ds(_mo(h * (D // 2), D // 2), D // 2), :])
                dst = acc if fused else acc1
                lhs = st[i]
                tk = take(clock[0])
                if tk is not None:
                    lhs = _as_bf16(tie(pltpu.bitcast(lhs, u32), tk))
                d = jnp.dot(lhs, w, preferred_element_type=f32)
                marks.append((clock[0] + BQ // 2, d[BQ // 2:BQ // 2 + 8]))
                marks.append((clock[0] + BQ, d[BQ - 8:BQ]))
                clock[0] += BQ
                a = d if first_head else dst[r0:r0 + BQ, :] + d
                dst[r0:r0 + BQ, :] = a
                if fused:
                    out_s[i * BQ:(i + 1) * BQ, :] = a.astype(bf16)
                    on_emit(i)

            out = []
            for kind, i, tk in (a_sched2 if fused else a_sched0 if first_head else a_sched1):
                hh = (h, 0) if kind[0] == "P" else (h + 1, 1)
                if kind in ("w", "G"):
                    fn = None
                elif kind[0] == "T":
                    t = "kqv".index(kind[1])
                    fn = functools.partial(proj, x_s if t == 1 else c_s, t, tmp_s.at[t], qscale if t == 1 else None,
                                           i, hh, tk)
                elif kind[0] == "C":
                    t = "kqv".index(kind[1])
                    fn = functools.partial(move, (k_s, q_s, v_s)[t], t)
                elif kind in ("Pk", "Nk"):
                    fn = functools.partial(proj, c_s, 0, k_s, None, i, hh, tk)
                elif kind in ("Pq", "Nq"):
                    fn = functools.partial(proj, x_s, 1, q_s, qscale, i, hh, tk)
                elif kind in ("Pv", "Nv"):
                    fn = functools.partial(proj, c_s, 2, v_s, None, i, hh, tk)
                elif kind == "S":
                    fn = functools.partial(scores, i)
                elif kind == "O":
                    fn = functools.partial(pv, i)
                else:
                    fn = functools.partial(outproj, i)
                out.append(((kind, i), fn))
            return out

        def unpack_b(p, t, c, tok):
            rows = pl.ds(c * (M // 4), M // 4)
            lo, hi = _unpack_pair_tok(st_b[_mod(p, 2), t, rows, :], tok)
            w_b[t * H + 2 * p, rows, :] = lo
            w_b[t * H + 2 * p + 1, rows, :] = hi

        gwv = {}

        def gate(h):
            if "gw" not in gwv:
                gwv["gw"] = gw_s[...].astype(f32).reshape(1, M)
            xg = _as_bf16(x_s[pl.ds(_mo(h * (BQ // 2), 8), BQ // 2), :]).astype(f32)
            g = jax.nn.sigmoid(jnp.sum(xg * gwv["gw"], axis=1, keepdims=True))
            gb = jnp.broadcast_to(g, (BQ, D))
            g_s[pl.ds(_mo(h * BQ, 8), BQ), :] = gb

        def a_head(h, first_head):
            if not isinstance(h, int):
                for cp in a_copies(h) + b_copies(h - 1):
                    cp.wait()

            nxt = [] if isinstance(h, int) else a_copies(_mod(h + 1, NP2)) + b_copies(h)

            def on_scores(i, tok):
                if 1 <= i <= 12 and not first_head:
                    unpack_b(h - 1, (i - 1) // 4, (i - 1) % 4, tok)

            if not first_head:
                gate(h)

            for n, (name, fn) in enumerate(a_tasks(h, False, on_scores, spar=h % 2 if isinstance(h, int) else None,
                                                   first_head=first_head)):
                if name[0] == "w":
                    for cp in name[1]:
                        named[cp].wait()
                elif name[0] == "G":
                    gate(h)
                else:
                    fn()
                if n == STARTPOS:
                    for cp in nxt:
                        cp.start()

        def a_body(h, carry):
            a_head(h, False)
            return carry

        a_head(0, True)
        cp_woa1.wait()
        cp_woa.start()
        jax.lax.fori_loop(1, SPLIT1, a_body, 0)
        cp_woa.wait()
        cp_wob.start()
        jax.lax.fori_loop(SPLIT1, H1, a_body, 0)

        cp_mem.wait()
        cp_wob.wait()

        def wb(t, h):
            return _as_bf16(w_b.bitcast(u32)[t * H + h])

        def wob(g):
            return _as_bf16(wo_b[g * GB * D // 2:(g + 1) * GB * D // 2, :])

        def tile4(g):
            return jnp.concatenate([g] * (M // D), axis=1)

        mem_s[...] = mem0_s[...].astype(f32)

        for cp in a_copies(0) + b_copies(H1 - 1):
            cp.wait()
        ztok = jnp.zeros((8, D), u32)
        for n in range(12):
            unpack_b(NP2 - 1, n // 4, n % 4, ztok)

        L = NM + SEG
        r80 = jax.lax.broadcasted_iota(jnp.int32, (2 * L, 2 * L), 0)
        c80 = jax.lax.broadcasted_iota(jnp.int32, (2 * L, 2 * L), 1)
        rhead = jnp.where(r80 < NM, 0, jnp.where(r80 < 2 * NM, 1, jnp.where(r80 < 2 * NM + SEG, 0, 1)))
        chead = jnp.where(c80 < L, 0, 1)
        rpos = jnp.where(r80 < 2 * NM, L - 1,
                         jnp.where(r80 < 2 * NM + SEG, r80 - 2 * NM + NM, r80 - 2 * NM - SEG + NM))
        cpos = jnp.where(c80 < L, c80, c80 - L)
        same = rhead == chead
        valid = jnp.logical_and(same, cpos <= rpos)
        fill = jnp.where(same, NEG, -3e38).astype(f32)

        def finalize(a0, n, z):
            acc[pl.ds(a0, n), :] += z + tile4(g_s[pl.ds(a0, n), :]) * (acc1[pl.ds(a0, n), :] - z)

        def b_step(step, get_xr, cur, stores, ox_parts, finish):
            v = {"z": None}
            memp, ps, om = {}, {}, {}

            def proj(h):
                if "lhs" not in v:
                    v["lhs"] = jnp.concatenate([mem_s[...], get_xr()], axis=0).astype(bf16)
                r = []
                for t in range(3):
                    y = jnp.dot(v["lhs"], wb(t, h), preferred_element_type=f32)
                    if t == 0:
                        y = y * qscale
                    c0 = (t * H + h) * D
                    for (y0, n, slot, d0) in stores:
                        qkv_s[slot, d0:d0 + n, c0:c0 + D] = y[y0:y0 + n]
                    r.append(y[:NM])
                memp[h] = r

            def scores(gg):
                for h0 in range(gg * GB, (gg + 1) * GB, 2):
                    h1 = h0 + 1

                    def xs(t, h):
                        return qkv_s[cur, :, (t * H + h) * D:(t * H + h + 1) * D]
                    q2 = jnp.concatenate([memp[h0][0], memp[h1][0], xs(0, h0), xs(0, h1)], axis=0).astype(bf16)
                    k2 = jnp.concatenate([memp[h0][1], xs(1, h0), memp[h1][1], xs(1, h1)], axis=0).astype(bf16)
                    v2 = jnp.concatenate([memp[h0][2], xs(2, h0), memp[h1][2], xs(2, h1)], axis=0).astype(bf16)
                    sc = jax.lax.dot_general(q2, k2, NT, preferred_element_type=f32)
                    sc = jnp.where(valid, sc, fill)
                    m = jnp.max(sc, axis=1, keepdims=True)
                    p = jnp.exp2(sc - m)
                    l = jnp.sum(p, axis=1, keepdims=True)
                    ps[h0] = (p.astype(bf16), _recip(l), v2)

            def pv(gg):
                for h0 in range(gg * GB, (gg + 1) * GB, 2):
                    h1 = h0 + 1
                    p, rl, v2 = ps.pop(h0)
                    o = jnp.dot(p, v2, preferred_element_type=f32) * rl
                    om[h0] = o[0:NM]
                    om[h1] = o[NM:2 * NM]
                    ox_s[cur, :, h0 * D:(h0 + 1) * D] = o[2 * NM:2 * NM + SEG]
                    ox_s[cur, :, h1 * D:(h1 + 1) * D] = o[2 * NM + SEG:]

            def oproj(gg):
                c0, c1 = gg * GB * D, (gg + 1) * GB * D
                parts = [jnp.concatenate([om[h] for h in range(gg * GB, (gg + 1) * GB)], axis=1)]
                parts += [ox_s[slot, r0:r1, c0:c1] for (slot, r0, r1) in ox_parts]
                lo = jnp.concatenate(parts, axis=0).astype(bf16)
                t = jnp.dot(lo, wob(gg), preferred_element_type=f32)
                v["z"] = t if v["z"] is None else v["z"] + t
                if gg == NG - 1:
                    mem_s[...] = v["z"][:NM].astype(bf16).astype(f32)
                    finish(v["z"][NM:])

            tasks = []
            for g in range(NG + 3):
                if g < NG:
                    for h in range(g * GB, (g + 1) * GB):
                        tasks.append(((step, "P", h), functools.partial(proj, h)))
                if 0 <= g - 1 < NG:
                    tasks.append(((step, "Sc", g - 1), functools.partial(scores, g - 1)))
                if 0 <= g - 2 < NG:
                    tasks.append(((step, "Pv", g - 2), functools.partial(pv, g - 2)))
                if 0 <= g - 3 < NG:
                    tasks.append(((step, "Op", g - 3), functools.partial(oproj, g - 3)))
                tasks.append(((step, "end", g), None))
            return tasks

        def b_pair(j, par):
            s0 = par * 2
            s1 = s0 + 1
            a0 = pl.multiple_of(j * 64, 64)
            v = {}

            def xn():
                if "xn" not in v:
                    v["xn"] = _as_bf16(x_s[pl.ds(pl.multiple_of(j * SEG, 8), SEG), :]).astype(f32)
                return v["xn"]

            ev = b_step(2 * par, lambda: xn()[0:40], s0, [(NM, SEG, s0, 0), (NM + SEG, NM, s1, 0)],
                        [(s0, 0, SEG - NM)],
                        lambda z: finalize(a0, 24, z))
            od = b_step(2 * par + 1, lambda: xn()[40:64], s1, [(NM, SEG - NM, s1, NM)],
                        [(s0, SEG - NM, SEG), (s1, 0, SEG)],
                        lambda z: finalize(pl.multiple_of(a0 + 24, 8), 40, z))
            return ev + od

        NI = H - H1
        bounds = [0] + [t + 1 for t in OSPLIT]
        assert bounds[-1] == NQ
        out_cp = [pltpu.make_async_copy(out_s.at[bounds[n] * BQ:bounds[n + 1] * BQ, :],
                                        out_hbm.at[bounds[n] * BQ:bounds[n + 1] * BQ, :], sem_out.at[n])
                  for n in range(len(bounds) - 1)]

        def f_body(i, carry):
            def on_emit(t):
                if t in OSPLIT:
                    @pl.when(i == NI - 1)
                    def _():
                        out_cp[OSPLIT.index(t)].start()

            at = a_tasks(H1 + i, True, lambda t, tok: None, on_emit)
            bt = b_pair(2 * i, 0) + b_pair(2 * i + 1, 1)
            for fn in _merge(at, bt):
                fn()
            return carry

        jax.lax.fori_loop(0, NI, f_body, 0)

        for cp in out_cp:
            cp.wait()

    scratch = [
        pltpu.VMEM((S // 2, M), u32),
        pltpu.VMEM((S // 2, M), u32),
        pltpu.VMEM((S, M), f32),
        pltpu.VMEM((S, M), f32),
        pltpu.VMEM((S, D), f32),
        pltpu.VMEM((S, D), bf16),
        pltpu.VMEM((S, D), bf16),
        pltpu.VMEM((S, D), bf16),
        pltpu.VMEM((NP2, 3, M, D), u32),
        pltpu.VMEM((HD // 2, M), u32),
        pltpu.VMEM((2, 3, M, D), u32),
        pltpu.VMEM((3 * H, M, D), bf16),
        pltpu.VMEM((HD // 2, M), u32),
        pltpu.VMEM((NM, M), bf16),
        pltpu.VMEM((M,), bf16),
        pltpu.VMEM((NM, M), f32),
        pltpu.VMEM((4, SEG, 3 * HD), f32),
        pltpu.VMEM((4, SEG, HD), f32),
        pltpu.VMEM((S, M), bf16),
        pltpu.VMEM((3, PCH, D), bf16),
        pltpu.VMEM((3, M // 2, D), u32),
        pltpu.SemaphoreType.DMA((4,)),
        pltpu.SemaphoreType.DMA((4,)),
        pltpu.SemaphoreType.DMA((4,)),
        pltpu.SemaphoreType.DMA((len(OSPLIT),)),
        pltpu.SemaphoreType.DMA((2 * NCH + 1,)),
        pltpu.SemaphoreType.DMA((3,)),
    ]
    return kernel, scratch


@functools.partial(jax.jit, static_argnames=("B_seg_len",))
def pallas_gated_mix__compressed_kv_cla__memory_aug_recurrent_mem_tr__prompt_kernel(
    A_x: jax.Array,
    A_c_kv: jax.Array,
    A_w_q: jax.Array,
    A_w_uk: jax.Array,
    A_w_uv: jax.Array,
    A_w_o: jax.Array,
    B_x: jax.Array,
    B_mem0: jax.Array,
    B_Wq: jax.Array,
    B_Wk: jax.Array,
    B_Wv: jax.Array,
    B_Wo: jax.Array,
    B_seg_len: int,
    gate_w: jax.Array,
):
    _, S, M = A_x.shape
    _, H, D = A_w_q.shape
    NM = B_mem0.shape[1]
    kernel, scratch = _make_kernel(S, M, H, D, NM, int(B_seg_len))
    any_spec = pl.BlockSpec(memory_space=pl.ANY)
    out = pl.pallas_call(
        kernel,
        out_shape=jax.ShapeDtypeStruct((S, M), bf16),
        in_specs=[any_spec] * 12,
        out_specs=any_spec,
        scratch_shapes=scratch,
        compiler_params=pltpu.CompilerParams(vmem_limit_bytes=100 * 1024 * 1024, disable_bounds_checks=True,
                                             disable_semaphore_checks=True),
    )(
        A_x.reshape(S, M), A_c_kv.reshape(S, M), A_w_q, A_w_uk, A_w_uv,
        A_w_o.reshape(H * D, M), B_mem0.reshape(NM, M),
        B_Wq, B_Wk, B_Wv, B_Wo.reshape(H * D, M), gate_w,
    )
    return out.reshape(1, S, M)
```

```python
import functools

import jax
import jax.numpy as jnp
import jax.experimental.pallas as pl
import jax.experimental.pallas.tpu as pltpu

bf16 = jnp.bfloat16
f32 = jnp.float32
u32 = jnp.uint32

LOG2E = 1.4426950408889634
NEG = -1e9 * LOG2E
NT = (((1,), (1,)), ((), ()))

BQ = 128
PCH = 512
GB = 4

JG = 4
JLA = 8
LA1 = 100000
LA2 = 256
MD2 = 448
JLA_A, LA_A, HALVED_A = {8: 11, 9: 7, 14: 10, 15: 10}, {11: 1024}, (14, 15)
JLA_F, LA_F, HALVED_F = {10: 7, 15: 10}, {14: 384, 15: 576}, (15,)
MMIN = 4
HALF = 256
SPLIT1 = 3
STARTPOS = 3
DORD = "gw wk c0a c0b wv wq x0 c1 x1 wo c2 x2 c3 x3 mem".split()
H0 = ("w:wk+c0a Pk0a Tk0a w:c0b+wv Pk0b Tk0b Pv0 Tv0 w:wq+x0+gw Pq0 G0 Tq0 S0 S1 O0 S2 O1 S3 O2 O3 "
      "w:c1 Pk1 Pv1 w:x1+wo Pq1 F0 F1 S4 F2 S5 O4 F3 S6 O5 F4 w:c2+x2 Pk2 S7 O6 F5 Pq2 O7 F6 Pv2 F7 S8 "
      "w:c3+x3 Pk3").split()
_MIDDLE = ("S3 O2 F1 S4 Pk2:2 O3 F2 S5 Pq2:3 O4 F3 S6 Pv2:4 O5 F4 S7 O6 F5 S8 Pk3:6 O7 F6 S9 Pq3:7 O8 F7 "
           "S10 Pv3:8 O9 F8 S11 O10 F9 S12 O11 F10 S13 O12 F11 S14 O13 F12 ")
A_ONLY = "Pk1 S0 S1 Pq1 O0 S2 Pv1 O1 F0 " + _MIDDLE + "Nq0:13 S15 O14 F13 Nk0:13 O15 F14 Nv0:13 F15"
A_FUSED = "S0 Pk1 S1 O0 Pq1 S2 O1 F0 Pv1 " + _MIDDLE + "Nq0:14 S15 O14 F13 O15 F14 F15 Nk0:13 Nv0:15"
MIDS = ((2, 5), (1, 3, 5), (2, 4, 6), (0, 2, 4, 6))
TSPLIT = (2, 5)
OSPLIT = (9, 13, 14, 15)


def _mo(x, m):
    return x if isinstance(x, int) else pl.multiple_of(x, m)


def _mod(x, n):
    assert n & (n - 1) == 0
    return x % n if isinstance(x, int) else jnp.bitwise_and(x, n - 1)


def _half(x):
    return x // 2 if isinstance(x, int) else jax.lax.shift_right_logical(x, 1)


def _as_bf16(words):
    return pltpu.bitcast(words, bf16)


def _recip(l):
    r = pl.reciprocal(l, approx=True)
    return r * (2.0 - l * r)


def _unpack_head(words, par):
    if isinstance(par, int):
        w = jnp.bitwise_and(words, jnp.uint32(0xFFFF0000)) if par else jnp.left_shift(words, jnp.uint32(16))
        return pltpu.bitcast(w, f32).astype(bf16)
    sh = ((1 - par) * 16).astype(u32)
    w = jnp.bitwise_and(jnp.left_shift(words, sh), jnp.uint32(0xFFFF0000))
    return pltpu.bitcast(w, f32).astype(bf16)


def _token(v):
    f = pltpu.bitcast(jnp.right_shift(pltpu.bitcast(v[0:8, 0:128], u32), jnp.uint32(2)), f32)
    return pltpu.bitcast(f - f, u32)


def _token_all(v):
    v3 = v.reshape(v.shape[0] // 8, 8, v.shape[1])
    n = v3.shape[0]
    parts = [v3[i] for i in range(n)]
    while len(parts) > 1:
        parts = [jnp.maximum(parts[i], parts[i + 1]) for i in range(0, len(parts), 2)]
    return _token(parts[0])


def _unpack_head_tok(words, par, tok):
    r, c = words.shape
    if isinstance(par, int):
        w3 = words.reshape(r // 8, 8, c)
        if par:
            w = jnp.bitwise_and(w3, jnp.bitwise_or(tok, jnp.uint32(0xFFFF0000))[None])
        else:
            w = jnp.left_shift(w3, (tok + jnp.uint32(16))[None])
        return pltpu.bitcast(w.reshape(r, c), f32).astype(bf16)
    sh = ((1 - par) * 16).astype(u32) + tok
    mask = jnp.bitwise_or(tok, jnp.uint32(0xFFFF0000))
    w = jnp.bitwise_and(jnp.left_shift(words.reshape(r // 8, 8, c), sh[None]), mask[None])
    return pltpu.bitcast(w.reshape(r, c), f32).astype(bf16)


def _unpack_pair_tok(words, tok):
    r, c = words.shape
    w3 = words.reshape(r // 8, 8, c)
    lo = jnp.left_shift(w3, (tok + jnp.uint32(16))[None])
    hi = jnp.bitwise_and(w3, jnp.bitwise_or(tok, jnp.uint32(0xFFFF0000))[None])
    return (pltpu.bitcast(lo.reshape(r, c), f32).astype(bf16),
            pltpu.bitcast(hi.reshape(r, c), f32).astype(bf16))


def _first_schedule(base):
    tk = {(k, i): t for k, i, t in base}
    head = []
    for s in H0:
        if s.startswith("w:"):
            head.append(("w", tuple(s[2:].split("+")), None))
        else:
            nm = (s[:-1], int(s[-1])) if s[0] in "SOFG" else (s[:2], int(s[2]) if len(s) == 3 else s[2:])
            head.append(nm + (tk.get(nm),))
    used = {(k, i) for k, i, _ in head}
    rest = [(k, i, t) for k, i, t in base if (k, i) not in used]
    rest = [("C" + k[1], i, t) if k[0] == "N" else (k, i, t) for k, i, t in rest]
    return head + rest


def _a_schedule(nq, bpc, fused):
    assert nq == 16 and bpc == 4
    out = []
    for s in (A_FUSED if fused else A_ONLY).split():
        name, _, tok = s.partition(":")
        n = 1 if name[0] in "SOF" else 2
        out.append((name[:n], int(name[n:]), int(tok) if tok else None))
    return out


def _units(a_tasks):
    units = []
    for name, fn in a_tasks:
        if name[0] == "S":
            units.append([])
        units[-1].append((name, fn))
    return units


def _merge(a_tasks, b_tasks):
    units = _units(a_tasks)
    plan = {}
    u = 0
    for step in range(4):
        for g in MIDS[step]:
            plan.setdefault((step, "end", g), []).extend(units[u])
            u += 1
        t = units[u]
        u += 1
        a, b = (1, 2) if step < 3 else TSPLIT
        plan[(step, "Sc", 7)] = t[0:a]
        plan[(step, "Pv", 7)] = t[a:b]
        plan[(step, "Op", 7)] = t[b:]
    assert u == len(units)
    out = []
    for name, fn in b_tasks:
        if fn is not None:
            out.append(fn)
        out += [f for _, f in plan.pop(name, [])]
    assert not plan, plan
    return out


def _make_kernel(S, M, H, D, NM, SEG):
    assert SEG == 32 and NM == 8 and D == 128 and S % PCH == 0 and H % 2 == 0 and H % GB == 0
    NQ = S // BQ
    NPAIR = S // (2 * SEG)
    NG = H // GB
    HD = H * D
    NCH = S // PCH
    H1 = H // 2
    NP2 = H // 2
    assert NPAIR == 2 * (H - H1) and NQ == H1 and NP2 == H1
    qscale = D ** -0.5 * LOG2E
    a_sched1 = _a_schedule(NQ, PCH // BQ, False)
    a_sched2 = _a_schedule(NQ, PCH // BQ, True)
    a_sched0 = _first_schedule(a_sched1)

    def kernel(x_hbm, c_hbm, wq_hbm, wk_hbm, wv_hbm, wo_hbm, mem0_hbm,
               bq_hbm, bk_hbm, bv_hbm, bo_hbm, gw_hbm, out_hbm,
               x_s, c_s, acc1, acc, g_s, q_s, k_s, v_s, st_a, wo_a, st_b, w_b, wo_b,
               mem0_s, gw_s, mem_s, qkv_s, ox_s, out_s, tmp_s, wu_s,
               sem_in, sem_a, sem_b, sem_out, sem_xc, sem_f):
        a_w_hbm = (wk_hbm, wq_hbm, wv_hbm)
        b_w_hbm = (bq_hbm, bk_hbm, bv_hbm)

        def a_copies(p, sem=sem_a):
            return [pltpu.make_async_copy(a_w_hbm[t].bitcast(u32).at[:, p, :], st_a.at[p, t],
                                          sem.at[t]) for t in range(3)]

        def b_copies(p):
            return [pltpu.make_async_copy(b_w_hbm[t].bitcast(u32).at[:, p, :], st_b.at[_mod(p, 2), t],
                                          sem_b.at[t]) for t in range(3)]

        cp_x = [pltpu.make_async_copy(x_hbm.bitcast(u32).at[c * (PCH // 2):(c + 1) * (PCH // 2), :],
                                      x_s.at[c * (PCH // 2):(c + 1) * (PCH // 2), :], sem_xc.at[c])
                for c in range(NCH)]
        cp_c = {c: pltpu.make_async_copy(c_hbm.bitcast(u32).at[c * (PCH // 2):(c + 1) * (PCH // 2), :],
                                         c_s.at[c * (PCH // 2):(c + 1) * (PCH // 2), :], sem_xc.at[NCH + c])
                for c in range(1, NCH)}
        cp_woa0 = pltpu.make_async_copy(wo_hbm.bitcast(u32).at[pl.ds(0, D), :], wo_a.at[pl.ds(0, D), :], sem_a.at[3])
        cp_woa1 = pltpu.make_async_copy(wo_hbm.bitcast(u32).at[D:2 * D, :], wo_a.at[D:2 * D, :], sem_in.at[3])
        cp_woa = pltpu.make_async_copy(wo_hbm.bitcast(u32).at[2 * D:HD // 2, :], wo_a.at[2 * D:HD // 2, :], sem_b.at[3])
        cp_wob = pltpu.make_async_copy(bo_hbm.bitcast(u32), wo_b, sem_in.at[2])
        cp_mem = pltpu.make_async_copy(mem0_hbm, mem0_s, sem_in.at[0])
        cp_gw = pltpu.make_async_copy(gw_hbm, gw_s, sem_in.at[1])

        first = a_copies(0, sem_f)
        named = {"gw": cp_gw, "wk": first[0], "wq": first[1], "wv": first[2], "wo": cp_woa0, "mem": cp_mem}
        named.update({"c%d" % c: cp_c[c] for c in range(1, NCH)})
        named.update({"x%d" % c: cp_x[c] for c in range(NCH)})
        named["c0a"] = pltpu.make_async_copy(c_hbm.bitcast(u32).at[0:HALF // 2, :], c_s.at[0:HALF // 2, :], sem_xc.at[NCH])
        named["c0b"] = pltpu.make_async_copy(c_hbm.bitcast(u32).at[HALF // 2:PCH // 2, :], c_s.at[HALF // 2:PCH // 2, :],
                                             sem_xc.at[2 * NCH])
        for nm in DORD:
            named[nm].start()
        for cp in a_copies(1) + b_copies(0) + [cp_woa1]:
            cp.start()
        acc[...] = jnp.zeros(acc.shape, f32)

        row = jax.lax.broadcasted_iota(jnp.int32, (BQ, BQ), 0)
        col = jax.lax.broadcasted_iota(jnp.int32, (BQ, BQ), 1)
        tri = col <= row

        def tie(words, tok, r=0):
            if tok is None:
                return words
            n, c = words.shape
            blk = words[r:r + 8]
            if c > 128:
                blk = jnp.concatenate([jnp.bitwise_or(blk[:, :128], tok), blk[:, 128:]], axis=1)
            else:
                blk = jnp.bitwise_or(blk, tok)
            parts = ([words[:r]] if r else []) + [blk] + ([words[r + 8:]] if r + 8 < n else [])
            return jnp.concatenate(parts, axis=0)

        def ldp(ref, r0, r1, tok=None):
            return _as_bf16(tie(ref.bitcast(u32)[r0 // 2:r1 // 2, :], tok))

        def a_tasks(h, fused, on_scores, on_emit=None, spar=None, first_head=False):
            st = {}
            toks = {}
            marks, clock, due = [], [0], []

            def take(time):
                tk = None
                for tm, v in [d for d in due if d[0] <= time]:
                    t = _token_all(v)
                    tk = t if tk is None else jnp.bitwise_or(tk, t)
                due[:] = [d for d in due if d[0] > time]
                return tk

            def anchor(time):
                best = None
                for tm, v in marks:
                    if tm <= time:
                        best = v
                return best

            def weight(t, hh, tk, keep):
                hh, nxt = hh
                if not fused and not first_head and not nxt:
                    return _as_bf16(wu_s[t])
                words = st_a[_mod(_half(hh), NP2), t]
                par = _mod(hh, 2) if spar is None else (spar + nxt) % 2
                if tk is None:
                    w = _unpack_head(words, par)
                else:
                    w = _unpack_head_tok(words, par, toks[tk])
                if nxt and keep and not fused:
                    wu_s[t] = pltpu.bitcast(w, u32)
                return w

            def proj(src, t, dst, sc, c, hh, tk):
                if isinstance(c, str):
                    r, n = (0, HALF) if c[1] == "a" else (HALF, PCH - HALF)
                else:
                    r, n = c * PCH, PCH
                w = weight(t, hh, tk, c != "0b")
                lhs = src[r // 2:(r + n) // 2, :]
                for rr in range(0, n, BQ):
                    lhs = tie(lhs, take(clock[0] + rr), rr // 2)
                y = jnp.dot(_as_bf16(lhs), w, preferred_element_type=f32)
                for rr in range(64, n, 64):
                    marks.append((clock[0] + rr, y[rr:rr + 8]))
                clock[0] += n
                if sc is not None:
                    y = y * sc
                dst[r:r + n, :] = y.astype(bf16)

            def move(dst, t):
                dst[0:PCH, :] = tmp_s[t]

            def scores(i):
                r0 = i * BQ
                qw = q_s.bitcast(u32)[r0 // 2:(r0 + BQ) // 2, :]
                ss = []
                mm = None
                for j in range(i + 1):
                    tk = take(clock[0] + (j // 4) * BQ) if j % 4 == 0 else None
                    s = jax.lax.dot_general(_as_bf16(tie(qw, tk)), ldp(k_s, j * BQ, (j + 1) * BQ), NT,
                                            preferred_element_type=f32)
                    marks.append((clock[0] + min(BQ * (j // 4 + 1), (i + 1) * BQ // 4), s))
                    if j == i:
                        s = jnp.where(tri, s, NEG)
                    mm = s if mm is None else jnp.maximum(mm, s)
                    if (j % 4 == 3 or j == i) and i >= MMIN and fused:
                        due.append((clock[0] + min(BQ * (j // 4 + 1), (i + 1) * BQ // 4) + MD2, mm))
                    ss.append(s)
                clock[0] += (i + 1) * BQ // 4
                toks[i] = _token(mm)
                m = jnp.max(mm, axis=1, keepdims=True)
                st[i] = (ss, m)
                on_scores(i, toks[i])

            def pv(i):
                ss, m = st[i]
                jla = (JLA_F if fused else JLA_A).get(i, JLA)
                la = LA_F.get(i, LA2) if fused else LA_A.get(i, LA1)
                n = BQ // 2 if i in (HALVED_F if fused else HALVED_A) else BQ
                outs = []
                for r0 in range(0, BQ, n):
                    c0 = clock[0] + (r0 // n) * ((i + 1) * n // 4)
                    mh = jnp.broadcast_to(m[r0:r0 + n], (n, BQ))
                    o = None
                    l = None
                    ts = []
                    for j, s in enumerate(ss):
                        tj = c0 + (j // 4) * n
                        if j % JG == 0:
                            av = ts[j - jla] if j >= jla else anchor(tj - la)
                            if av is not None:
                                tok = pltpu.bitcast(_token(av), f32)
                                mh = (mh.reshape(n // 8, 8, BQ) + tok[None]).reshape(n, BQ)
                        p = jnp.exp2(s[r0:r0 + n] - mh)
                        l = p if l is None else l + p
                        tk = take(tj) if j % 4 == 0 else None
                        pb = p.astype(bf16)
                        if tk is not None:
                            pb = _as_bf16(tie(pltpu.bitcast(pb, u32), tk))
                        t = jnp.dot(pb, ldp(v_s, j * BQ, (j + 1) * BQ), preferred_element_type=f32)
                        ts.append(t)
                        o = t if o is None else o + t
                    for j, t in enumerate(ts):
                        marks.append((c0 + min(n * (j // 4 + 1), (i + 1) * n // 4), t))
                    o = o * _recip(jnp.sum(l, axis=1, keepdims=True))
                    if fused:
                        o = o * g_s[i * BQ + r0:i * BQ + r0 + n, :]
                    outs.append(o.astype(bf16))
                clock[0] += (i + 1) * BQ // 4
                st[i] = outs[0] if n == BQ else jnp.concatenate(outs, axis=0)

            def outproj(i):
                r0 = i * BQ
                w = _as_bf16(wo_a[pl.ds(_mo(h * (D // 2), D // 2), D // 2), :])
                dst = acc if fused else acc1
                lhs = st[i]
                tk = take(clock[0])
                if tk is not None:
                    lhs = _as_bf16(tie(pltpu.bitcast(lhs, u32), tk))
                d = jnp.dot(lhs, w, preferred_element_type=f32)
                marks.append((clock[0] + BQ // 2, d[BQ // 2:BQ // 2 + 8]))
                marks.append((clock[0] + BQ, d[BQ - 8:BQ]))
                clock[0] += BQ
                a = d if first_head else dst[r0:r0 + BQ, :] + d
                dst[r0:r0 + BQ, :] = a
                if fused:
                    out_s[i * BQ:(i + 1) * BQ, :] = a.astype(bf16)
                    on_emit(i)

            out = []
            for kind, i, tk in (a_sched2 if fused else a_sched0 if first_head else a_sched1):
                hh = (h, 0) if kind[0] == "P" else (h + 1, 1)
                if kind in ("w", "G"):
                    fn = None
                elif kind[0] == "T":
                    t = "kqv".index(kind[1])
                    fn = functools.partial(proj, x_s if t == 1 else c_s, t, tmp_s.at[t], qscale if t == 1 else None,
                                           i, hh, tk)
                elif kind[0] == "C":
                    t = "kqv".index(kind[1])
                    fn = functools.partial(move, (k_s, q_s, v_s)[t], t)
                elif kind in ("Pk", "Nk"):
                    fn = functools.partial(proj, c_s, 0, k_s, None, i, hh, tk)
                elif kind in ("Pq", "Nq"):
                    fn = functools.partial(proj, x_s, 1, q_s, qscale, i, hh, tk)
                elif kind in ("Pv", "Nv"):
                    fn = functools.partial(proj, c_s, 2, v_s, None, i, hh, tk)
                elif kind == "S":
                    fn = functools.partial(scores, i)
                elif kind == "O":
                    fn = functools.partial(pv, i)
                else:
                    fn = functools.partial(outproj, i)
                out.append(((kind, i), fn))
            return out

        def unpack_b(p, t, c, tok):
            rows = pl.ds(c * (M // 4), M // 4)
            lo, hi = _unpack_pair_tok(st_b[_mod(p, 2), t, rows, :], tok)
            w_b[t * H + 2 * p, rows, :] = lo
            w_b[t * H + 2 * p + 1, rows, :] = hi

        gwv = {}

        def gate(h):
            if "gw" not in gwv:
                gwv["gw"] = gw_s[...].astype(f32).reshape(1, M)
            xg = _as_bf16(x_s[pl.ds(_mo(h * (BQ // 2), 8), BQ // 2), :]).astype(f32)
            g = jax.nn.sigmoid(jnp.sum(xg * gwv["gw"], axis=1, keepdims=True))
            gb = jnp.broadcast_to(g, (BQ, D))
            g_s[pl.ds(_mo(h * BQ, 8), BQ), :] = gb

        def a_head(h, first_head):
            if not isinstance(h, int):
                for cp in a_copies(h) + b_copies(h - 1):
                    cp.wait()

            nxt = [] if isinstance(h, int) else a_copies(_mod(h + 1, NP2)) + b_copies(h)

            def on_scores(i, tok):
                if 1 <= i <= 12 and not first_head:
                    unpack_b(h - 1, (i - 1) // 4, (i - 1) % 4, tok)

            if not first_head:
                gate(h)

            for n, (name, fn) in enumerate(a_tasks(h, False, on_scores, spar=h % 2 if isinstance(h, int) else None,
                                                   first_head=first_head)):
                if name[0] == "w":
                    for cp in name[1]:
                        named[cp].wait()
                elif name[0] == "G":
                    gate(h)
                else:
                    fn()
                if n == STARTPOS:
                    for cp in nxt:
                        cp.start()

        def a_body(h, carry):
            a_head(h, False)
            return carry

        a_head(0, True)
        cp_woa1.wait()
        cp_woa.start()
        jax.lax.fori_loop(1, SPLIT1, a_body, 0)
        cp_woa.wait()
        cp_wob.start()
        jax.lax.fori_loop(SPLIT1, H1, a_body, 0)

        cp_mem.wait()
        cp_wob.wait()

        def wb(t, h):
            return _as_bf16(w_b.bitcast(u32)[t * H + h])

        def wob(g):
            return _as_bf16(wo_b[g * GB * D // 2:(g + 1) * GB * D // 2, :])

        def tile4(g):
            return jnp.concatenate([g] * (M // D), axis=1)

        mem_s[...] = mem0_s[...].astype(f32)

        for cp in a_copies(0) + b_copies(H1 - 1):
            cp.wait()
        ztok = jnp.zeros((8, D), u32)
        for n in range(12):
            unpack_b(NP2 - 1, n // 4, n % 4, ztok)

        L = NM + SEG
        r80 = jax.lax.broadcasted_iota(jnp.int32, (2 * L, 2 * L), 0)
        c80 = jax.lax.broadcasted_iota(jnp.int32, (2 * L, 2 * L), 1)
        rhead = jnp.where(r80 < NM, 0, jnp.where(r80 < 2 * NM, 1, jnp.where(r80 < 2 * NM + SEG, 0, 1)))
        chead = jnp.where(c80 < L, 0, 1)
        rpos = jnp.where(r80 < 2 * NM, L - 1,
                         jnp.where(r80 < 2 * NM + SEG, r80 - 2 * NM + NM, r80 - 2 * NM - SEG + NM))
        cpos = jnp.where(c80 < L, c80, c80 - L)
        same = rhead == chead
        valid = jnp.logical_and(same, cpos <= rpos)
        fill = jnp.where(same, NEG, -3e38).astype(f32)

        def finalize(a0, n, z):
            acc[pl.ds(a0, n), :] += z + tile4(g_s[pl.ds(a0, n), :]) * (acc1[pl.ds(a0, n), :] - z)

        def b_step(step, get_xr, cur, stores, ox_parts, finish):
            v = {"z": None}
            memp, ps, om = {}, {}, {}

            def proj(h):
                if "lhs" not in v:
                    v["lhs"] = jnp.concatenate([mem_s[...], get_xr()], axis=0).astype(bf16)
                r = []
                for t in range(3):
                    y = jnp.dot(v["lhs"], wb(t, h), preferred_element_type=f32)
                    if t == 0:
                        y = y * qscale
                    c0 = (t * H + h) * D
                    for (y0, n, slot, d0) in stores:
                        qkv_s[slot, d0:d0 + n, c0:c0 + D] = y[y0:y0 + n]
                    r.append(y[:NM])
                memp[h] = r

            def scores(gg):
                for h0 in range(gg * GB, (gg + 1) * GB, 2):
                    h1 = h0 + 1

                    def xs(t, h):
                        return qkv_s[cur, :, (t * H + h) * D:(t * H + h + 1) * D]
                    q2 = jnp.concatenate([memp[h0][0], memp[h1][0], xs(0, h0), xs(0, h1)], axis=0).astype(bf16)
                    k2 = jnp.concatenate([memp[h0][1], xs(1, h0), memp[h1][1], xs(1, h1)], axis=0).astype(bf16)
                    v2 = jnp.concatenate([memp[h0][2], xs(2, h0), memp[h1][2], xs(2, h1)], axis=0).astype(bf16)
                    sc = jax.lax.dot_general(q2, k2, NT, preferred_element_type=f32)
                    sc = jnp.where(valid, sc, fill)
                    m = jnp.max(sc, axis=1, keepdims=True)
                    p = jnp.exp2(sc - m)
                    l = jnp.sum(p, axis=1, keepdims=True)
                    ps[h0] = (p.astype(bf16), _recip(l), v2)

            def pv(gg):
                for h0 in range(gg * GB, (gg + 1) * GB, 2):
                    h1 = h0 + 1
                    p, rl, v2 = ps.pop(h0)
                    o = jnp.dot(p, v2, preferred_element_type=f32) * rl
                    om[h0] = o[0:NM]
                    om[h1] = o[NM:2 * NM]
                    ox_s[cur, :, h0 * D:(h0 + 1) * D] = o[2 * NM:2 * NM + SEG]
                    ox_s[cur, :, h1 * D:(h1 + 1) * D] = o[2 * NM + SEG:]

            def oproj(gg):
                c0, c1 = gg * GB * D, (gg + 1) * GB * D
                parts = [jnp.concatenate([om[h] for h in range(gg * GB, (gg + 1) * GB)], axis=1)]
                parts += [ox_s[slot, r0:r1, c0:c1] for (slot, r0, r1) in ox_parts]
                lo = jnp.concatenate(parts, axis=0).astype(bf16)
                t = jnp.dot(lo, wob(gg), preferred_element_type=f32)
                v["z"] = t if v["z"] is None else v["z"] + t
                if gg == NG - 1:
                    mem_s[...] = v["z"][:NM].astype(bf16).astype(f32)
                    finish(v["z"][NM:])

            tasks = []
            for g in range(NG + 3):
                if g < NG:
                    for h in range(g * GB, (g + 1) * GB):
                        tasks.append(((step, "P", h), functools.partial(proj, h)))
                if 0 <= g - 1 < NG:
                    tasks.append(((step, "Sc", g - 1), functools.partial(scores, g - 1)))
                if 0 <= g - 2 < NG:
                    tasks.append(((step, "Pv", g - 2), functools.partial(pv, g - 2)))
                if 0 <= g - 3 < NG:
                    tasks.append(((step, "Op", g - 3), functools.partial(oproj, g - 3)))
                tasks.append(((step, "end", g), None))
            return tasks

        def b_pair(j, par):
            s0 = par * 2
            s1 = s0 + 1
            a0 = pl.multiple_of(j * 64, 64)
            v = {}

            def xn():
                if "xn" not in v:
                    v["xn"] = _as_bf16(x_s[pl.ds(pl.multiple_of(j * SEG, 8), SEG), :]).astype(f32)
                return v["xn"]

            ev = b_step(2 * par, lambda: xn()[0:40], s0, [(NM, SEG, s0, 0), (NM + SEG, NM, s1, 0)],
                        [(s0, 0, SEG - NM)],
                        lambda z: finalize(a0, 24, z))
            od = b_step(2 * par + 1, lambda: xn()[40:64], s1, [(NM, SEG - NM, s1, NM)],
                        [(s0, SEG - NM, SEG), (s1, 0, SEG)],
                        lambda z: finalize(pl.multiple_of(a0 + 24, 8), 40, z))
            return ev + od

        NI = H - H1
        bounds = [0] + [t + 1 for t in OSPLIT]
        assert bounds[-1] == NQ
        out_cp = [pltpu.make_async_copy(out_s.at[bounds[n] * BQ:bounds[n + 1] * BQ, :],
                                        out_hbm.at[bounds[n] * BQ:bounds[n + 1] * BQ, :], sem_out.at[n])
                  for n in range(len(bounds) - 1)]

        def f_body(i, carry):
            def on_emit(t):
                if t in OSPLIT:
                    @pl.when(i == NI - 1)
                    def _():
                        out_cp[OSPLIT.index(t)].start()

            at = a_tasks(H1 + i, True, lambda t, tok: None, on_emit)
            bt = b_pair(2 * i, 0) + b_pair(2 * i + 1, 1)
            for fn in _merge(at, bt):
                fn()
            return carry

        jax.lax.fori_loop(0, NI, f_body, 0)

        for cp in out_cp:
            cp.wait()

    scratch = [
        pltpu.VMEM((S // 2, M), u32),
        pltpu.VMEM((S // 2, M), u32),
        pltpu.VMEM((S, M), f32),
        pltpu.VMEM((S, M), f32),
        pltpu.VMEM((S, D), f32),
        pltpu.VMEM((S, D), bf16),
        pltpu.VMEM((S, D), bf16),
        pltpu.VMEM((S, D), bf16),
        pltpu.VMEM((NP2, 3, M, D), u32),
        pltpu.VMEM((HD // 2, M), u32),
        pltpu.VMEM((2, 3, M, D), u32),
        pltpu.VMEM((3 * H, M, D), bf16),
        pltpu.VMEM((HD // 2, M), u32),
        pltpu.VMEM((NM, M), bf16),
        pltpu.VMEM((M,), bf16),
        pltpu.VMEM((NM, M), f32),
        pltpu.VMEM((4, SEG, 3 * HD), f32),
        pltpu.VMEM((4, SEG, HD), f32),
        pltpu.VMEM((S, M), bf16),
        pltpu.VMEM((3, PCH, D), bf16),
        pltpu.VMEM((3, M // 2, D), u32),
        pltpu.SemaphoreType.DMA((4,)),
        pltpu.SemaphoreType.DMA((4,)),
        pltpu.SemaphoreType.DMA((4,)),
        pltpu.SemaphoreType.DMA((len(OSPLIT),)),
        pltpu.SemaphoreType.DMA((2 * NCH + 1,)),
        pltpu.SemaphoreType.DMA((3,)),
    ]
    return kernel, scratch


@functools.partial(jax.jit, static_argnames=("B_seg_len",))
def pallas_gated_mix__compressed_kv_cla__memory_aug_recurrent_mem_tr__prompt_kernel(
    A_x: jax.Array,
    A_c_kv: jax.Array,
    A_w_q: jax.Array,
    A_w_uk: jax.Array,
    A_w_uv: jax.Array,
    A_w_o: jax.Array,
    B_x: jax.Array,
    B_mem0: jax.Array,
    B_Wq: jax.Array,
    B_Wk: jax.Array,
    B_Wv: jax.Array,
    B_Wo: jax.Array,
    B_seg_len: int,
    gate_w: jax.Array,
):
    _, S, M = A_x.shape
    _, H, D = A_w_q.shape
    NM = B_mem0.shape[1]
    kernel, scratch = _make_kernel(S, M, H, D, NM, int(B_seg_len))
    any_spec = pl.BlockSpec(memory_space=pl.ANY)
    out = pl.pallas_call(
        kernel,
        out_shape=jax.ShapeDtypeStruct((S, M), bf16),
        in_specs=[any_spec] * 12,
        out_specs=any_spec,
        scratch_shapes=scratch,
        compiler_params=pltpu.CompilerParams(vmem_limit_bytes=100 * 1024 * 1024, disable_bounds_checks=True,
                                             disable_semaphore_checks=True),
    )(
        A_x.reshape(S, M), A_c_kv.reshape(S, M), A_w_q, A_w_uk, A_w_uv,
        A_w_o.reshape(H * D, M), B_mem0.reshape(NM, M),
        B_Wq, B_Wk, B_Wv, B_Wo.reshape(H * D, M), gate_w,
    )
    return out.reshape(1, S, M)
```
